```python
import jax
import jax.numpy as jnp

def _softmax(x, axis=-1):
    return jax.nn.softmax(x, axis=axis)
def _gelu(x):
    return jax.nn.gelu(x, approximate=True)
def _silu(x):
    return jax.nn.silu(x)
def _sigmoid(x):
    return jax.nn.sigmoid(x)
def _layernorm(x, axis=-1, eps=1e-5):
    m = jnp.mean(x, axis=axis, keepdims=True)
    v = jnp.var(x, axis=axis, keepdims=True)
    return (x - m) / jnp.sqrt(v + eps)
def _scatter_add(tgt, idx, src, axis=0):
    return tgt.at[idx].add(src)
def _segment_sum(src, seg, n):
    return jax.ops.segment_sum(src, seg, n)
class _Rng:
    def __init__(self, key):
        self._k = key
    def _next(self):
        self._k, sub = jax.random.split(self._k)
        return sub
    def normal(self, shape):
        return jax.random.normal(self._next(), shape, dtype=jnp.bfloat16)
    def randint(self, lo, hi, shape):
        return jax.random.randint(self._next(), shape, lo, hi, dtype=jnp.int32)
    def uniform(self, shape, lo=0.0, hi=1.0):
        return jax.random.uniform(self._next(), shape, jnp.bfloat16, lo, hi)
    def permutation(self, n):
        return jax.random.permutation(self._next(), n)


kernel_name = 'parallel_sum__linear_kernel_hedgehog__glu_gated_geglu__prompt'

def _fwd_setup_inputs():
    _rng = _Rng(jax.random.key(int.from_bytes(__import__("os").urandom(4), "little")))
    _w = (lambda a: (lambda t: t.astype(jnp.bfloat16) if jnp.issubdtype(t.dtype, jnp.floating) else t)(jnp.asarray(a)))
    def _A_setup():
        B, S, D, H = 1, 2048, 448, 16
        Dh = D // H
        return {
            "x": _w((lambda *s: _rng.normal(s) * 0.05)(B, S, D)),
            "wqkv": _w((lambda *s: _rng.normal(s) * 0.05)(D, 3 * D)),
            "w_phi": _w((lambda *s: _rng.normal(s) * 0.05)(H, Dh, Dh) * (Dh ** -0.5)),
            "wo": _w((lambda *s: _rng.normal(s) * 0.05)(D, D)),
        }
    _A_in = _A_setup()

    def _B_setup():
        B, S, Dm, Df = 1, 2048, 448, 1792
        return {
            "x": _w((lambda *s: _rng.normal(s) * 0.05)(B, S, Dm)),
            "w_gate": _w((lambda *s: _rng.normal(s) * 0.05)(Dm, Df) * (Dm ** -0.5)),
            "w_up": _w((lambda *s: _rng.normal(s) * 0.05)(Dm, Df) * (Dm ** -0.5)),
            "w_down": _w((lambda *s: _rng.normal(s) * 0.05)(Df, Dm) * (Df ** -0.5)),
        }
    _B_in = _B_setup()

    return {
        "A_x": _A_in["x"],
        "A_wqkv": _A_in["wqkv"],
        "A_w_phi": _A_in["w_phi"],
        "A_wo": _A_in["wo"],
        "B_x": _B_in["x"],
        "B_w_gate": _B_in["w_gate"],
        "B_w_up": _B_in["w_up"],
        "B_w_down": _B_in["w_down"],
    }

def _fwd_reference(A_x, A_wqkv, A_w_phi, A_wo, B_x, B_w_gate, B_w_up, B_w_down):
    def _A_ref(x, wqkv, w_phi, wo):
        B, S, D = x.shape
        H = 16; Dh = D // H
        qkv = (lambda x, *d: x.transpose(*d))((x @ wqkv).reshape(B, S, 3, H, Dh), 2, 0, 3, 1, 4)
        q, k, v = qkv[0], qkv[1], qkv[2]
        pq = jnp.einsum("bhsd,hdf->bhsf", q, w_phi)
        pk = jnp.einsum("bhsd,hdf->bhsf", k, w_phi)
        phi_q = jnp.concatenate([_softmax(pq, axis=-1), _softmax(-pq, axis=-1)], axis=-1)
        phi_k = jnp.concatenate([_softmax(pk, axis=-1), _softmax(-pk, axis=-1)], axis=-1)
        kv = jnp.einsum("bhsf,bhsd->bhfd", phi_k, v)
        z  = jnp.einsum("bhsf->bhf", phi_k)
        num = jnp.einsum("bhqf,bhfd->bhqd", phi_q, kv)
        den = jnp.einsum("bhqf,bhf->bhq", phi_q, z)[..., None] + 1e-6
        o = num / den
        return (lambda x, *d: x.transpose(*d))(o, 0, 2, 1, 3).reshape(B, S, D) @ wo

    def _B_ref(x, w_gate, w_up, w_down):
        g = jnp.einsum("bsd,df->bsf", x, w_gate)
        u = jnp.einsum("bsd,df->bsf", x, w_up)
        h = _gelu(g) * u
        return jnp.einsum("bsf,fd->bsd", h, w_down)

    x = A_x
    xn = _layernorm(x, axis=-1)
    return x + _A_ref(xn, A_wqkv, A_w_phi, A_wo) + _B_ref(xn, B_w_gate, B_w_up, B_w_down)


def setup_inputs():
    _inp = _fwd_setup_inputs()
    _gk = jax.random.fold_in(jax.random.key(int.from_bytes(__import__("os").urandom(4), "little")), 2**31 - 1)
    _shapes = [[1, 2048, 448]]
    _dtypes = ['bfloat16']
    _gks = jax.random.split(_gk, len(_shapes))
    _gs = [jax.random.normal(k, s, dtype=jnp.dtype(d)) * 0.05 for k, s, d in zip(_gks, _shapes, _dtypes)]
    _inp["grad_out"] = _gs[0]
    return _inp

def reference(A_x, A_wqkv, A_w_phi, A_wo, B_w_gate, B_w_up, B_w_down, B_x, grad_out):
    _const = dict(B_x=B_x)
    def _f(*_d):
        return _fwd_reference(**{'A_x': _d[0], 'A_wqkv': _d[1], 'A_w_phi': _d[2], 'A_wo': _d[3], 'B_w_gate': _d[4], 'B_w_up': _d[5], 'B_w_down': _d[6], **_const})
    _out, _vjp = jax.vjp(_f, A_x, A_wqkv, A_w_phi, A_wo, B_w_gate, B_w_up, B_w_down)
    _grads = _vjp(grad_out)
    _out0 = jnp.asarray(_out)
    return (_out0, *[jnp.asarray(_g) for _g in _grads])
```

```python
import functools
import math

import jax
import jax.numpy as jnp
from jax import lax
import jax.experimental.pallas as pl
import jax.experimental.pallas.tpu as pltpu

S, D, H, DH, DF = 2048, 448, 16, 28, 1792
NP = H // 2
PR = 2 * DH
PF = 2 * PR
PE = PR + 8
NG = H // 4
TS = 256
NT = S // TS
FC = 256
MLP_SPLIT = (512, 768, 512)
LN_EPS = 1e-5
DEN_EPS = 1e-6
C0 = math.sqrt(2.0 / math.pi)
C1 = 0.044715
F32, BF16 = jnp.float32, jnp.bfloat16


def _nn(a, b):
    return lax.dot_general(a, b, (((1,), (0,)), ((), ())), preferred_element_type=F32)


def _nt(a, b):
    return lax.dot_general(a, b, (((1,), (1,)), ((), ())), preferred_element_type=F32)


def _tn(a, b):
    return lax.dot_general(a, b, (((0,), (0,)), ((), ())), preferred_element_type=F32)


def _tree(op, xs):
    xs = list(xs)
    while len(xs) > 1:
        nxt = [op(xs[i], xs[i + 1]) for i in range(0, len(xs) - 1, 2)]
        if len(xs) % 2:
            nxt.append(xs[-1])
        xs = nxt
    return xs[0]


def _rows8(a):
    return [a[8 * i:8 * i + 8] for i in range(a.shape[0] // 8)]


def _pair_reduce(op, rows):
    v = _tree(op, rows)
    v = op(v, pltpu.roll(v, 2, 0))
    return op(v, pltpu.roll(v, 4, 0))


def _softmax_pair(p):
    rows = _rows8(p)
    mx = _pair_reduce(jnp.maximum, rows)
    mn = _pair_reduce(jnp.minimum, rows)
    ep = [jnp.exp(r - mx) for r in rows]
    en = [jnp.exp(mn - r) for r in rows]
    rp = 1.0 / _pair_reduce(jnp.add, ep)
    rn = 1.0 / _pair_reduce(jnp.add, en)
    return jnp.concatenate([e * rp for e in ep] + [e * rn for e in en], axis=0)


def _softmax_pair_bwd(phi, dphi):
    pr, dr = _rows8(phi), _rows8(dphi)
    t = [a * b for a, b in zip(pr, dr)]
    sp = _pair_reduce(jnp.add, t[:7])
    sn = _pair_reduce(jnp.add, t[7:])
    out = [(t[i] - t[7 + i]) - (pr[i] * sp - pr[7 + i] * sn) for i in range(7)]
    return jnp.concatenate(out, axis=0)


def _acc(ref, idx, first, val):
    new = jnp.where(first, 0.0, ref[idx]) + val
    ref[idx] = new
    return new


def _kernel(xT_h, wqkv_h, wphi_h, wo_h, wg_h, wu_h, wdT_h, dyT_h,
            outT_h, dxT_h, dwqkv_h, dwphi_h, dwo_h, dwg_h, dwu_h, dwdT_h,
            xT_s, dyT_s, xnT_s, xn_s, dy_s, rstd_s,
            wqkv_s, wphi_s, wo_s, wg_s, wu_s, wdT_s,
            wqkT_s, bd_s, wpqT_s, wpkvT_s, wpq_s, wpkv_s, woT_s, tmpa_s, tmpb_s,
            phik_s, vext_s, kv_acc, dkv_acc, kvT_s, kv_s,
            out_acc, dxn_acc, dwg_acc, dwu_acc, dwd_acc, gq_acc, gkv_acc, dwo_acc,
            out_st, dx_st, dwqkv_st, dwphi_st, dwo_st, dwg_st, dwu_st, dwd_st,
            sem_w, sem_x, sem_dy, sem_mlp, sem_out, sem_dx, sem_ow, sem_omlp):
    cols = []
    a = 0
    for w in MLP_SPLIT:
        cols.append((a, a + w))
        a += w

    def x_copy(i):
        return pltpu.make_async_copy(xT_h.at[:, pl.ds(i * TS, TS)], xT_s.at[i], sem_x.at[i])

    def dy_copy(i):
        return pltpu.make_async_copy(dyT_h.at[:, pl.ds(i * TS, TS)], dyT_s.at[i], sem_dy.at[i])

    def mlp_in(p):
        lo, hi = cols[p]
        return [pltpu.make_async_copy(src.at[:, pl.ds(lo, hi - lo)], dst.at[:, pl.ds(lo, hi - lo)],
                                      sem_mlp.at[3 * p + k])
                for k, (src, dst) in enumerate(((wg_h, wg_s), (wu_h, wu_s), (wdT_h, wdT_s)))]

    def mlp_out(p):
        lo, hi = cols[p]
        return [pltpu.make_async_copy(src.at[:, pl.ds(lo, hi - lo)], dst.at[:, pl.ds(lo, hi - lo)],
                                      sem_omlp.at[3 * p + k])
                for k, (src, dst) in enumerate(((dwg_st, dwg_h), (dwu_st, dwu_h), (dwd_st, dwdT_h)))]

    def out_copy(i):
        return pltpu.make_async_copy(out_st.at[i], outT_h.at[:, pl.ds(i * TS, TS)], sem_out.at[i])

    def dx_copy(i):
        return pltpu.make_async_copy(dx_st.at[i], dxT_h.at[:, pl.ds(i * TS, TS)], sem_dx.at[i])

    c_wphi = pltpu.make_async_copy(wphi_h, wphi_s, sem_w.at[0])
    c_wqkv = pltpu.make_async_copy(wqkv_h, wqkv_s, sem_w.at[1])
    c_wo = pltpu.make_async_copy(wo_h, wo_s, sem_w.at[2])
    c_dwqkv = pltpu.make_async_copy(dwqkv_st, dwqkv_h, sem_ow.at[0])
    c_dwphi = pltpu.make_async_copy(dwphi_st, dwphi_h, sem_ow.at[1])
    c_dwo = pltpu.make_async_copy(dwo_st, dwo_h, sem_ow.at[2])

    c_wphi.start()
    c_wqkv.start()
    x_copy(0).start()
    dy_copy(0).start()
    for c in mlp_in(0):
        c.start()
    for i in range(1, NT):
        x_copy(i).start()
        dy_copy(i).start()
    c_wo.start()
    for p in (1, 2):
        for c in mlp_in(p):
            c.start()

    def head_mask(shape, row_head):
        col = lax.broadcasted_iota(jnp.int32, shape, 1)
        return row_head == 2 * (col >= PR).astype(jnp.int32) + (col & 1)

    r112 = lax.broadcasted_iota(jnp.int32, (PF, PF), 0)
    bd_mask = head_mask((PF, PF), (r112 >= DH).astype(jnp.int32) + (r112 >= 2 * DH).astype(jnp.int32)
                        + (r112 >= 3 * DH).astype(jnp.int32))
    sel_c = lax.broadcasted_iota(jnp.int32, (DH, PF), 1)
    sel_r = lax.broadcasted_iota(jnp.int32, (DH, PF), 0)
    sel = jnp.where(((sel_c - PR * (sel_c >= PR).astype(jnp.int32)) >> 1) == sel_r, 1.0, 0.0).astype(BF16)

    c_wphi.wait()
    tmpa_s[...] = wphi_s[...].astype(F32)
    for d in range(DH):
        tmpb_s[pl.ds(d, H, stride=DH), :] = tmpa_s[H * d:H * d + H, :]
    expand = _nn(tmpb_s[...].astype(BF16), sel)
    for g in range(NG):
        bd_s[PF * g:PF * g + PF, :] = jnp.where(bd_mask, expand[PF * g:PF * g + PF], 0.0).astype(BF16)

    c_wqkv.wait()
    wqkT_s[...] = wqkv_s[:, 0:2 * D].T
    wpkvT_s[0:D, :] = wqkv_s[:, 2 * D:3 * D].T
    for g in range(NG):
        bd = bd_s[PF * g:PF * g + PF, :]
        wpqT_s[PF * g:PF * g + PF, :] = _tn(bd, wqkT_s[PF * g:PF * g + PF, :]).astype(BF16)
        wpkvT_s[D + PF * g:D + PF * g + PF, :] = _tn(bd, wqkT_s[D + PF * g:D + PF * g + PF, :]).astype(BF16)
    wpq_s[...] = wpqT_s[...].T
    wpkv_s[...] = wpkvT_s[...].T

    def mlp(i, p, first):
        lo, hi = cols[p]
        out_p, dxn_p = None, None
        for a in range(lo, hi, FC):
            cs = slice(a, min(a + FC, hi))
            xn = xn_s[i]
            g = _nn(xn, wg_s[:, cs])
            u = _nn(xn, wu_s[:, cs])
            dh = _nn(dy_s[i], wdT_s[:, cs])
            g2 = g * g
            s = 0.5 * jnp.tanh(g * (C0 + (C0 * C1) * g2)) + 0.5
            gelu = g * s
            dgelu = s + gelu * (1.0 - s) * (2.0 * C0 + (6.0 * C0 * C1) * g2)
            h = (gelu * u).astype(BF16)
            du = (dh * gelu).astype(BF16)
            dg = (dh * u * dgelu).astype(BF16)
            o = _nt(wdT_s[:, cs], h)
            dx = _nt(wg_s[:, cs], dg) + _nt(wu_s[:, cs], du)
            out_p = o if out_p is None else out_p + o
            dxn_p = dx if dxn_p is None else dxn_p + dx
            idx = (slice(None), cs)
            dwg_st[idx] = _acc(dwg_acc, idx, first, _nn(xnT_s[i], dg)).astype(BF16)
            dwu_st[idx] = _acc(dwu_acc, idx, first, _nn(xnT_s[i], du)).astype(BF16)
            dwd_st[idx] = _acc(dwd_acc, idx, first, _nn(dyT_s[i], h)).astype(BF16)
        return out_p, dxn_p

    r64 = lax.broadcasted_iota(jnp.int32, (PE, PF), 0)
    c64 = lax.broadcasted_iota(jnp.int32, (PE, PF), 1)
    kv_row_head = jnp.where(r64 < PR, (r64 >= DH).astype(jnp.int32), (r64 >= PR + 4).astype(jnp.int32))

    def finalize_kv(acc):
        for c in range(NP):
            m = jnp.where(kv_row_head == (c64 & 1), acc[c], 0.0)
            kvT_s[c] = m.astype(BF16)
            kv_s[c] = m.T.astype(BF16)

    for c in mlp_in(0):
        c.wait()

    def phase1(i, carry):
        first = i == 0
        x_copy(i).wait()
        dy_copy(i).wait()
        x32 = xT_s[i].astype(F32)
        mean = jnp.sum(x32, axis=0, keepdims=True) * (1.0 / D)
        xc = x32 - mean
        var = jnp.sum(xc * xc, axis=0, keepdims=True) * (1.0 / D)
        rstd = lax.rsqrt(var + LN_EPS)
        xnT = (xc * rstd).astype(BF16)
        rstd_s[i] = jnp.broadcast_to(rstd, (8, TS))
        xnT_s[i] = xnT
        xn_s[i] = xnT.T
        dy_s[i] = dyT_s[i].T

        pkv = _nn(wpkvT_s[...], xnT)
        ones = jnp.ones((8, TS), F32)
        for c in range(NP):
            phik = _softmax_pair(pkv[D + PR * c:D + PR * c + PR]).astype(BF16)
            phik_s[i, PF * c:PF * c + PF, :] = phik
            vext = jnp.concatenate([pkv[PR * c:PR * c + PR], ones], axis=0).astype(BF16)
            vext_s[i, PE * c:PE * c + PE, :] = vext
            _acc(kv_acc, c, first, _nt(vext, phik))

        o, dx = mlp(i, 0, first)
        out_acc[i] = xT_s[i].astype(F32) + o
        dxn_acc[i] = dx
        return carry

    lax.fori_loop(0, NT, phase1, 0)
    for c in mlp_out(0):
        c.start()
    finalize_kv(kv_acc)
    c_wo.wait()
    woT_s[...] = wo_s[...].T
    for c in mlp_in(1):
        c.wait()

    sub = lax.broadcasted_iota(jnp.int32, (8, TS), 0)
    lo4 = sub < 4

    def phase2(i, carry):
        first = i == 0
        pq = _nn(wpqT_s[...], xnT_s[i])
        doT = _nn(wo_s[...], dyT_s[i])
        o_all, dp_all = [], []
        for c in range(NP):
            phi = _softmax_pair(pq[PR * c:PR * c + PR])
            phib = phi.astype(BF16)
            ne = _rows8(_nn(kvT_s[c], phib))
            r = 1.0 / (ne[7] + DEN_EPS)
            rr = pltpu.roll(r, 4, 0)
            ra = jnp.where(lo4, r, rr)
            rb = jnp.where(lo4, rr, r)
            rs = [ra, ra, ra, r, rb, rb, rb]
            o = [n * w for n, w in zip(ne[:7], rs)]
            dnum = [n * w for n, w in zip(_rows8(doT[PR * c:PR * c + PR]), rs)]
            t = [a * b for a, b in zip(dnum, o)]
            sa = t[0] + t[1] + t[2]
            sb = t[4] + t[5] + t[6]
            e = jnp.where(lo4, sa, sb) + pltpu.roll(jnp.where(lo4, sb, sa), 4, 0) + t[3]
            dne = jnp.concatenate(dnum + [-e], axis=0).astype(BF16)
            _acc(dkv_acc, c, first, _nt(dne, phib))
            dphi = _nn(kv_s[c], dne)
            dp_all.append(_softmax_pair_bwd(phi, dphi))
            o_all.extend(o)
        oT = jnp.concatenate(o_all, axis=0).astype(BF16)
        dpq = jnp.concatenate(dp_all, axis=0).astype(BF16)
        full = (slice(None), slice(None))
        dwo_st[...] = _acc(dwo_acc, full, first, _nn(oT, dy_s[i])).astype(BF16)
        _acc(gq_acc, full, first, _nn(dpq, xn_s[i]))

        o, dx = mlp(i, 1, first)
        out_acc[i] += o + _nn(woT_s[...], oT)
        dxn_acc[i] += dx + _nn(wpq_s[...], dpq)
        return carry

    lax.fori_loop(0, NT, phase2, 0)
    for c in mlp_out(1):
        c.start()
    c_dwo.start()
    finalize_kv(dkv_acc)
    for c in mlp_in(2):
        c.wait()

    def phase3(i, carry):
        first = i == 0
        dv_all, dp_all = [], []
        for c in range(NP):
            phik = phik_s[i, PF * c:PF * c + PF, :]
            dphik = _nn(kv_s[c], vext_s[i, PE * c:PE * c + PE, :])
            dv_all.append(_nn(kvT_s[c], phik)[0:PR])
            dp_all.append(_softmax_pair_bwd(phik.astype(F32), dphik))
        dpkv = jnp.concatenate(dv_all + dp_all, axis=0).astype(BF16)
        full = (slice(None), slice(None))
        _acc(gkv_acc, full, first, _nt(xnT_s[i], dpkv))

        o, dx = mlp(i, 2, first)
        out_st[i] = (out_acc[i] + o).astype(BF16)
        out_copy(i).start()
        dxn = dxn_acc[i] + dx + _nn(wpkv_s[...], dpkv)
        xn32 = xnT_s[i].astype(F32)
        m1 = jnp.sum(dxn, axis=0, keepdims=True) * (1.0 / D)
        m2 = jnp.sum(dxn * xn32, axis=0, keepdims=True) * (1.0 / D)
        rstd = rstd_s[i][0:1]
        dx_st[i] = (dyT_s[i].astype(F32) + rstd * (dxn - m1 - xn32 * m2)).astype(BF16)
        dx_copy(i).start()
        return carry

    lax.fori_loop(0, NT, phase3, 0)
    for c in mlp_out(2):
        c.start()

    gqT = gq_acc[...].astype(BF16)
    gkT = gkv_acc[:, 3 * 128:].astype(BF16).T[64:]
    dwqkv_st[:, 2 * D:3 * D] = gkv_acc[:, 0:D].astype(BF16)
    dwT = []
    for gT in (gqT, gkT):
        for g in range(NG):
            dwT.append(_nn(bd_s[PF * g:PF * g + PF, :], gT[PF * g:PF * g + PF]).astype(BF16))
    dwqkv_st[:, 0:2 * D] = jnp.concatenate(dwT, axis=0).T
    c_dwqkv.start()
    for g in range(NG):
        rows = slice(PF * g, PF * g + PF)
        dg = (_nt(wqkT_s[rows, :], gqT[rows]) + _nt(wqkT_s[D + PF * g:D + PF * g + PF, :], gkT[rows]))
        dg = jnp.where(bd_mask, dg, 0.0).astype(BF16)
        tmpa_s[rows, :] = _nt(dg, sel)
    for d in range(DH):
        dwphi_st[H * d:H * d + H, :] = tmpa_s[pl.ds(d, H, stride=DH), :].astype(BF16)
    c_dwphi.start()

    for p in range(3):
        for c in mlp_out(p):
            c.wait()
    c_dwo.wait()
    for i in range(NT):
        out_copy(i).wait()
        dx_copy(i).wait()
    c_dwqkv.wait()
    c_dwphi.wait()


@jax.jit
def pallas_parallel_sum__linear_kernel_hedgehog__glu_gated_geglu__prompt_kernel(
    A_x: jax.Array,
    A_wqkv: jax.Array,
    A_w_phi: jax.Array,
    A_wo: jax.Array,
    B_x: jax.Array,
    B_w_gate: jax.Array,
    B_w_up: jax.Array,
    B_w_down: jax.Array,
    grad_out: jax.Array,
):
    del B_x
    xT = A_x.reshape(S, D).T
    dyT = grad_out.reshape(S, D).T
    wphi2 = A_w_phi.transpose(1, 0, 2).reshape(D, DH)
    wdT = B_w_down.T

    V = pltpu.VMEM
    scratch = [
        V((NT, D, TS), BF16), V((NT, D, TS), BF16), V((NT, D, TS), BF16),
        V((NT, TS, D), BF16), V((NT, TS, D), BF16), V((NT, 8, TS), F32),
        V((D, 3 * D), BF16), V((D, DH), BF16), V((D, D), BF16),
        V((D, DF), BF16), V((D, DF), BF16), V((D, DF), BF16),
        V((2 * D, D), BF16), V((D, PF), BF16), V((D, D), BF16), V((2 * D, D), BF16),
        V((D, D), BF16), V((D, 2 * D), BF16), V((D, D), BF16),
        V((D, DH), F32), V((D, DH), F32),
        V((NT, NP * PF, TS), BF16), V((NT, NP * PE, TS), BF16),
        V((NP, PE, PF), F32), V((NP, PE, PF), F32),
        V((NP, PE, PF), BF16), V((NP, PF, PE), BF16),
        V((NT, D, TS), F32), V((NT, D, TS), F32),
        V((D, DF), F32), V((D, DF), F32), V((D, DF), F32),
        V((D, D), F32), V((D, 2 * D), F32), V((D, D), F32),
        V((NT, D, TS), BF16), V((NT, D, TS), BF16),
        V((D, 3 * D), BF16), V((D, DH), BF16), V((D, D), BF16),
        V((D, DF), BF16), V((D, DF), BF16), V((D, DF), BF16),
        pltpu.SemaphoreType.DMA((3,)), pltpu.SemaphoreType.DMA((NT,)), pltpu.SemaphoreType.DMA((NT,)),
        pltpu.SemaphoreType.DMA((9,)), pltpu.SemaphoreType.DMA((NT,)), pltpu.SemaphoreType.DMA((NT,)),
        pltpu.SemaphoreType.DMA((3,)), pltpu.SemaphoreType.DMA((9,)),
    ]
    sds = jax.ShapeDtypeStruct
    out_shape = (
        sds((D, S), BF16), sds((D, S), BF16), sds((D, 3 * D), BF16), sds((D, DH), BF16),
        sds((D, D), BF16), sds((D, DF), BF16), sds((D, DF), BF16), sds((D, DF), BF16),
    )
    any_spec = pl.BlockSpec(memory_space=pl.ANY)
    outT, dxT, dwqkv, dwphi2, dwo, dwg, dwu, dwdT = pl.pallas_call(
        _kernel,
        out_shape=out_shape,
        in_specs=[any_spec] * 8,
        out_specs=[any_spec] * 8,
        scratch_shapes=scratch,
        compiler_params=pltpu.CompilerParams(vmem_limit_bytes=110 * 1024 * 1024),
        name="hedgehog_geglu",
    )(xT, A_wqkv, wphi2, A_wo, B_w_gate, B_w_up, wdT, dyT)
    return (
        outT.T.reshape(1, S, D),
        dxT.T.reshape(1, S, D),
        dwqkv,
        dwphi2.reshape(DH, H, DH).transpose(1, 0, 2),
        dwo,
        dwg,
        dwu,
        dwdT.T,
    )
```

```python
import math

import jax
import jax.numpy as jnp
from jax import lax
import jax.experimental.pallas as pl
import jax.experimental.pallas.tpu as pltpu

S, D, H, DH, DF = 2048, 448, 16, 28, 1792
NP = H // 2
PR = 2 * DH
PF = 2 * PR
PE = PR + 8
NG = H // 4
TS = 256
NT = S // TS
SB, DB = TS // 2, D // 2
AORD = (6, 5, 0, 3, 4, 7, 8)
PORD = (1, 3, 2, 4, 0, 6, 5)
XEXT = (None, 7, 8, 9, 7, 8, 9)
FEXT = (None, 8, 9, 9, 7, 8, 7)
KS, KG = 256, 64
BORD = (0, 2, 6, 5, 3, 4, 1)
CHUNKS = (((0, 256), (256, 256)),
          ((512, 256), (768, 256), (1024, 256)),
          ((1280, 256), (1536, 256)))
LN_EPS = 1e-5
DEN_EPS = 1e-6
C0 = math.sqrt(2.0 / math.pi)
C1 = 0.044715
F32, BF16, U32 = jnp.float32, jnp.bfloat16, jnp.uint32


def _nn(a, b):
    return lax.dot_general(a, b, (((1,), (0,)), ((), ())), preferred_element_type=F32)


def _nt(a, b):
    return lax.dot_general(a, b, (((1,), (1,)), ((), ())), preferred_element_type=F32)


def _tn(a, b):
    return lax.dot_general(a, b, (((0,), (0,)), ((), ())), preferred_element_type=F32)


def _tree(op, xs):
    xs = list(xs)
    while len(xs) > 1:
        nxt = [op(xs[i], xs[i + 1]) for i in range(0, len(xs) - 1, 2)]
        if len(xs) % 2:
            nxt.append(xs[-1])
        xs = nxt
    return xs[0]


def _rows8(a):
    return [a[8 * i:8 * i + 8] for i in range(a.shape[0] // 8)]


def _pair_reduce(op, rows):
    v = _tree(op, rows)
    v = op(v, pltpu.roll(v, 2, 0))
    return op(v, pltpu.roll(v, 4, 0))


def _softmax_pair(p):
    rows = _rows8(p)
    mx = _pair_reduce(jnp.maximum, rows)
    mn = _pair_reduce(jnp.minimum, rows)
    ep = [jnp.exp(r - mx) for r in rows]
    en = [jnp.exp(mn - r) for r in rows]
    rp = 1.0 / _pair_reduce(jnp.add, ep)
    rn = 1.0 / _pair_reduce(jnp.add, en)
    return jnp.concatenate([e * rp for e in ep] + [e * rn for e in en], axis=0)


def _softmax_pair_bwd(phi, dphi):
    pr, dr = _rows8(phi), _rows8(dphi)
    t = [a * b for a, b in zip(pr, dr)]
    sp = _pair_reduce(jnp.add, t[:7])
    sn = _pair_reduce(jnp.add, t[7:])
    out = [(t[i] - t[7 + i]) - (pr[i] * sp - pr[7 + i] * sn) for i in range(7)]
    return jnp.concatenate(out, axis=0)


def _pk(a):
    return pltpu.bitcast(a, U32)


def _up(a):
    return pltpu.bitcast(a, BF16)


def _cat(xs, axis=0):
    return jnp.concatenate(xs, axis=axis)


def _split(a):
    w = _pk(a)
    return [pltpu.unpack_elementwise(w, index=j, packed_dtype=BF16, unpacked_dtype=F32) for j in range(2)]


def _pack(e, o):
    return pltpu.pack_elementwise([e, o], packed_dtype=BF16)


def _pack16(a):
    r = _rows8(a)
    return _pack(_cat(r[0::2]), _cat(r[1::2]))


def _unpack16(w):
    e, o = [_rows8(pltpu.unpack_elementwise(w, index=j, packed_dtype=BF16, unpacked_dtype=F32)) for j in range(2)]
    return _cat([x for p in zip(e, o) for x in p])


def _bf(xs):
    return [a.astype(BF16) for a in xs]


def _combos(x11, x12, x21, x22):
    return [x11 + x22, x21 + x22, x11, x22, x11 + x12, x21 - x11, x12 - x22]


def _combos_t(x11, x12, x21, x22):
    return _combos(x11, x21, x12, x22)


def _uncombos(m):
    return (m[0] + m[3] - m[4] + m[6], m[2] + m[4], m[1] + m[3], m[0] - m[1] + m[2] + m[5])


def _uncombos_t(m):
    c11, c12, c21, c22 = _uncombos(m)
    return c11, c21, c12, c22


def _quarters(x):
    r, c = x.shape[0] // 2, x.shape[1] // 2
    return x[:r, :c], x[:r, c:], x[r:, :c], x[r:, c:]


def _join(x11, x12, x21, x22):
    return _cat([_cat([x11, x12], 1), _cat([x21, x22], 1)])


def _set_a(x):
    x11, x12, x21, x22 = _quarters(x)
    return [x11, x21, x12, x22, x11 + x12, x21 + x22, x11 + x22, x21 - x11, x12 - x22]


def _groups(x):
    n = x.shape[0] // 7
    return x[:4 * n], [x[(4 + j) * n:(5 + j) * n] for j in range(3)]


def _halves(x, axis=1):
    n = x.shape[axis] // 2
    return (x[:, :n], x[:, n:]) if axis else (x[:n], x[n:])


def _set_x(x):
    top, g = _groups(x)
    (l1, r1), (l2, r2), (l3, r3) = [_halves(a) for a in g]
    return _combos(*_quarters(top)) + [_cat([l2, r3]), _cat([r1, l2 + r2]), _cat([l1, l3 + r3])]


def _set_w(x):
    top, g = _groups(x)
    (l1, r1), (l2, r2), (l3, r3) = [_halves(a) for a in g]
    d1 = r1 - l1
    ext = [[], [r2, -r3], [l1, l2], [r1, r3], [-l2, l3], [d1, r2 - l2], [-d1, l3 - r3]]
    return [_cat([c] + e) for c, e in zip(_combos_t(*_quarters(top)), ext)]


def _set_f(x):
    top, g = _groups(x)
    (l1, r1), (l2, r2), (l3, r3) = [_halves(a) for a in g]
    return _combos_t(*_quarters(top)) + [_cat([l1, l2 - r2]), _cat([r1, r3 - l3]), _cat([r2, l3])]


def _wf_set(t):
    low = lax.broadcasted_iota(jnp.int32, (DB, 128), 1) < KG
    (a0, b0), (a1, b1), (a2, b2), (a3, b3) = [_halves(a, 0) for a in t]
    d2 = b2 - a2
    ext = [None, jnp.where(low, b3, -b3), a2, jnp.where(low, b2, b3), jnp.where(low, -a3, a3), d2,
           jnp.where(low, -d2, a3 - b3)]
    return [c if e is None else _cat([c, e], 1) for c, e in zip(_combos(a0, a1, b0, b1), ext)]


def _wb_set(t):
    low = lax.broadcasted_iota(jnp.int32, (DB, 128), 1) < KG
    (a0, b0), (a1, b1), (a2, b2), (a3, b3) = [_halves(a, 0) for a in t]
    a13, b13 = jnp.where(low, a2, a3), jnp.where(low, b2, b3)
    ext = [None, a13, b3, a3, b2, a13 + b13, a2 + b2]
    c = _combos_t(a0, a1, b0, b1)
    return [c[BORD[k]] if e is None else _cat([c[BORD[k]], e], 1) for k, e in enumerate(ext)]


def _unit(ref, idx, k, rows=DB // 2, n=1):
    return _up(ref[idx + (slice(rows * k, rows * (k + n)),)])


def _acc(ref, idx, first, val):
    ref[idx] = val if first else ref[idx] + val


TILES = ((0, 128), (128, 256), (256, 384), (320, 448))


def _kernel(xT_h, wqkv_h, wphi_h, wo_h, wg_h, wu_h, wdT_h, dyT_h,
            outT_h, dxT_h, dwqkv_h, dwphi_h, dwo_h, dwg_h, dwu_h, dwdT_h,
            xT_s, dyT_s, rstd_s, doT_s, xa_s, ya_s, xb_s, xbt_s, ybt_s, tr_s,
            wqkv_s, wphi_s, wo_s, wg_s, wu_s, wdT_s,
            wT_s, bd_s, wf_s, wb_s,
            wa_gu, wa_d, wb_gu, wb_d, tmpa_s, tmpb_s,
            hc_s, dguc_s, phik_s, vext_s, kv_acc, kvt_s, kv_s,
            out_acc, dxn_acc, dwgu_acc, dwd_acc, g_acc,
            out_st, dx_st, dwqkv_st, dwphi_st, dwo_st, dwg_st, dwu_st, dwd_st,
            sem_w, sem_x, sem_dy, sem_mlp, sem_out, sem_dx, sem_ow, sem_omlp):
    def x_copy(i):
        return pltpu.make_async_copy(xT_h.at[:, pl.ds(i * TS, TS)], xT_s.at[i], sem_x.at[i])

    def dy_copy(i):
        return pltpu.make_async_copy(dyT_h.at[:, pl.ds(i * TS, TS)], dyT_s.at[i], sem_dy.at[i])

    def col_copies(chunks, pairs, sem, base):
        lo, hi = chunks[0][0], chunks[-1][0] + chunks[-1][1]
        return [pltpu.make_async_copy(src.at[:, pl.ds(lo, hi - lo)], dst.at[:, pl.ds(lo, hi - lo)],
                                      sem.at[base + k]) for k, (src, dst) in enumerate(pairs)]

    in_groups = [CHUNKS[0][:1], CHUNKS[0][1:], CHUNKS[1] + CHUNKS[2]]
    out_groups = [CHUNKS[0], CHUNKS[1], CHUNKS[2][:1], CHUNKS[2][1:]]

    def mlp_in(g):
        return col_copies(in_groups[g], ((wg_h, wg_s), (wu_h, wu_s), (wdT_h, wdT_s)), sem_mlp, 3 * g)

    def mlp_out(g):
        return col_copies(out_groups[g], ((dwg_st, dwg_h), (dwu_st, dwu_h), (dwd_st, dwdT_h)), sem_omlp, 3 * g)

    def out_copy(i):
        return pltpu.make_async_copy(out_st.at[i], outT_h.at[:, pl.ds(i * TS, TS)], sem_out.at[i])

    def dx_copy(i):
        return pltpu.make_async_copy(dx_st.at[i], dxT_h.at[:, pl.ds(i * TS, TS)], sem_dx.at[i])

    c_wphi = pltpu.make_async_copy(wphi_h, wphi_s, sem_w.at[0])
    c_wqkv = pltpu.make_async_copy(wqkv_h, wqkv_s, sem_w.at[1])
    c_wo = pltpu.make_async_copy(wo_h, wo_s, sem_w.at[2])
    c_dwqkv = pltpu.make_async_copy(dwqkv_st, dwqkv_h, sem_ow.at[0])
    c_dwphi = pltpu.make_async_copy(dwphi_st, dwphi_h, sem_ow.at[1])
    c_dwo = pltpu.make_async_copy(dwo_st, dwo_h, sem_ow.at[2])

    def start(cs):
        for c in cs:
            c.start()

    def wait(cs):
        for c in cs:
            c.wait()

    def bd_consts():
        r = lax.broadcasted_iota(jnp.int32, (PF, PF), 0)
        c = lax.broadcasted_iota(jnp.int32, (PF, PF), 1)
        row_head = ((r >= DH).astype(jnp.int32) + (r >= 2 * DH).astype(jnp.int32)
                    + (r >= 3 * DH).astype(jnp.int32))
        mask = row_head == 2 * (c >= PR).astype(jnp.int32) + (c & 1)
        sc = lax.broadcasted_iota(jnp.int32, (DH, PF), 1)
        sr = lax.broadcasted_iota(jnp.int32, (DH, PF), 0)
        sel = jnp.where(((sc - PR * (sc >= PR).astype(jnp.int32)) >> 1) == sr, 1.0, 0.0).astype(BF16)
        return mask, sel

    def kv_operands(s):
        r = lax.broadcasted_iota(jnp.int32, (PE, PF), 0)
        c = lax.broadcasted_iota(jnp.int32, (PE, PF), 1)
        row_head = jnp.where(r < PR, (r >= DH).astype(jnp.int32), (r >= PR + 4).astype(jnp.int32))
        mask = row_head == (c & 1)
        for p in range(NP):
            m = jnp.where(mask, kv_acc[s, p], 0.0)
            kvt_s[s, p] = _pk(m.astype(BF16))
            kv_s[s, p] = _pk(m.T.astype(BF16))

    def untile(t):
        return _cat([t[0].T, t[1].T, t[2].T, t[3].T[KG:]])

    def prep_qkv():
        mask, sel = bd_consts()
        tmpa_s[...] = wphi_s[...].astype(F32)
        for d in range(DH):
            tmpb_s[pl.ds(d, H, stride=DH), :] = tmpa_s[H * d:H * d + H, :]
        expand = _nn(tmpb_s[...].astype(BF16), sel)
        for g in range(NG):
            bd_s[PF * g:PF * g + PF, :] = jnp.where(mask, expand[PF * g:PF * g + PF], 0.0).astype(BF16)
        for j, (a, b) in enumerate(TILES):
            wT_s[:, 128 * j:128 * j + 128] = _pk(wqkv_s[a:b, :].T)

    def fold(t):
        w = _cat([_tn(bd_s[PF * g:PF * g + PF, :], _unit(wT_s, (), NG * t + g, PR)) for g in range(NG)])
        return [w[:, 128 * j:128 * j + 128] for j in range(4)]

    def store_set(ref, t, ws):
        for k, w in enumerate(ws):
            ref[t, k, :, :w.shape[1]] = _pk(w.astype(BF16))

    def wunit(ref, t, k):
        return _up(ref[t, k, :, :256 if k else 128])

    def prep_qk(t):
        w = fold(t)
        store_set(wf_s, t, _wf_set(w))
        store_set(wb_s, t, _wb_set([untile([c[a:b] for c in w]) for a, b in TILES]))

    def prep_v():
        w = _unit(wT_s, (), 2, DB).astype(F32)
        store_set(wf_s, 2, _wf_set([w[:, 128 * j:128 * j + 128] for j in range(4)]))

    def prep_v_t():
        store_set(wb_s, 2, _wb_set([wqkv_s[:, 2 * D + a:2 * D + b].astype(F32) for a, b in TILES]))

    def prep_wo():
        store_set(wf_s, 3, _wf_set([wo_s[:, a:b].astype(F32) for a, b in TILES]))

    def prep_wo_t():
        store_set(wb_s, 3, _wb_set([wo_s[a:b, :].T.astype(F32) for a, b in TILES]))

    def prep_mlp(ch, which):
        a, w = ch
        f = w // 2
        mats = (((wg_s, a), (wu_s, a + f)), ((wdT_s, a // 2),))[which]
        wa, wb = ((wa_gu, wb_gu), (wa_d, wb_d))[which]
        for ref, off in mats:
            e, o = _split(ref[:, a:a + w])
            for k, (p, q) in enumerate(zip(_set_w(e), _set_w(o))):
                wb[k, :p.shape[0], off:off + f] = _pack(p, q)
            for k, (p, q) in enumerate(zip(_combos_t(*_quarters(e)), _combos_t(*_quarters(o)))):
                wa[k, :, off:off + f] = _pack(p, q)

    def unfold_phi(gT, t):
        dphi, dwT = [], []
        low = lax.broadcasted_iota(jnp.int32, (PF, 512), 1)
        dup = (low >= 3 * 128) & (low < 3 * 128 + KG)
        for g in range(NG):
            r = slice(PF * g, PF * g + PF)
            dphi.append(_nt(jnp.where(dup, 0, _unit(wT_s, (), NG * t + g, PR)), gT[r]))
            dwT.append(_nn(bd_s[r, :], gT[r]).astype(BF16))
        return dphi, dwT

    def ragged(get, k, ext, axis):
        return get(k) if ext is None else _cat([get(k), get(ext)], axis)

    def project(w, xs):
        m = {k: _nn(wunit(wf_s, w, k), ragged(xs, BORD[k], XEXT[k], 0)) for k in PORD}
        return _join(*_uncombos(m))

    def back_project(w, fs, m):
        return [m[k] + _nn(wunit(wb_s, w, k), ragged(lambda j: fs[j], k, FEXT[k], 0)) for k in range(7)]

    def outer(w, a_s, i, fs, first):
        for k in range(7):
            _acc(g_acc, (w, slice(DB * k, DB * k + DB)), first, _nt(_unit(a_s, (i,), AORD[k]), fs[BORD[k]]))
        for k in range(3):
            _acc(g_acc, (w, slice(DB * (7 + 2 * k), DB * (9 + 2 * k))), first,
                 _nt(_unit(a_s, (i,), 2 * k, n=2), fs[7 + k]))

    def outer_result(w):
        c11, c12, c21, c22 = _uncombos([g_acc[w, DB * k:DB * k + DB] for k in range(7)])
        p = [g_acc[w, DB * (7 + 2 * k):DB * (9 + 2 * k)] for k in range(3)]
        low = lax.broadcasted_iota(jnp.int32, (D, 128), 1) < KG
        t = [_cat([c11, c21]), _cat([c12, c22]),
             p[0] + jnp.where(low, p[1], pltpu.roll(p[2], KG, 1)), p[1] + p[2]]
        return [a.astype(BF16) for a in t]

    def mlp_pre(bt_s, i, wb, a, w, k):
        lhs = ragged(lambda j: _unit(bt_s, (i,), j, 64), BORD[k], XEXT[k], 1)
        return _nn(lhs, _up(wb[k, :128 if k else 64, a:a + w]))

    def mlp_gu(i, ch, k):
        return mlp_pre(xbt_s, i, wb_gu, ch[0], ch[1], k)

    def mlp_dh(i, ch, k):
        return mlp_pre(ybt_s, i, wb_d, ch[0] // 2, ch[1] // 2, k)

    def mlp_s1(i, n, ch, gum=None, dhm=None):
        gum, dhm = dict(gum or {}), dict(dhm or {})
        for k in PORD:
            if k not in dhm:
                dhm[k] = mlp_dh(i, ch, k)
            if k not in gum:
                gum[k] = mlp_gu(i, ch, k)
        f = ch[1] // 2
        hs, dgus = [], []
        for gu, dh in zip(_uncombos_t(gum), _uncombos_t(dhm)):
            g, u = gu[:, :f], gu[:, f:]
            g2 = g * g
            s = 0.5 * jnp.tanh(g * (C0 + (C0 * C1) * g2)) + 0.5
            gelu = g * s
            dgelu = s + gelu * (1.0 - s) * (2.0 * C0 + (6.0 * C0 * C1) * g2)
            hs.append(gelu * u)
            dgus.append(_cat([dh * u * dgelu, dh * gelu], 1))
        for k, (h, dgu) in enumerate(zip(_combos(*hs), _combos(*dgus))):
            hc_s[k, :, f * n:f * n + f] = pack_tokens(h)
            dguc_s[k, :, 2 * f * n:2 * f * n + 2 * f] = pack_tokens(dgu)

    def pack_tokens(a):
        r = _rows8(a)
        return _pack(_cat([x for j, x in enumerate(r) if not j & 2]), _cat([x for j, x in enumerate(r) if j & 2]))

    def mlp_out_p(chunks):
        a, w = chunks[0][0], sum(c[1] for c in chunks)
        return [_nt(_up(wa_d[BORD[k], :, a // 2:(a + w) // 2]), _up(hc_s[k, :, :w // 2])) for k in range(7)]

    def mlp_dx_p(chunks):
        a, w = chunks[0][0], sum(c[1] for c in chunks)
        return [_nt(_up(wa_gu[BORD[k], :, a:a + w]), _up(dguc_s[k, :, :w])) for k in range(7)]

    def mlp_s2b(i, n, ch, mode):
        a, w = ch
        f = w // 2
        for a_s, src, acc, wd, dsts in ((ya_s, hc_s, dwd_acc, f, (dwd_st,)),
                                        (xa_s, dguc_s, dwgu_acc, w, (dwg_st, dwu_st))):
            m = []
            for k in range(7):
                v = _nn(_unit(a_s, (i,), AORD[k]), _up(src[BORD[k], :, wd * n:wd * n + wd]))
                idx = (k, slice(None), slice(wd * n, wd * n + wd))
                if mode == 'last':
                    m.append(acc[idx] + v)
                else:
                    _acc(acc, idx, mode == 'first', v)
            if mode == 'last':
                q = _uncombos(m)
                for j, dst in enumerate(dsts):
                    dst[:, a:a + w] = _join(*[v[:, f * j:f * j + f] for v in q]).astype(BF16)

    def store_sets(i, e, o, a_s, bt_s, slot):
        b = [_pack(p, q) for p, q in zip(_set_x(e), _set_x(o))]
        for k, w in enumerate(b):
            tr_s[slot, 64 * k:64 * k + 64] = _pk(_up(w).T)
            for j in range(4):
                base = 64 * k + 16 * j
                p, q = [_split(_up(tr_s[slot, pl.ds(base + c, 8, stride=2), :])) for c in range(2)]
                bt_s[i, base:base + 16] = _cat([_pack(p[0], q[0]), _pack(p[1], q[1])])
        a_s[i, :9 * DB // 2] = _cat([_pack(p, q) for p, q in zip(_set_a(e), _set_a(o))])
        return b

    def dy_sets(i):
        return [_up(w) for w in store_sets(i, *_split(dyT_s[i]), ya_s, ybt_s, 0)]

    def layernorm(i):
        e, o = _split(xT_s[i])
        mean = jnp.sum(e + o, axis=0, keepdims=True) * (1.0 / D)
        e, o = e - mean, o - mean
        var = jnp.sum(e * e + o * o, axis=0, keepdims=True) * (1.0 / D)
        rstd = lax.rsqrt(var + LN_EPS)
        rstd_s[i, 0:8] = jnp.broadcast_to(rstd, (8, TS))
        xb_s[i] = _cat(store_sets(i, e * rstd, o * rstd, xa_s, xbt_s, 1))

    def xproj(i, t):
        return project(t, lambda k: _unit(xb_s, (i,), k, 64))

    def do_proj(i, yb):
        doT_s[i] = _pack16(project(3, lambda k: yb[k]))

    def key_side(i, pk, v, first):
        ones = jnp.ones((8, TS), F32)
        for c in range(NP):
            phik = _softmax_pair(pk[PR * c:PR * c + PR]).astype(BF16)
            phik_s[i, PR * c:PR * c + PR, :] = _pk(phik)
            vext = _cat([v[PR * c:PR * c + PR], ones]).astype(BF16)
            vext_s[i, 32 * c:32 * c + 32, :] = _pk(vext)
            _acc(kv_acc, (0, c), first, _nt(vext, phik))

    def phase1_tail(i):
        for k, (o, dx) in enumerate(zip(mlp_out_p(CHUNKS[0]), mlp_dx_p(CHUNKS[0]))):
            out_acc[i, k] = o
            dxn_acc[i, k] = dx

    c0, c1 = CHUNKS[0]
    start([x_copy(0)] + mlp_in(0) + [dy_copy(0)])
    with jax.named_scope('w_0'):
        wait([x_copy(0), dy_copy(0)] + mlp_in(0))
    start(mlp_in(1) + [c_wo])
    layernorm(0)
    prep_mlp(c0, 0)
    gu = {k: mlp_gu(0, c0, k) for k in PORD}
    yb = dy_sets(0)
    prep_mlp(c0, 1)
    mlp_s1(0, 0, c0, gu)
    with jax.named_scope('w_1'):
        wait(mlp_in(1) + [c_wo])
    start([c_wphi, c_wqkv])
    prep_wo()
    do_proj(0, yb)
    prep_mlp(c1, 0)
    prep_mlp(c1, 1)
    mlp_s1(0, 1, c1)
    mlp_s2b(0, 0, c0, 'first')
    with jax.named_scope('w_2'):
        wait([c_wphi, c_wqkv])
    start([x_copy(1), dy_copy(1), x_copy(2), dy_copy(2)])
    prep_qkv()
    mlp_s2b(0, 1, c1, 'first')
    prep_v()
    v = xproj(0, 2)
    prep_qk(1)
    pk = xproj(0, 1)
    key_side(0, pk, v, True)
    for i in range(3, NT):
        start([x_copy(i), dy_copy(i)])
    start(mlp_in(2))

    def phase1(i, mode):
        wait([dy_copy(i), x_copy(i)])
        phase1_tail(i - 1)
        yb = dy_sets(i)
        layernorm(i)
        do_proj(i, yb)
        mlp_s1(i, 0, c0)
        pk = xproj(i, 1)
        mlp_s1(i, 1, c1)
        v = xproj(i, 2)
        mlp_s2b(i, 0, c0, mode)
        key_side(i, pk, v, False)
        mlp_s2b(i, 1, c1, mode)

    def loop(name, f):
        def body(i, carry):
            with jax.named_scope('it' + name):
                f(i, 'mid')
            return carry
        with jax.named_scope('p' + name):
            lax.fori_loop(1, NT - 1, body, 0)

    loop('1', phase1)
    wait(mlp_in(2))
    prep_qk(0)
    prep_wo_t()
    phase1(NT - 1, 'last')
    start(mlp_out(0))
    kv_operands(0)
    phase1_tail(NT - 1)

    def phase2(i, mode):
        first = mode == 'first'
        lo4 = lax.broadcasted_iota(jnp.int32, (8, TS), 0) < 4
        ch = CHUNKS[1]

        def s1(n):
            if first:
                prep_mlp(ch[n], 0)
                prep_mlp(ch[n], 1)
            mlp_s1(i, n, ch[n])

        pq = xproj(i, 0)
        s1(0)
        phis, phibs, nes = [], [], []
        for c in range(NP):
            phi = _softmax_pair(pq[PR * c:PR * c + PR])
            phis.append(phi)
            phibs.append(phi.astype(BF16))
            nes.append(_rows8(_nn(_up(kvt_s[0, c]), phibs[c])))
        s1(1)
        o_all, dp_all = [], []
        doT = _unpack16(doT_s[i])
        for c in range(NP):
            ne = nes[c]
            r = 1.0 / (ne[7] + DEN_EPS)
            rr = pltpu.roll(r, 4, 0)
            ra = jnp.where(lo4, r, rr)
            rb = jnp.where(lo4, rr, r)
            rs = [ra, ra, ra, r, rb, rb, rb]
            o = [n * w for n, w in zip(ne[:7], rs)]
            dnum = [n * w for n, w in zip(_rows8(doT[PR * c:PR * c + PR]), rs)]
            t = [a * b for a, b in zip(dnum, o)]
            sa = t[0] + t[1] + t[2]
            sb = t[4] + t[5] + t[6]
            e = jnp.where(lo4, sa, sb) + pltpu.roll(jnp.where(lo4, sb, sa), 4, 0) + t[3]
            dne = _cat(dnum + [-e]).astype(BF16)
            dphi = _nn(_up(kv_s[0, c]), dne)
            _acc(kv_acc, (1, c), first, _nt(dne, phibs[c]))
            dp_all.append(_softmax_pair_bwd(phis[c], dphi))
            o_all.extend(o)
        s1(2)
        ob = _bf(_set_f(_cat(o_all)))
        dpb = _bf(_set_f(_cat(dp_all)))
        outer(3, ya_s, i, ob, first)
        mlp_s2b(i, 0, ch[0], mode)
        outer(0, xa_s, i, dpb, first)
        mlp_s2b(i, 1, ch[1], mode)
        o = back_project(3, ob, [out_acc[i, k] + m for k, m in enumerate(mlp_out_p(ch))])
        for k in range(7):
            out_acc[i, k] = o[k]
        dx = back_project(0, dpb, [dxn_acc[i, k] + m for k, m in enumerate(mlp_dx_p(ch))])
        for k in range(7):
            dxn_acc[i, k] = dx[k]
        mlp_s2b(i, 2, ch[2], mode)

    phase2(0, 'first')
    loop('2', phase2)
    phase2(NT - 1, 'last')
    start(mlp_out(1))
    kv_operands(1)

    def key_bwd(i):
        dv_all, dp_all = [], []
        for c in range(NP):
            phik = _up(phik_s[i, PR * c:PR * c + PR, :])
            dphik = _nn(_up(kv_s[1, c]), _up(vext_s[i, 32 * c:32 * c + 32, :]))
            dv_all.append(_nn(_up(kvt_s[1, c]), phik)[0:PR])
            dp_all.append(_softmax_pair_bwd(phik.astype(F32), dphik))
        return _bf(_set_f(_cat(dp_all))), _bf(_set_f(_cat(dv_all)))

    def finish_dx(i, dkb, dvb):
        m = back_project(1, dkb, back_project(2, dvb, [dxn_acc[i, k] for k in range(7)]))
        dxn = _join(*_uncombos_t([a + b for a, b in zip(m, mlp_dx_p(CHUNKS[2]))]))
        xn32 = _cat([_unit(xa_s, (i,), 0, n=2), _unit(xa_s, (i,), 2, n=2)], 1).astype(F32)
        m1 = jnp.sum(dxn, axis=0, keepdims=True) * (1.0 / D)
        m2 = jnp.sum(dxn * xn32, axis=0, keepdims=True) * (1.0 / D)
        rstd = rstd_s[i, 0:8][0:1]
        dx_st[i] = (dyT_s[i].astype(F32) + rstd * (dxn - m1 - xn32 * m2)).astype(BF16)

    def finish_out(i):
        o = [out_acc[i, k] + m for k, m in enumerate(mlp_out_p(CHUNKS[2]))]
        out_st[i] = (xT_s[i].astype(F32) + _join(*_uncombos_t(o))).astype(BF16)

    def phase3(i, mode):
        first = mode == 'first'
        ch = CHUNKS[2]
        if first:
            prep_mlp(ch[0], 0)
            prep_mlp(ch[0], 1)
            mlp_s1(i, 0, ch[0])
            dkb, dvb = key_bwd(i)
            prep_mlp(ch[1], 0)
            prep_mlp(ch[1], 1)
        else:
            dkb, dvb = key_bwd(i)
            mlp_s1(i, 0, ch[0])
        mlp_s1(i, 1, ch[1])
        outer(2, xa_s, i, dvb, first)
        outer(1, xa_s, i, dkb, first)
        finish_dx(i, dkb, dvb)
        finish_out(i)
        mlp_s2b(i, 0, ch[0], mode)
        mlp_s2b(i, 1, ch[1], mode)
        start([out_copy(i), dx_copy(i)])

    def tiles_t(t):
        return _cat([untile([a[lo:hi] for a in t]) for lo, hi in TILES], 1)

    prep_v_t()
    phase3(0, 'first')
    dwo_t = outer_result(3)
    dwo_st[...] = _cat([a.T for a in dwo_t[:3]] + [dwo_t[3].T[KG:]])
    start([c_dwo])
    loop('3', phase3)

    i = NT - 1
    ch = CHUNKS[2]
    dkb, dvb = key_bwd(i)
    mlp_s1(i, 0, ch[0])
    mlp_s1(i, 1, ch[1])
    dphi_q, dwT_q = unfold_phi(tiles_t(outer_result(0)), 0)
    mlp_s2b(i, 0, ch[0], 'last')
    start(mlp_out(2))
    outer(1, xa_s, i, dkb, False)
    outer(2, xa_s, i, dvb, False)
    gv = outer_result(2)
    dwqkv_st[:, 2 * D:3 * D] = _cat(gv[:3] + [gv[3][:, KG:]], 1)
    mlp_s2b(i, 1, ch[1], 'last')
    start(mlp_out(3))
    dphi_k, dwT_k = unfold_phi(tiles_t(outer_result(1)), 1)
    dwT = _cat(dwT_q + dwT_k)
    dwqkv_st[:, 0:2 * D] = untile([dwT[:, 128 * j:128 * j + 128] for j in range(4)])
    mask, sel = bd_consts()
    for g in range(NG):
        dg = jnp.where(mask, dphi_q[g] + dphi_k[g], 0.0).astype(BF16)
        tmpa_s[PF * g:PF * g + PF, :] = _nt(dg, sel)
    for d in range(DH):
        dwphi_st[H * d:H * d + H, :] = tmpa_s[pl.ds(d, H, stride=DH), :].astype(BF16)
    start([c_dwqkv, c_dwphi])
    finish_dx(i, dkb, dvb)
    start([dx_copy(i)])
    finish_out(i)
    start([out_copy(i)])

    with jax.named_scope('w_end'):
        for g in range(4):
            wait(mlp_out(g))
        wait([c_dwo, c_dwqkv, c_dwphi])
        for i in range(NT):
            wait([out_copy(i), dx_copy(i)])


@jax.jit
def pallas_parallel_sum__linear_kernel_hedgehog__glu_gated_geglu__prompt_kernel(
    A_x: jax.Array,
    A_wqkv: jax.Array,
    A_w_phi: jax.Array,
    A_wo: jax.Array,
    B_x: jax.Array,
    B_w_gate: jax.Array,
    B_w_up: jax.Array,
    B_w_down: jax.Array,
    grad_out: jax.Array,
):
    del B_x
    xT = A_x.reshape(S, D).T
    dyT = grad_out.reshape(S, D).T
    wphi2 = A_w_phi.transpose(1, 0, 2).reshape(D, DH)
    wdT = B_w_down.T

    V = pltpu.VMEM
    dma = pltpu.SemaphoreType.DMA
    scratch = [
        V((NT, D, TS), BF16), V((NT, D, TS), BF16),
        V((NT, 32, TS), F32), V((NT, DB, TS), U32),
        V((NT, 1024, SB), U32), V((NT, 1024, SB), U32),
        V((NT, 640, SB), U32), V((NT, 640, 128), U32), V((NT, 640, 128), U32),
        V((2, 640, 128), U32),
        V((D, 3 * D), BF16), V((D, DH), BF16), V((D, D), BF16),
        V((D, DF), BF16), V((D, DF), BF16), V((D, DF), BF16),
        V((3 * DB, 512), U32), V((D, PF), BF16),
        V((4, 7, DB // 2, 256), U32), V((4, 7, DB // 2, 256), U32),
        V((7, DB // 2, DF), U32), V((7, DB // 2, DF // 2), U32),
        V((7, 128, DF), U32), V((7, 128, DF // 2), U32),
        V((D, DH), F32), V((D, DH), F32),
        V((7, SB // 2, 384), U32), V((7, SB // 2, 768), U32),
        V((NT, NP * PR, TS), U32), V((NT, NP * 32, TS), U32),
        V((2, NP, PE, PF), F32), V((2, NP, PE // 2, PF), U32), V((2, NP, PR, PE), U32),
        V((NT, 8, DB, SB), F32), V((NT, 8, DB, SB), F32),
        V((7, DB, 768), F32), V((7, DB, 384), F32),
        V((4, 13 * DB, 128), F32),
        V((NT, D, TS), BF16), V((NT, D, TS), BF16),
        V((D, 3 * D), BF16), V((D, DH), BF16), V((D, D), BF16),
        V((D, DF), BF16), V((D, DF), BF16), V((D, DF), BF16),
        dma((3,)), dma((NT,)), dma((NT,)), dma((9,)), dma((NT,)), dma((NT,)), dma((3,)), dma((12,)),
    ]
    sds = jax.ShapeDtypeStruct
    out_shape = (
        sds((D, S), BF16), sds((D, S), BF16), sds((D, 3 * D), BF16), sds((D, DH), BF16),
        sds((D, D), BF16), sds((D, DF), BF16), sds((D, DF), BF16), sds((D, DF), BF16),
    )
    any_spec = pl.BlockSpec(memory_space=pl.ANY)
    outT, dxT, dwqkv, dwphi2, dwo, dwg, dwu, dwdT = pl.pallas_call(
        _kernel,
        out_shape=out_shape,
        in_specs=[any_spec] * 8,
        out_specs=[any_spec] * 8,
        scratch_shapes=scratch,
        compiler_params=pltpu.CompilerParams(vmem_limit_bytes=120 * 1024 * 1024),
        name="hedgehog_geglu",
    )(xT, A_wqkv, wphi2, A_wo, B_w_gate, B_w_up, wdT, dyT)
    return (
        outT.T.reshape(1, S, D),
        dxT.T.reshape(1, S, D),
        dwqkv,
        dwphi2.reshape(DH, H, DH).transpose(1, 0, 2),
        dwo,
        dwg,
        dwu,
        dwdT.T,
    )
```

```python
import math

import jax
import jax.numpy as jnp
from jax import lax
import jax.experimental.pallas as pl
import jax.experimental.pallas.tpu as pltpu

S, D, H, DH, DF = 2048, 448, 16, 28, 1792
NP = H // 2
PR = 2 * DH
PF = 2 * PR
PE = PR + 8
NG = H // 4
TS = 256
NT = S // TS
SB, DB = TS // 2, D // 2
AORD = (6, 5, 0, 3, 4, 7, 8)
PORD = (1, 3, 2, 4, 0, 6, 5)
TORD = (1, 3, 0, 4, 6, 2, 5)
RORD = {'ab': (0, 7, 4, 11, 1, 8, 5, 12, 2, 9, 6, 13, 3, 10), 'a': (0, 7, 1, 8, 2, 9, 3, 10, 4, 11, 5, 12, 6, 13),
        'b': (0, 4, 1, 5, 2, 6, 3, 7, 8, 9, 10, 11, 12, 13), 'n': tuple(range(14))}
XEXT = (None, 7, 8, 9, 7, 8, 9)
FEXT = (None, 8, 9, 9, 7, 8, 7)
KS, KG = 256, 64
BORD = (0, 2, 6, 5, 3, 4, 1)
CHUNKS = (((0, 256), (256, 256)),
          ((512, 256), (768, 256), (1024, 256)),
          ((1280, 256), (1536, 256)))
LN_EPS = 1e-5
DEN_EPS = 1e-6
C0 = math.sqrt(2.0 / math.pi)
C1 = 0.044715
F32, BF16, U32 = jnp.float32, jnp.bfloat16, jnp.uint32


def _nn(a, b):
    return lax.dot_general(a, b, (((1,), (0,)), ((), ())), preferred_element_type=F32)


def _nt(a, b):
    return lax.dot_general(a, b, (((1,), (1,)), ((), ())), preferred_element_type=F32)


def _tn(a, b):
    return lax.dot_general(a, b, (((0,), (0,)), ((), ())), preferred_element_type=F32)


def _tree(op, xs):
    xs = list(xs)
    while len(xs) > 1:
        nxt = [op(xs[i], xs[i + 1]) for i in range(0, len(xs) - 1, 2)]
        if len(xs) % 2:
            nxt.append(xs[-1])
        xs = nxt
    return xs[0]


def _rows8(a):
    return [a[8 * i:8 * i + 8] for i in range(a.shape[0] // 8)]


def _pair_reduce(op, rows):
    v = _tree(op, rows)
    v = op(v, pltpu.roll(v, 2, 0))
    return op(v, pltpu.roll(v, 4, 0))


def _softmax_pair(p):
    rows = _rows8(p)
    mx = _pair_reduce(jnp.maximum, rows)
    mn = _pair_reduce(jnp.minimum, rows)
    ep = [jnp.exp(r - mx) for r in rows]
    en = [jnp.exp(mn - r) for r in rows]
    rp = 1.0 / _pair_reduce(jnp.add, ep)
    rn = 1.0 / _pair_reduce(jnp.add, en)
    return jnp.concatenate([e * rp for e in ep] + [e * rn for e in en], axis=0)


def _softmax_pair_bwd(phi, dphi):
    pr, dr = _rows8(phi), _rows8(dphi)
    t = [a * b for a, b in zip(pr, dr)]
    sp = _pair_reduce(jnp.add, t[:7])
    sn = _pair_reduce(jnp.add, t[7:])
    out = [(t[i] - t[7 + i]) - (pr[i] * sp - pr[7 + i] * sn) for i in range(7)]
    return jnp.concatenate(out, axis=0)


def _pk(a):
    return pltpu.bitcast(a, U32)


def _up(a):
    return pltpu.bitcast(a, BF16)


def _cat(xs, axis=0):
    return jnp.concatenate(xs, axis=axis)


def _split(a):
    w = _pk(a)
    return [pltpu.unpack_elementwise(w, index=j, packed_dtype=BF16, unpacked_dtype=F32) for j in range(2)]


def _pack(e, o):
    return pltpu.pack_elementwise([e, o], packed_dtype=BF16)


def _pack16(a):
    r = _rows8(a)
    return _pack(_cat(r[0::2]), _cat(r[1::2]))


def _unpack16(w):
    e, o = [_rows8(pltpu.unpack_elementwise(w, index=j, packed_dtype=BF16, unpacked_dtype=F32)) for j in range(2)]
    return _cat([x for p in zip(e, o) for x in p])


def _bf(xs):
    return [a.astype(BF16) for a in xs]


def _combos(x11, x12, x21, x22):
    return [x11 + x22, x21 + x22, x11, x22, x11 + x12, x21 - x11, x12 - x22]


def _combos_t(x11, x12, x21, x22):
    return _combos(x11, x21, x12, x22)


def _uncombos(m):
    return (m[0] + m[3] - m[4] + m[6], m[2] + m[4], m[1] + m[3], m[0] - m[1] + m[2] + m[5])


def _uncombos_t(m):
    c11, c12, c21, c22 = _uncombos(m)
    return c11, c21, c12, c22


def _quarters(x):
    r, c = x.shape[0] // 2, x.shape[1] // 2
    return x[:r, :c], x[:r, c:], x[r:, :c], x[r:, c:]


def _join(x11, x12, x21, x22):
    return _cat([_cat([x11, x12], 1), _cat([x21, x22], 1)])


def _set_a(x):
    x11, x12, x21, x22 = _quarters(x)
    return [x11, x21, x12, x22, x11 + x12, x21 + x22, x11 + x22, x21 - x11, x12 - x22]


def _groups(x):
    n = x.shape[0] // 7
    return x[:4 * n], [x[(4 + j) * n:(5 + j) * n] for j in range(3)]


def _halves(x, axis=1):
    n = x.shape[axis] // 2
    return (x[:, :n], x[:, n:]) if axis else (x[:n], x[n:])


def _set_x(x):
    top, g = _groups(x)
    (l1, r1), (l2, r2), (l3, r3) = [_halves(a) for a in g]
    return _combos(*_quarters(top)) + [_cat([l2, r3]), _cat([r1, l2 + r2]), _cat([l1, l3 + r3])]


def _set_w(x):
    top, g = _groups(x)
    (l1, r1), (l2, r2), (l3, r3) = [_halves(a) for a in g]
    d1 = r1 - l1
    ext = [[], [r2, -r3], [l1, l2], [r1, r3], [-l2, l3], [d1, r2 - l2], [-d1, l3 - r3]]
    return [_cat([c] + e) for c, e in zip(_combos_t(*_quarters(top)), ext)]


def _set_f(x):
    top, g = _groups(x)
    (l1, r1), (l2, r2), (l3, r3) = [_halves(a) for a in g]
    return _combos_t(*_quarters(top)) + [_cat([l1, l2 - r2]), _cat([r1, r3 - l3]), _cat([r2, l3])]


def _wf_set(t):
    low = lax.broadcasted_iota(jnp.int32, (t[0].shape[0] // 2, 128), 1) < KG
    (a0, b0), (a1, b1), (a2, b2), (a3, b3) = [_halves(a, 0) for a in t]
    d2 = b2 - a2
    ext = [None, jnp.where(low, b3, -b3), a2, jnp.where(low, b2, b3), jnp.where(low, -a3, a3), d2,
           jnp.where(low, -d2, a3 - b3)]
    return [c if e is None else _cat([c, e], 1) for c, e in zip(_combos(a0, a1, b0, b1), ext)]


def _wb_set(t):
    low = lax.broadcasted_iota(jnp.int32, (t[0].shape[0] // 2, 128), 1) < KG
    (a0, b0), (a1, b1), (a2, b2), (a3, b3) = [_halves(a, 0) for a in t]
    a13, b13 = jnp.where(low, a2, a3), jnp.where(low, b2, b3)
    ext = [None, a13, b3, a3, b2, a13 + b13, a2 + b2]
    c = _combos_t(a0, a1, b0, b1)
    return [c[BORD[k]] if e is None else _cat([c[BORD[k]], e], 1) for k, e in enumerate(ext)]


def _unit(ref, idx, k, rows=DB // 2, n=1):
    return _up(ref[idx + (slice(rows * k, rows * (k + n)),)])


def _acc(ref, idx, first, val):
    ref[idx] = val if first else ref[idx] + val


TILES = ((0, 128), (128, 256), (256, 384), (320, 448))


def _kernel(xT_h, wqkv_h, wphi_h, wo_h, wg_h, wu_h, wdT_h, dyT_h,
            outT_h, dxT_h, dwqkv_h, dwphi_h, dwo_h, dwg_h, dwu_h, dwdT_h,
            xT_s, dyT_s, rstd_s, doT_s, xa_s, ya_s, xb_s, xbt_s, ybt_s, tr_s,
            wqkv_s, wphi_s, wo_s, wg_s, wu_s, wdT_s,
            wT_s, bd_s, wf_s, wb_s,
            wa_gu, wa_d, wb_gu, wb_d, tmpa_s, tmpb_s,
            hc_s, dguc_s, phik_s, vext_s, kv_acc, kvt_s, kv_s,
            out_acc, dxn_acc, dwgu_acc, dwd_acc, g_acc,
            fold_s, zero_s, dxn_s, out_st, dx_st, dwqkv_st, dwphi_st, dwo_st, dwg_st, dwu_st, dwd_st,
            sem):
    def cols(src, dst, lo, hi, k):
        return pltpu.make_async_copy(src.at[:, pl.ds(lo, hi - lo)], dst.at[:, pl.ds(lo, hi - lo)], sem.at[k])

    def x_copy(i, k):
        return pltpu.make_async_copy(xT_h.at[:, pl.ds(i * TS, TS)], xT_s.at[i], sem.at[k])

    def dy_copy(i, k):
        return pltpu.make_async_copy(dyT_h.at[:, pl.ds(i * TS, TS)], dyT_s.at[i], sem.at[k])

    def xy_in(i):
        return [dy_copy(i, i), x_copy(i, i)]

    def mlp_in(lo, hi, k, mats=slice(None)):
        return [cols(src, dst, lo, hi, k) for src, dst in ((wg_h, wg_s), (wu_h, wu_s), (wdT_h, wdT_s))[mats]]

    def mlp_out(chunks, k):
        lo, hi = chunks[0][0], chunks[-1][0] + chunks[-1][1]
        return [cols(src, dst, lo, hi, k) for src, dst in ((dwg_st, dwg_h), (dwu_st, dwu_h), (dwd_st, dwdT_h))]

    def out_copy(i):
        return pltpu.make_async_copy(out_st.at[i], outT_h.at[:, pl.ds(i * TS, TS)], sem.at[NT + 5])

    def dx_copy(i):
        return pltpu.make_async_copy(dx_st.at[i], dxT_h.at[:, pl.ds(i * TS, TS)], sem.at[NT + 5])

    in_x = [x_copy(0, 0)]
    in_g = mlp_in(0, 256, NT, slice(0, 1)) + [dy_copy(0, NT)]
    in_ud = mlp_in(0, 256, NT + 1, slice(1, 3))
    in_c1 = mlp_in(256, 512, NT + 2)
    in_kv = [pltpu.make_async_copy(wo_h, wo_s, sem.at[NT + 3]), pltpu.make_async_copy(wphi_h, wphi_s, sem.at[NT + 3]),
             cols(wqkv_h, wqkv_s, 384, 3 * D, NT + 3)]
    in_rest = [cols(wqkv_h, wqkv_s, 0, 384, NT + 4)] + mlp_in(512, DF, NT + 4)
    out_mlp = [mlp_out(g, NT + 5) for g in (CHUNKS[0], CHUNKS[1], CHUNKS[2][:1], CHUNKS[2][1:])]
    out_wqkv = [cols(dwqkv_st, dwqkv_h, lo, hi, NT + 5) for lo, hi in ((0, 384), (384, 2 * D), (2 * D, 3 * D))]
    c_dwphi = pltpu.make_async_copy(dwphi_st, dwphi_h, sem.at[NT + 5])
    c_dwo = pltpu.make_async_copy(dwo_st, dwo_h, sem.at[NT + 5])

    def start(cs):
        for c in cs:
            c.start()

    def wait(cs):
        for c in cs:
            c.wait()

    def tied(w, dep):
        return _up(w | _cat([dep] * (w.shape[0] // 8))).astype(F32)

    def tie(v):
        return lax.bitcast_convert_type(v[:8, :128], U32) & zero_s[...]

    def paced(marks, n, lo=0.0, hi=1.0):
        total, deps = sum(t for _, t in marks), []
        for j in range(n):
            pos = (lo + (hi - lo) * j / n) * total
            for v, t in marks:
                if pos < t:
                    break
                pos -= t
            deps.append(tie(v[8 * min(int(pos / t * (v.shape[0] // 8)), v.shape[0] // 8 - 1):]))
        return deps

    def unpack_paced(w, deps, order):
        if deps is not None:
            per = len(order) // len(deps)
            w = w | _cat([_cat([deps[order.index(j) // per]] * (w.shape[1] // 128), 1)
                          for j in range(len(order)) for _ in range(2)])
        return [pltpu.unpack_elementwise(w, index=j, packed_dtype=BF16, unpacked_dtype=F32) for j in range(2)]

    def held(a, dep):
        top = lax.bitcast_convert_type(a[:8], U32) | _cat([dep] * (a.shape[1] // 128), 1)
        top = lax.bitcast_convert_type(top, F32)
        return _cat([top, a[8:]]) if a.shape[0] > 8 else top

    def bd_consts(perm=False):
        def col(shape):
            c = lax.broadcasted_iota(jnp.int32, shape, 1)
            return (c & -16) + 2 * (c & 7) + ((c >> 3) & 1) if perm else c

        r = lax.broadcasted_iota(jnp.int32, (PF, PF), 0)
        c = col((PF, PF))
        row_head = ((r >= DH).astype(jnp.int32) + (r >= 2 * DH).astype(jnp.int32)
                    + (r >= 3 * DH).astype(jnp.int32))
        mask = row_head == 2 * (c >= PR).astype(jnp.int32) + (c & 1)
        sc = col((DH, PF))
        sr = lax.broadcasted_iota(jnp.int32, (DH, PF), 0)
        sel = jnp.where(((sc - PR * (sc >= PR).astype(jnp.int32)) >> 1) == sr, 1.0, 0.0).astype(BF16)
        return mask, sel

    def kv_operands(s):
        def source(p):
            return (p & -16) + ((p & 15) >> 1) + 8 * (p & 1)

        def restore(a):
            return _unpack16(_pk(a.astype(BF16))).astype(BF16)

        r = lax.broadcasted_iota(jnp.int32, (PE, PF), 0)
        c = source(lax.broadcasted_iota(jnp.int32, (PE, PF), 1))
        r = r if s else source(r)
        row_head = jnp.where(r < PR, (r >= DH).astype(jnp.int32), (r >= PR + 4).astype(jnp.int32))
        mask = row_head == (c & 1)
        for p in range(NP):
            m = jnp.where(mask, kv_acc[s, p], 0.0)
            rows, cols = (m.astype(BF16), _up(_pack16(m))) if s else (restore(m), restore(m))
            kvt_s[s, p] = _pk(rows)
            kv_s[s, p] = _pk(restore(cols.astype(F32).T))

    def untile(t):
        return _cat([t[0].T, t[1].T, t[2].T, t[3].T[KG:]])

    def prep_phi():
        tmpa_s[...] = wphi_s[...].astype(F32)
        for d in range(DH):
            tmpb_s[pl.ds(d, H, stride=DH), :] = tmpa_s[H * d:H * d + H, :]

    def prep_bd(perm):
        mask, sel = bd_consts(perm)
        expand = _nn(tmpb_s[...].astype(BF16), sel)
        for g in range(NG):
            bd_s[PF * g:PF * g + PF, :] = jnp.where(mask, expand[PF * g:PF * g + PF], 0.0).astype(BF16)

    def prep_wt(lo, hi):
        for j, (a, b) in enumerate(TILES):
            wT_s[lo // 2:hi // 2, 128 * j:128 * j + 128] = _pk(wqkv_s[a:b, lo:hi].T)

    def fold(t):
        w = _rows8(_cat([_tn(bd_s[PF * g:PF * g + PF, :], _unit(wT_s, (), NG * t + g, PR)) for g in range(NG)]))
        return [[v[:, 128 * j:128 * j + 128] for j in range(4)] for v in (_cat(w[0::2]), _cat(w[1::2]))]

    def store_set(ref, t, make, e, o):
        for k, (p, q) in enumerate(zip(make(e), make(o))):
            ref[t, k, :, :p.shape[1]] = _pack(p, q)

    def split_tiles(tiles, deps=None):
        return zip(*[unpack_paced(_pk(a), deps, RORD['a']) for a in tiles])

    def wunit(ref, t, k):
        return _up(ref[t, k, :, :256 if k else 128])

    def prep_qk(t):
        e, o = fold(t)
        store_set(wf_s, t, _wf_set, e, o)
        return [_up(_pack(p, q)) for p, q in zip(e, o)]

    def prep_qk_t(t, w, deps=None):
        store_set(wb_s, t, _wb_set, *split_tiles([untile([c[a:b] for c in w]) for a, b in TILES], deps))

    def prep_v(deps=None):
        w = _unit(wT_s, (), 2, DB)
        store_set(wf_s, 2, _wf_set, *split_tiles([w[:, 128 * j:128 * j + 128] for j in range(4)], deps))

    def prep_v_t(deps=None):
        store_set(wb_s, 2, _wb_set, *split_tiles([wqkv_s[:, 2 * D + a:2 * D + b] for a, b in TILES], deps))

    def prep_wo(deps=None):
        store_set(wf_s, 3, _wf_set, *split_tiles([wo_s[:, a:b] for a, b in TILES], deps))

    def prep_wo_t(deps=None):
        store_set(wb_s, 3, _wb_set, *split_tiles([wo_s[a:b, :].T for a, b in TILES], deps))

    def prep_mlp(chunks, mats, part, marks=None, lo=0.0, hi=1.0):
        items = [(ch, m) for ch in chunks for m in mats]
        deps = None if marks is None else paced(marks, 7 * len(items), lo, hi)
        for n, ((a, w), m) in enumerate(items):
            f = w // 2
            ref, off, wa, wb = {'g': (wg_s, a, wa_gu, wb_gu), 'u': (wu_s, a + f, wa_gu, wb_gu),
                                'd': (wdT_s, a // 2, wa_d, wb_d)}[m]
            e, o = unpack_paced(_pk(ref[:, a:a + w]), deps and deps[7 * n:7 * n + 7], RORD[part])
            if 'b' in part:
                for k, (p, q) in enumerate(zip(_set_w(e), _set_w(o))):
                    wb[k, :p.shape[0], off:off + f] = _pack(p, q)
            if 'a' in part:
                for k, (p, q) in enumerate(zip(_combos_t(*_quarters(e)), _combos_t(*_quarters(o)))):
                    wa[k, :, off:off + f] = _pack(p, q)

    def unfold_phi(gT, t):
        dphi, dwT = [], []
        low = lax.broadcasted_iota(jnp.int32, (PF, 512), 1)
        dup = (low >= 3 * 128) & (low < 3 * 128 + KG)
        for g in range(NG):
            r = slice(PF * g, PF * g + PF)
            dphi.append(_nt(jnp.where(dup, 0, _unit(wT_s, (), NG * t + g, PR)), gT[r]))
            dwT.append(_nn(bd_s[r, :], gT[r]).astype(BF16))
        return dphi, dwT

    def ragged(get, k, ext, axis):
        return get(k) if ext is None else _cat([get(k), get(ext)], axis)

    def project(w, xs, marks):
        m = {k: _nn(wunit(wf_s, w, k), ragged(xs, BORD[k], XEXT[k], 0)) for k in PORD}
        marks.extend((m[k], 2 if k else 1) for k in PORD)
        return _join(*_uncombos(m))

    def back_project(w, fs, k):
        return _nn(wunit(wb_s, w, k), ragged(lambda j: fs[j], k, FEXT[k], 0))

    def outer(w, a_s, i, fs, first):
        marks = []
        for k in range(7):
            marks.append((_nt(_unit(a_s, (i,), AORD[k]), fs[BORD[k]]), 1))
            _acc(g_acc, (w, slice(DB * k, DB * k + DB)), first, marks[-1][0])
        for k in range(3):
            marks.append((_nt(_unit(a_s, (i,), 2 * k, n=2), fs[7 + k]), 2))
            _acc(g_acc, (w, slice(DB * (7 + 2 * k), DB * (9 + 2 * k))), first, marks[-1][0])
        return marks

    def outer_result(w):
        c11, c12, c21, c22 = _uncombos([g_acc[w, DB * k:DB * k + DB] for k in range(7)])
        p = [g_acc[w, DB * (7 + 2 * k):DB * (9 + 2 * k)] for k in range(3)]
        low = lax.broadcasted_iota(jnp.int32, (D, 128), 1) < KG
        t = [_cat([c11, c21]), _cat([c12, c22]),
             p[0] + jnp.where(low, p[1], pltpu.roll(p[2], KG, 1)), p[1] + p[2]]
        return [a.astype(BF16) for a in t]

    def mlp_pre(bt_s, i, wb, a, w, k):
        lhs = ragged(lambda j: _unit(bt_s, (i,), j, 64), BORD[k], XEXT[k], 1)
        return _nn(lhs, _up(wb[k, :128 if k else 64, a:a + w]))

    def mlp_gu(i, ch, k):
        return mlp_pre(xbt_s, i, wb_gu, ch[0], ch[1], k)

    def mlp_dh(i, ch, k):
        return mlp_pre(ybt_s, i, wb_d, ch[0] // 2, ch[1] // 2, k)

    def mlp_s1(i, n, ch, gum=None, dhm=None):
        gum, dhm = dict(gum or {}), dict(dhm or {})
        for k in PORD:
            if k not in dhm:
                dhm[k] = mlp_dh(i, ch, k)
            if k not in gum:
                gum[k] = mlp_gu(i, ch, k)
        f = ch[1] // 2
        hs, dgus = [], []
        for gu, dh in zip(_uncombos_t(gum), _uncombos_t(dhm)):
            g, u = gu[:, :f], gu[:, f:]
            g2 = g * g
            s = 0.5 * jnp.tanh(g * (C0 + (C0 * C1) * g2)) + 0.5
            gelu = g * s
            dgelu = s + gelu * (1.0 - s) * (2.0 * C0 + (6.0 * C0 * C1) * g2)
            hs.append(gelu * u)
            dgus.append(_cat([dh * u * dgelu, dh * gelu], 1))
        for k, (h, dgu) in enumerate(zip(_combos(*hs), _combos(*dgus))):
            hc_s[k, :, f * n:f * n + f] = pack_tokens(h)
            dguc_s[k, :, 2 * f * n:2 * f * n + 2 * f] = pack_tokens(dgu)

    def pack_tokens(a):
        r = _rows8(a)
        return _pack(_cat([x for j, x in enumerate(r) if not j & 2]), _cat([x for j, x in enumerate(r) if j & 2]))

    def mlp_out_p(chunks, k):
        a, w = chunks[0][0], sum(c[1] for c in chunks)
        return _nt(_up(wa_d[BORD[k], :, a // 2:(a + w) // 2]), _up(hc_s[k, :, :w // 2]))

    def mlp_dx_p(chunks, k):
        a, w = chunks[0][0], sum(c[1] for c in chunks)
        return _nt(_up(wa_gu[BORD[k], :, a:a + w]), _up(dguc_s[k, :, :w]))

    def mlp_s2b(i, n, ch, mode, hooks={}):
        a, w = ch
        marks = []
        f = w // 2
        for a_s, src, acc, wd, dsts in ((ya_s, hc_s, dwd_acc, f, (dwd_st,)),
                                        (xa_s, dguc_s, dwgu_acc, w, (dwg_st, dwu_st))):
            m = []
            for k in range(7):
                v = _nn(_unit(a_s, (i,), AORD[k]), _up(src[BORD[k], :, wd * n:wd * n + wd]))
                idx = (k, slice(None), slice(wd * n, wd * n + wd))
                marks.append((v, wd // 128))
                if len(marks) in hooks:
                    hooks[len(marks)](marks)
                if mode == 'last':
                    m.append(acc[idx] + v)
                else:
                    _acc(acc, idx, mode == 'first', v)
            if mode == 'last':
                q = _uncombos(m)
                for j, dst in enumerate(dsts):
                    dst[:, a:a + w] = _join(*[v[:, f * j:f * j + f] for v in q]).astype(BF16)
        return marks

    def store_sets(i, e, o, a_s, bt_s, slot):
        b = [_pack(p, q) for p, q in zip(_set_x(e), _set_x(o))]
        for k, w in enumerate(b):
            tr_s[slot, 64 * k:64 * k + 64] = _pk(_up(w).T)
            for j in range(4):
                base = 64 * k + 16 * j
                p, q = [_split(_up(tr_s[slot, pl.ds(base + c, 8, stride=2), :])) for c in range(2)]
                bt_s[i, base:base + 16] = _cat([_pack(p[0], q[0]), _pack(p[1], q[1])])
        a_s[i, :9 * DB // 2] = _cat([_pack(p, q) for p, q in zip(_set_a(e), _set_a(o))])
        return b

    def dy_sets(i, deps=None):
        return [_up(w) for w in store_sets(i, *unpack_paced(_pk(dyT_s[i]), deps, RORD['ab']), ya_s, ybt_s, 0)]

    def all_rows(v):
        v = _tree(jnp.add, _rows8(v))
        return _pair_reduce(jnp.add, [v + pltpu.roll(v, 1, 0)])

    def layernorm(i, deps=(None, None, None)):
        w = _pk(xT_s[i])
        e, o = unpack_paced(w, deps[0], RORD['n'])
        mean = _cat([all_rows(e + o) * (1.0 / D)] * (DB // 8))
        e, o = [v - mean for v in unpack_paced(w, deps[1], RORD['n'])]
        rstd = lax.rsqrt(all_rows(e * e + o * o) * (1.0 / D) + LN_EPS)
        rstd_s[i, 0:8] = rstd
        rstd = _cat([rstd] * (DB // 8))
        e, o = [(v - mean) * rstd for v in unpack_paced(w, deps[2], RORD['ab'])]
        xb_s[i] = _cat(store_sets(i, e, o, xa_s, xbt_s, 1))

    def xproj(i, t, marks=None):
        return project(t, lambda k: _unit(xb_s, (i,), k, 64), [] if marks is None else marks)

    def do_proj(i, yb, marks=None):
        doT_s[i] = _pack16(project(3, lambda k: yb[k], [] if marks is None else marks))

    def key_side(i, pk, v, first, deps=None):
        ones = jnp.ones((8, TS), F32)
        for c in range(NP):
            p = pk[PR * c:PR * c + PR]
            phik = _pack16(_softmax_pair(p if deps is None else held(p, deps[c])))
            phik_s[i, PR * c:PR * c + PR, :] = phik
            vext = _pack16(_cat([v[PR * c:PR * c + PR], ones]))
            vext_s[i, 32 * c:32 * c + 32, :] = vext
            _acc(kv_acc, (0, c), first, _nt(_up(vext), _up(phik)))

    def phase1_tail(i):
        mo = [mlp_out_p(CHUNKS[0], k) for k in range(7)]
        mdx = [mlp_dx_p(CHUNKS[0], k) for k in range(7)]
        for k, (o, dx) in enumerate(zip(mo, mdx)):
            out_acc[i, k] = o
            dxn_acc[i, k] = dx
        return [(o, 1) for o in mo] + [(dx, 2) for dx in mdx]

    c0, c1 = CHUNKS[0]
    start(in_x + in_g + in_ud + in_c1 + in_kv)
    for i in range(1, NT):
        start(xy_in(i))
    start(in_rest)
    with jax.named_scope('w_0'):
        wait(in_x)
    zero_s[...] = (_pk(xT_s[0, 0:16, 0:128]) >> 16) >> 16
    layernorm(0)
    with jax.named_scope('w_1'):
        wait(in_g)
    prep_mlp([c0], 'g', 'ab')
    g = {k: mlp_pre(xbt_s, 0, wb_gu, 0, 128, k) for k in PORD}
    yb = dy_sets(0)
    with jax.named_scope('w_2'):
        wait(in_ud)
    prep_mlp([c0], 'ud', 'b')
    gu = {k: _cat([g[k], mlp_pre(xbt_s, 0, wb_gu, 128, 128, k)], 1) for k in PORD}
    mlp_s1(0, 0, c0, gu)

    def next_chunk(marks):
        prep_mlp([c0], 'ud', 'a', marks, 0.0, 0.9)
        with jax.named_scope('w_4'):
            wait(in_c1)

    marks = mlp_s2b(0, 0, c0, 'first', {10: next_chunk})
    prep_mlp([c1], 'dgu', 'b', marks[10:])
    mlp_s1(0, 1, c1)
    folded = []

    def attn_prep(marks):
        prep_mlp([c1], 'd', 'a', marks, 0.0, 0.8)
        with jax.named_scope('w_5'):
            wait(in_kv)
        prep_phi()
        prep_wt(384, 2 * D)

    marks = mlp_s2b(0, 1, c1, 'first', {7: attn_prep, 10: lambda m: prep_bd(True),
                                        12: lambda m: folded.extend(prep_qk(1))})
    prep_wo(paced(marks[7:], 7))
    marks = []
    pk = xproj(0, 1, marks)
    prep_wt(2 * D, 3 * D)
    prep_v(paced(marks, 7, 0.5))
    marks = []
    v = xproj(0, 2, marks)
    do_proj(0, yb, marks)
    key_side(0, pk, v, True, paced(marks, NP, 0.0, 0.7))
    prep_mlp([c1], 'gu', 'a', marks, 0.5, 0.95)
    fold_s[...] = _pk(_cat(folded, 1))

    def phase1(i, mode):
        wait(xy_in(i))
        marks = phase1_tail(i - 1)
        yb = dy_sets(i, paced(marks, 14, 0.0, 0.3))
        layernorm(i, (paced(marks, 7, 0.3, 0.42), paced(marks, 7, 0.44, 0.58), paced(marks, 14, 0.6, 1.0)))
        do_proj(i, yb)
        mlp_s1(i, 0, c0)
        pk = xproj(i, 1)
        mlp_s1(i, 1, c1)
        v = xproj(i, 2)
        if mode == 'last':
            prep_wt(0, 384)
            prep_qk_t(0, prep_qk(0))
        marks = mlp_s2b(i, 0, c0, mode)
        key_side(i, pk, v, False, paced(marks, NP, 0.0, 0.8) if mode == 'mid' else None)
        mlp_s2b(i, 1, c1, mode)

    def loop(name, f):
        def body(i, carry):
            with jax.named_scope('it' + name):
                f(i, 'mid')
            return carry
        with jax.named_scope('p' + name):
            lax.fori_loop(1, NT - 1, body, 0)

    loop('1', phase1)
    wait(in_rest)
    phase1(NT - 1, 'last')
    start(out_mlp[0])
    kv_operands(0)
    prep_mlp(CHUNKS[1], 'dgu', 'b', phase1_tail(NT - 1))

    def phase2(i, mode):
        first = mode == 'first'
        lo4 = lax.broadcasted_iota(jnp.int32, (8, TS), 0) < 4
        ch = CHUNKS[1]

        def s1(n):
            mlp_s1(i, n, ch[n])

        s1(0)
        pq = xproj(i, 0)
        marks = mlp_s2b(i, 0, ch[0], mode)
        deps = paced(marks, NP, 0.0, 0.8)
        phibs, nes = [], []
        for c in range(NP):
            phi = _softmax_pair(held(pq[PR * c:PR * c + PR], deps[c]))
            phibs.append(_up(_pack16(phi)))
            nes.append(_rows8(_nn(_up(kvt_s[0, c]), phibs[c])))
        s1(1)
        o_all, dp_all = [], []
        doT = _unpack16(doT_s[i])
        for c in range(NP):
            ne = nes[c]
            r = 1.0 / (ne[7] + DEN_EPS)
            rr = pltpu.roll(r, 4, 0)
            ra = jnp.where(lo4, r, rr)
            rb = jnp.where(lo4, rr, r)
            rs = [ra, ra, ra, r, rb, rb, rb]
            o = [n * w for n, w in zip(ne[:7], rs)]
            dnum = [n * w for n, w in zip(_rows8(doT[PR * c:PR * c + PR]), rs)]
            t = [a * b for a, b in zip(dnum, o)]
            sa = t[0] + t[1] + t[2]
            sb = t[4] + t[5] + t[6]
            e = jnp.where(lo4, sa, sb) + pltpu.roll(jnp.where(lo4, sb, sa), 4, 0) + t[3]
            dne = _cat(dnum + [-e]).astype(BF16)
            dphi = _nn(_up(kv_s[0, c]), dne)
            _acc(kv_acc, (1, c), first, _nt(dne, phibs[c]))
            dp_all.append(_softmax_pair_bwd(_unpack16(_pk(phibs[c])), dphi))
            o_all.extend(o)
        marks = mlp_s2b(i, 1, ch[1], mode)
        deps = paced(marks, 14, 0.45, 0.95)
        o_all = [held(o, deps[RORD['b'].index(j // 4)]) for j, o in enumerate(o_all)]
        s1(2)
        ob = _bf(_set_f(_cat(o_all)))
        dpb = _bf(_set_f(_cat(dp_all)))
        marks = outer(3, ya_s, i, ob, first)
        marks += outer(0, xa_s, i, dpb, first)
        if first:
            marks += mlp_s2b(i, 2, ch[2], mode)
            prep_mlp(ch, 'dgu', 'a', marks, 0.2, 0.95)
            prep_wo_t()
        marks = []
        for k in range(7):
            marks.append((out_acc[i, k] + mlp_out_p(ch, k) + back_project(3, ob, k), 5))
            out_acc[i, k] = marks[-1][0]
        for k in range(7):
            marks.append((dxn_acc[i, k] + mlp_dx_p(ch, k) + back_project(0, dpb, k), 8))
            dxn_acc[i, k] = marks[-1][0]
        if mode == 'last':
            prep_mlp(CHUNKS[2], 'dgu', 'ab', marks, 0.0, 0.7)
            prep_v_t(paced(marks, 7, 0.7, 0.8))
            prep_qk_t(1, [_up(fold_s[:, 128 * j:128 * j + 128]) for j in range(4)], paced(marks, 7, 0.8, 0.9))
        if not first:
            mlp_s2b(i, 2, ch[2], mode)

    phase2(0, 'first')
    loop('2', phase2)
    phase2(NT - 1, 'last')
    start(out_mlp[1])
    kv_operands(1)

    def key_bwd(i):
        dv_all, dp_all = [], []
        for c in range(NP):
            phik = _up(phik_s[i, PR * c:PR * c + PR, :])
            dphik = _nn(_up(kv_s[1, c]), _up(vext_s[i, 32 * c:32 * c + 32, :]))
            dv_all.append(_nn(_up(kvt_s[1, c]), phik)[0:PR])
            dp_all.append(_softmax_pair_bwd(_unpack16(_pk(phik)), dphik))
        return _bf(_set_f(_cat(dp_all))), _bf(_set_f(_cat(dv_all)))

    def dx_products(i, dkb, dvb, deps={}):
        acc = {k: held(dxn_acc[i, k], deps[k]) if k in deps else dxn_acc[i, k] for k in PORD}
        return {k: acc[k] + back_project(2, dvb, k) + back_project(1, dkb, k) + mlp_dx_p(CHUNKS[2], k)
                for k in PORD}

    def rows_of(a_s, i, r, n, dep):
        return _cat([tied(a_s[i, DB * h + r // 2:DB * h + (r + n) // 2], dep) for h in range(2)], 1)

    def finish_dx(i, m, marks):
        q = _uncombos_t(m)
        s1, s2 = [None, None], [None, None]
        for j in (1, 2, 0, 3):
            h = j & 1
            for r in range(0, DB, 32):
                d = q[j][r:r + 32]
                dxn_s[DB * (j >> 1) + r:DB * (j >> 1) + r + 32, SB * h:SB * h + SB] = d
                t1 = _tree(jnp.add, _rows8(d))
                w = DB * h + (DB * (j >> 1) + r) // 2
                t2 = _tree(jnp.add, _rows8(d * tied(xa_s[i, w:w + 16], tie(t1 if s2[h] is None else s2[h]))))
                s1[h], s2[h] = (t1, t2) if s1[h] is None else (s1[h] + t1, s2[h] + t2)
        m1, m2 = [_cat([all_rows(v) * (1.0 / D)] * 2) for v in (_cat(s1, 1), _cat(s2, 1))]
        rstd = _cat([rstd_s[i, 0:8]] * 2)
        for r, dep in zip(range(0, D, 16), paced(marks, D // 16)):
            t = dxn_s[r:r + 16] - (rows_of(xa_s, i, r, 16, dep) * m2 + m1)
            t = rows_of(ya_s, i, r, 16, dep) + rstd * t
            dx_st[i, r:r + 16] = t.astype(BF16)

    def finish_out(i):
        m = {k: out_acc[i, k] + mlp_out_p(CHUNKS[2], k) for k in TORD}
        out_st[i] = (xT_s[i].astype(F32) + _join(*_uncombos_t(m))).astype(BF16)
        return [(m[k], 1) for k in TORD]

    def phase3(i, mode):
        first = mode == 'first'
        ch = CHUNKS[2]
        if first:
            mlp_s1(i, 0, ch[0])
            dkb, dvb = key_bwd(i)
        else:
            dkb, dvb = key_bwd(i)
            mlp_s1(i, 0, ch[0])
        mlp_s1(i, 1, ch[1])
        outer(2, xa_s, i, dvb, first)
        outer(1, xa_s, i, dkb, first)
        m = dx_products(i, dkb, dvb)
        finish_out(i)
        marks = mlp_s2b(i, 0, ch[0], mode)
        mlp_s2b(i, 1, ch[1], mode)
        finish_dx(i, m, marks)
        start([out_copy(i), dx_copy(i)])

    def tiles_t(t):
        return _cat([untile([a[lo:hi] for a in t]) for lo, hi in TILES], 1)

    phase3(0, 'first')
    prep_bd(False)
    dwo_t = outer_result(3)
    dwo_st[...] = _cat([a.T for a in dwo_t[:3]] + [dwo_t[3].T[KG:]])
    start([c_dwo])
    loop('3', phase3)

    i = NT - 1
    ch = CHUNKS[2]
    dkb, dvb = key_bwd(i)
    mlp_s1(i, 0, ch[0])
    dphi_q, dwT_q = unfold_phi(tiles_t(outer_result(0)), 0)
    dwT_q = _cat(dwT_q)
    dwqkv_st[:, 0:384] = untile([dwT_q[:384, 128 * j:128 * j + 128] for j in range(4)])
    start(out_wqkv[:1])
    mlp_s1(i, 1, ch[1])
    outer(1, xa_s, i, dkb, False)
    outer(2, xa_s, i, dvb, False)
    gv = outer_result(2)
    dwqkv_st[:, 2 * D:3 * D] = _cat(gv[:3] + [gv[3][:, KG:]], 1)
    start(out_wqkv[2:])
    dphi_k, dwT_k = unfold_phi(tiles_t(outer_result(1)), 1)
    mlp_s2b(i, 0, ch[0], 'last')
    start(out_mlp[2])
    dwT = _cat([dwT_q[384:]] + dwT_k)
    dwk = untile([dwT[:, 128 * j:128 * j + 128] for j in range(4)])
    dwqkv_st[:, 384:2 * D] = dwk
    done = [_pk(dwk[r - 16:r, 128 * j:128 * j + 128]) for j in range(4) for r in (128, 256, 384, 448)]
    mask, sel = bd_consts()
    for g in range(NG):
        dg = jnp.where(mask, dphi_q[g] + dphi_k[g], 0.0).astype(BF16)
        tmpa_s[PF * g:PF * g + PF, :] = _nt(dg, sel)
    for d in range(DH):
        dwphi_st[H * d:H * d + H, :] = tmpa_s[pl.ds(d, H, stride=DH), :].astype(BF16)
    mlp_s2b(i, 1, ch[1], 'last')
    start(out_mlp[3] + [out_wqkv[1], c_dwphi])
    m = dx_products(i, dkb, dvb, {PORD[0]: _tree(jnp.bitwise_or, done) & zero_s[...]})
    finish_dx(i, m, finish_out(i)[1:6])
    start([dx_copy(i), out_copy(i)])

    with jax.named_scope('w_end'):
        wait(sum(out_mlp, []) + out_wqkv + [c_dwo, c_dwphi])
        for i in range(NT):
            wait([out_copy(i), dx_copy(i)])


@jax.jit
def pallas_parallel_sum__linear_kernel_hedgehog__glu_gated_geglu__prompt_kernel(
    A_x: jax.Array,
    A_wqkv: jax.Array,
    A_w_phi: jax.Array,
    A_wo: jax.Array,
    B_x: jax.Array,
    B_w_gate: jax.Array,
    B_w_up: jax.Array,
    B_w_down: jax.Array,
    grad_out: jax.Array,
):
    del B_x
    xT = A_x.reshape(S, D).T
    dyT = grad_out.reshape(S, D).T
    wphi2 = A_w_phi.transpose(1, 0, 2).reshape(D, DH)
    wdT = B_w_down.T

    V = pltpu.VMEM
    dma = pltpu.SemaphoreType.DMA
    scratch = [
        V((NT, D, TS), BF16), V((NT, D, TS), BF16),
        V((NT, 32, TS), F32), V((NT, DB, TS), U32),
        V((NT, 1024, SB), U32), V((NT, 1024, SB), U32),
        V((NT, 640, SB), U32), V((NT, 640, 128), U32), V((NT, 640, 128), U32),
        V((2, 640, 128), U32),
        V((D, 3 * D), BF16), V((D, DH), BF16), V((D, D), BF16),
        V((D, DF), BF16), V((D, DF), BF16), V((D, DF), BF16),
        V((3 * DB, 512), U32), V((D, PF), BF16),
        V((4, 7, DB // 2, 256), U32), V((4, 7, DB // 2, 256), U32),
        V((7, DB // 2, DF), U32), V((7, DB // 2, DF // 2), U32),
        V((7, 128, DF), U32), V((7, 128, DF // 2), U32),
        V((D, DH), F32), V((D, DH), F32),
        V((7, SB // 2, 384), U32), V((7, SB // 2, 768), U32),
        V((NT, NP * PR, TS), U32), V((NT, NP * 32, TS), U32),
        V((2, NP, PE, PF), F32), V((2, NP, PE // 2, PF), U32), V((2, NP, PR, PE), U32),
        V((NT, 8, DB, SB), F32), V((NT, 8, DB, SB), F32),
        V((7, DB, 768), F32), V((7, DB, 384), F32),
        V((4, 13 * DB, 128), F32),
        V((DB, 512), U32), V((8, 128), U32), V((D, TS), F32),
        V((NT, D, TS), BF16), V((NT, D, TS), BF16),
        V((D, 3 * D), BF16), V((D, DH), BF16), V((D, D), BF16),
        V((D, DF), BF16), V((D, DF), BF16), V((D, DF), BF16),
        dma((NT + 6,)),
    ]
    sds = jax.ShapeDtypeStruct
    out_shape = (
        sds((D, S), BF16), sds((D, S), BF16), sds((D, 3 * D), BF16), sds((D, DH), BF16),
        sds((D, D), BF16), sds((D, DF), BF16), sds((D, DF), BF16), sds((D, DF), BF16),
    )
    any_spec = pl.BlockSpec(memory_space=pl.ANY)
    outT, dxT, dwqkv, dwphi2, dwo, dwg, dwu, dwdT = pl.pallas_call(
        _kernel,
        out_shape=out_shape,
        in_specs=[any_spec] * 8,
        out_specs=[any_spec] * 8,
        scratch_shapes=scratch,
        compiler_params=pltpu.CompilerParams(vmem_limit_bytes=120 * 1024 * 1024),
        name="hedgehog_geglu",
    )(xT, A_wqkv, wphi2, A_wo, B_w_gate, B_w_up, wdT, dyT)
    return (
        outT.T.reshape(1, S, D),
        dxT.T.reshape(1, S, D),
        dwqkv,
        dwphi2.reshape(DH, H, DH).transpose(1, 0, 2),
        dwo,
        dwg,
        dwu,
        dwdT.T,
    )
```

```python
import math

import jax
import jax.numpy as jnp
from jax import lax
import jax.experimental.pallas as pl
import jax.experimental.pallas.tpu as pltpu

S, D, H, DH, DF = 2048, 448, 16, 28, 1792
NP = H // 2
PR = 2 * DH
PF = 2 * PR
PE = PR + 8
NG = H // 4
TS = 256
NT = S // TS
SB, DB = TS // 2, D // 2
AORD = (6, 5, 0, 3, 4, 7, 8)
PORD = (1, 3, 2, 4, 0, 6, 5)
TORD = (1, 3, 0, 4, 6, 2, 5)
RORD = {'ab': (0, 7, 4, 11, 1, 8, 5, 12, 2, 9, 6, 13, 3, 10), 'a': (0, 7, 1, 8, 2, 9, 3, 10, 4, 11, 5, 12, 6, 13),
        'b': (0, 4, 1, 5, 2, 6, 3, 7, 8, 9, 10, 11, 12, 13), 'n': tuple(range(14))}
XEXT = (None, 7, 8, 9, 7, 8, 9)
FEXT = (None, 8, 9, 9, 7, 8, 7)
KS, KG = 256, 64
BORD = (0, 2, 6, 5, 3, 4, 1)
CHUNKS = (((0, 256), (256, 256)),
          ((512, 256), (768, 256), (1024, 256)),
          ((1280, 256), (1536, 256)))
QPLAN = {
    'mid': {0: [('f', (0, 1))], 1: [('f', (2,))], 2: [('f', (3,))], 3: [('f', (4,))], 4: [('f', (5,))], 5: [('f', (6,)), ('n', (0, 1, 2, 3))], 6: [('f', (7,))], 7: [('b', (0, 1))], 10: [('b', (2, 3))], 13: [('n', (4, 5, 6, 7))], 20: [('b', (4, 5))], 27: [('b', (6, 7))]},
    'first': {0: [('f', (0, 1))], 1: [('f', (2, 3))], 2: [('f', (4, 5))], 3: [('f', (6, 7)), ('n', (0, 1, 2, 3))],
              5: [('b', (0, 1))], 7: [('b', (2, 3)), ('n', (4, 5, 6, 7))], 9: [('b', (4, 5))], 12: [('b', (6, 7))]},
}
LN_EPS = 1e-5
DEN_EPS = 1e-6
C0 = math.sqrt(2.0 / math.pi)
C1 = 0.044715
F32, BF16, U32 = jnp.float32, jnp.bfloat16, jnp.uint32


def _nn(a, b):
    return lax.dot_general(a, b, (((1,), (0,)), ((), ())), preferred_element_type=F32)


def _nt(a, b):
    return lax.dot_general(a, b, (((1,), (1,)), ((), ())), preferred_element_type=F32)


def _tn(a, b):
    return lax.dot_general(a, b, (((0,), (0,)), ((), ())), preferred_element_type=F32)


def _tree(op, xs):
    xs = list(xs)
    while len(xs) > 1:
        nxt = [op(xs[i], xs[i + 1]) for i in range(0, len(xs) - 1, 2)]
        if len(xs) % 2:
            nxt.append(xs[-1])
        xs = nxt
    return xs[0]


def _rows8(a):
    return [a[8 * i:8 * i + 8] for i in range(a.shape[0] // 8)]


def _pair_reduce(op, rows):
    v = _tree(op, rows)
    v = op(v, pltpu.roll(v, 2, 0))
    return op(v, pltpu.roll(v, 4, 0))


def _softmax_pair(p):
    rows = _rows8(p)
    mx = _pair_reduce(jnp.maximum, rows)
    mn = _pair_reduce(jnp.minimum, rows)
    ep = [jnp.exp(r - mx) for r in rows]
    en = [jnp.exp(mn - r) for r in rows]
    rp = 1.0 / _pair_reduce(jnp.add, ep)
    rn = 1.0 / _pair_reduce(jnp.add, en)
    return jnp.concatenate([e * rp for e in ep] + [e * rn for e in en], axis=0)


def _softmax_pair_bwd(phi, dphi):
    pr, dr = _rows8(phi), _rows8(dphi)
    t = [a * b for a, b in zip(pr, dr)]
    sp = _pair_reduce(jnp.add, t[:7])
    sn = _pair_reduce(jnp.add, t[7:])
    out = [(t[i] - t[7 + i]) - (pr[i] * sp - pr[7 + i] * sn) for i in range(7)]
    return jnp.concatenate(out, axis=0)


def _pk(a):
    return pltpu.bitcast(a, U32)


def _up(a):
    return pltpu.bitcast(a, BF16)


def _cat(xs, axis=0):
    return jnp.concatenate(xs, axis=axis)


def _split(a):
    w = _pk(a)
    return [pltpu.unpack_elementwise(w, index=j, packed_dtype=BF16, unpacked_dtype=F32) for j in range(2)]


def _pack(e, o):
    return pltpu.pack_elementwise([e, o], packed_dtype=BF16)


def _pack16(a):
    r = _rows8(a)
    return _pack(_cat(r[0::2]), _cat(r[1::2]))


def _unpack16(w):
    e, o = [_rows8(pltpu.unpack_elementwise(w, index=j, packed_dtype=BF16, unpacked_dtype=F32)) for j in range(2)]
    return _cat([x for p in zip(e, o) for x in p])


def _bf(xs):
    return [a.astype(BF16) for a in xs]


def _combos(x11, x12, x21, x22):
    return [x11 + x22, x21 + x22, x11, x22, x11 + x12, x21 - x11, x12 - x22]


def _combos_t(x11, x12, x21, x22):
    return _combos(x11, x21, x12, x22)


def _uncombos(m):
    return (m[0] + m[3] - m[4] + m[6], m[2] + m[4], m[1] + m[3], m[0] - m[1] + m[2] + m[5])


def _uncombos_t(m):
    c11, c12, c21, c22 = _uncombos(m)
    return c11, c21, c12, c22


def _quarters(x):
    r, c = x.shape[0] // 2, x.shape[1] // 2
    return x[:r, :c], x[:r, c:], x[r:, :c], x[r:, c:]


def _join(x11, x12, x21, x22):
    return _cat([_cat([x11, x12], 1), _cat([x21, x22], 1)])


def _set_a(x):
    x11, x12, x21, x22 = _quarters(x)
    return [x11, x21, x12, x22, x11 + x12, x21 + x22, x11 + x22, x21 - x11, x12 - x22]


def _groups(x):
    n = x.shape[0] // 7
    return x[:4 * n], [x[(4 + j) * n:(5 + j) * n] for j in range(3)]


def _halves(x, axis=1):
    n = x.shape[axis] // 2
    return (x[:, :n], x[:, n:]) if axis else (x[:n], x[n:])


def _set_x(x):
    top, g = _groups(x)
    (l1, r1), (l2, r2), (l3, r3) = [_halves(a) for a in g]
    return _combos(*_quarters(top)) + [_cat([l2, r3]), _cat([r1, l2 + r2]), _cat([l1, l3 + r3])]


def _set_w(x):
    top, g = _groups(x)
    (l1, r1), (l2, r2), (l3, r3) = [_halves(a) for a in g]
    d1 = r1 - l1
    ext = [[], [r2, -r3], [l1, l2], [r1, r3], [-l2, l3], [d1, r2 - l2], [-d1, l3 - r3]]
    return [_cat([c] + e) for c, e in zip(_combos_t(*_quarters(top)), ext)]


def _set_f(x):
    top, g = _groups(x)
    (l1, r1), (l2, r2), (l3, r3) = [_halves(a) for a in g]
    return _combos_t(*_quarters(top)) + [_cat([l1, l2 - r2]), _cat([r1, r3 - l3]), _cat([r2, l3])]


def _wf_set(t):
    low = lax.broadcasted_iota(jnp.int32, (t[0].shape[0] // 2, 128), 1) < KG
    (a0, b0), (a1, b1), (a2, b2), (a3, b3) = [_halves(a, 0) for a in t]
    d2 = b2 - a2
    ext = [None, jnp.where(low, b3, -b3), a2, jnp.where(low, b2, b3), jnp.where(low, -a3, a3), d2,
           jnp.where(low, -d2, a3 - b3)]
    return [c if e is None else _cat([c, e], 1) for c, e in zip(_combos(a0, a1, b0, b1), ext)]


def _wb_set(t):
    low = lax.broadcasted_iota(jnp.int32, (t[0].shape[0] // 2, 128), 1) < KG
    (a0, b0), (a1, b1), (a2, b2), (a3, b3) = [_halves(a, 0) for a in t]
    a13, b13 = jnp.where(low, a2, a3), jnp.where(low, b2, b3)
    ext = [None, a13, b3, a3, b2, a13 + b13, a2 + b2]
    c = _combos_t(a0, a1, b0, b1)
    return [c[BORD[k]] if e is None else _cat([c[BORD[k]], e], 1) for k, e in enumerate(ext)]


def _unit(ref, idx, k, rows=DB // 2, n=1):
    return _up(ref[idx + (slice(rows * k, rows * (k + n)),)])


def _acc(ref, idx, first, val):
    ref[idx] = val if first else ref[idx] + val


TILES = ((0, 128), (128, 256), (256, 384), (320, 448))


def _kernel(xT_h, wqkv_h, wphi_h, wo_h, wg_h, wu_h, wdT_h, dyT_h,
            outT_h, dxT_h, dwqkv_h, dwphi_h, dwo_h, dwg_h, dwu_h, dwdT_h,
            xT_s, dyT_s, rstd_s, doT_s, xa_s, ya_s, xb_s, xbt_s, ybt_s, qs_s,
            wqkv_s, wphi_s, wo_s, wg_s, wu_s, wdT_s,
            wT_s, bd_s, wf_s, wb_s,
            wa_gu, wa_d, wb_gu, wb_d, tmpa_s, tmpb_s,
            hc_s, dguc_s, phik_s, vext_s, kv_acc, kvt_s, kv_s,
            out_acc, dxn_acc, dwgu_acc, dwd_acc, g_acc,
            fold_s, zero_s, dxn_s, out_st, dx_st, dwqkv_st, dwphi_st, dwo_st, dwg_st, dwu_st, dwd_st,
            sem):
    def cols(src, dst, lo, hi, k):
        return pltpu.make_async_copy(src.at[:, pl.ds(lo, hi - lo)], dst.at[:, pl.ds(lo, hi - lo)], sem.at[k])

    def x_copy(i, k):
        return pltpu.make_async_copy(xT_h.at[:, pl.ds(i * TS, TS)], xT_s.at[i], sem.at[k])

    def dy_copy(i, k):
        return pltpu.make_async_copy(dyT_h.at[:, pl.ds(i * TS, TS)], dyT_s.at[i], sem.at[k])

    def xy_in(i):
        return [dy_copy(i, i), x_copy(i, i)]

    def mlp_in(lo, hi, k, mats=slice(None)):
        return [cols(src, dst, lo, hi, k) for src, dst in ((wg_h, wg_s), (wu_h, wu_s), (wdT_h, wdT_s))[mats]]

    def mlp_out(chunks, k):
        lo, hi = chunks[0][0], chunks[-1][0] + chunks[-1][1]
        return [cols(src, dst, lo, hi, k) for src, dst in ((dwg_st, dwg_h), (dwu_st, dwu_h), (dwd_st, dwdT_h))]

    def tile_out(i, r=0, n=D):
        return [pltpu.make_async_copy(src.at[i, pl.ds(r, n)], dst.at[pl.ds(r, n), pl.ds(i * TS, TS)], sem.at[NT + 5])
                for src, dst in ((dx_st, dxT_h), (out_st, outT_h))]

    in_x = [x_copy(0, 0)]
    in_g = mlp_in(0, 256, NT, slice(0, 1))
    in_y = [dy_copy(0, NT + 7)]
    in_ud = mlp_in(0, 256, NT + 1, slice(1, 3))
    in_c1 = mlp_in(256, 512, NT + 2)
    in_kv = [pltpu.make_async_copy(wphi_h, wphi_s, sem.at[NT + 3]), cols(wqkv_h, wqkv_s, 384, 2 * D, NT + 3)]
    in_vo = [pltpu.make_async_copy(wo_h, wo_s, sem.at[NT + 6]), cols(wqkv_h, wqkv_s, 2 * D, 3 * D, NT + 6)]
    in_rest = [cols(wqkv_h, wqkv_s, 0, 384, NT + 4)] + mlp_in(512, DF, NT + 4)
    out_mlp = [mlp_out(g, NT + 5) for g in (CHUNKS[0], CHUNKS[1], CHUNKS[2][:1], CHUNKS[2][1:])]
    out_wqkv = [cols(dwqkv_st, dwqkv_h, lo, hi, NT + 5) for lo, hi in ((0, 384), (384, 2 * D), (2 * D, 3 * D))]
    c_dwphi = pltpu.make_async_copy(dwphi_st, dwphi_h, sem.at[NT + 5])
    c_dwo = pltpu.make_async_copy(dwo_st, dwo_h, sem.at[NT + 5])

    def start(cs):
        for c in cs:
            c.start()

    def wait(cs):
        for c in cs:
            c.wait()

    def tied(w, dep):
        return _up(w | _cat([dep] * (w.shape[0] // 8))).astype(F32)

    def tie(v):
        return lax.bitcast_convert_type(v[:8, :128], U32) & zero_s[...]

    def paced(marks, n, lo=0.0, hi=1.0):
        total, deps = sum(t for _, t in marks), []
        for j in range(n):
            pos = (lo + (hi - lo) * j / n) * total
            for v, t in marks:
                if pos < t:
                    break
                pos -= t
            deps.append(tie(v[8 * min(int(pos / t * (v.shape[0] // 8)), v.shape[0] // 8 - 1):]))
        return deps

    def unpack_paced(w, deps, order):
        if deps is not None:
            per = len(order) // len(deps)
            w = w | _cat([_cat([deps[order.index(j) // per]] * (w.shape[1] // 128), 1)
                          for j in range(len(order)) for _ in range(2)])
        return [pltpu.unpack_elementwise(w, index=j, packed_dtype=BF16, unpacked_dtype=F32) for j in range(2)]

    def held(a, dep):
        top = lax.bitcast_convert_type(a[:8], U32) | _cat([dep] * (a.shape[1] // 128), 1)
        top = lax.bitcast_convert_type(top, F32)
        return _cat([top, a[8:]]) if a.shape[0] > 8 else top

    def bd_consts(perm=False):
        def col(shape):
            c = lax.broadcasted_iota(jnp.int32, shape, 1)
            return (c & -16) + 2 * (c & 7) + ((c >> 3) & 1) if perm else c

        r = lax.broadcasted_iota(jnp.int32, (PF, PF), 0)
        c = col((PF, PF))
        row_head = ((r >= DH).astype(jnp.int32) + (r >= 2 * DH).astype(jnp.int32)
                    + (r >= 3 * DH).astype(jnp.int32))
        mask = row_head == 2 * (c >= PR).astype(jnp.int32) + (c & 1)
        sc = col((DH, PF))
        sr = lax.broadcasted_iota(jnp.int32, (DH, PF), 0)
        sel = jnp.where(((sc - PR * (sc >= PR).astype(jnp.int32)) >> 1) == sr, 1.0, 0.0).astype(BF16)
        return mask, sel

    def kv_operands(s):
        def source(p):
            return (p & -16) + ((p & 15) >> 1) + 8 * (p & 1)

        def restore(a):
            return _unpack16(_pk(a.astype(BF16))).astype(BF16)

        r = lax.broadcasted_iota(jnp.int32, (PE, PF), 0)
        c = source(lax.broadcasted_iota(jnp.int32, (PE, PF), 1))
        r = r if s else source(r)
        row_head = jnp.where(r < PR, (r >= DH).astype(jnp.int32), (r >= PR + 4).astype(jnp.int32))
        mask = row_head == (c & 1)
        for p in range(NP):
            m = jnp.where(mask, kv_acc[s, p], 0.0)
            rows, cols = (m.astype(BF16), _up(_pack16(m))) if s else (restore(m), restore(m))
            kvt_s[s, p] = _pk(rows)
            kv_s[s, p] = _pk(restore(cols.astype(F32).T))

    def untile(t):
        return _cat([t[0].T, t[1].T, t[2].T, t[3].T[KG:]])

    def prep_phi():
        tmpa_s[...] = wphi_s[...].astype(F32)
        for d in range(DH):
            tmpb_s[pl.ds(d, H, stride=DH), :] = tmpa_s[H * d:H * d + H, :]

    def prep_bd(perm):
        mask, sel = bd_consts(perm)
        expand = _nn(tmpb_s[...].astype(BF16), sel)
        for g in range(NG):
            bd_s[PF * g:PF * g + PF, :] = jnp.where(mask, expand[PF * g:PF * g + PF], 0.0).astype(BF16)

    def prep_wt(lo, hi):
        for j, (a, b) in enumerate(TILES):
            wT_s[lo // 2:hi // 2, 128 * j:128 * j + 128] = _pk(wqkv_s[a:b, lo:hi].T)

    def fold(t):
        w = _rows8(_cat([_tn(bd_s[PF * g:PF * g + PF, :], _unit(wT_s, (), NG * t + g, PR)) for g in range(NG)]))
        return [[v[:, 128 * j:128 * j + 128] for j in range(4)] for v in (_cat(w[0::2]), _cat(w[1::2]))]

    def store_set(ref, t, make, e, o):
        done = []
        for k, (p, q) in enumerate(zip(make(e), make(o))):
            w = _pack(p, q)
            ref[t, k, :, :p.shape[1]] = w
            done.extend(w[r:r + 8, -128:] for r in (0, 56, 104))
        return _tree(jnp.bitwise_or, done) & zero_s[...]

    def split_tiles(tiles, deps=None):
        return zip(*[unpack_paced(_pk(a), deps, RORD['a']) for a in tiles])

    def wunit(ref, t, k):
        return _up(ref[t, k, :, :256 if k else 128])

    def prep_qk(t):
        e, o = fold(t)
        store_set(wf_s, t, _wf_set, e, o)
        return [_up(_pack(p, q)) for p, q in zip(e, o)]

    def prep_qk_t(t, w, deps=None):
        return store_set(wb_s, t, _wb_set, *split_tiles([untile([c[a:b] for c in w]) for a, b in TILES], deps))

    def prep_v(deps=None):
        w = _unit(wT_s, (), 2, DB)
        store_set(wf_s, 2, _wf_set, *split_tiles([w[:, 128 * j:128 * j + 128] for j in range(4)], deps))

    def prep_v_t(deps=None):
        store_set(wb_s, 2, _wb_set, *split_tiles([wqkv_s[:, 2 * D + a:2 * D + b] for a, b in TILES], deps))

    def prep_wo(deps=None):
        store_set(wf_s, 3, _wf_set, *split_tiles([wo_s[:, a:b] for a, b in TILES], deps))

    def prep_wo_t(deps=None):
        return store_set(wb_s, 3, _wb_set, *split_tiles([wo_s[a:b, :].T for a, b in TILES], deps))

    def prep_mlp(chunks, mats, part, marks=None, lo=0.0, hi=1.0):
        items = [(ch, m) for ch in chunks for m in mats]
        deps = None if marks is None else paced(marks, 7 * len(items), lo, hi)
        for n, ((a, w), m) in enumerate(items):
            f = w // 2
            ref, off, wa, wb = {'g': (wg_s, a, wa_gu, wb_gu), 'u': (wu_s, a + f, wa_gu, wb_gu),
                                'd': (wdT_s, a // 2, wa_d, wb_d)}[m]
            e, o = unpack_paced(_pk(ref[:, a:a + w]), deps and deps[7 * n:7 * n + 7], RORD[part])
            if 'b' in part:
                for k, (p, q) in enumerate(zip(_set_w(e), _set_w(o))):
                    wb[k, :p.shape[0], off:off + f] = _pack(p, q)
            if 'a' in part:
                for k, (p, q) in enumerate(zip(_combos_t(*_quarters(e)), _combos_t(*_quarters(o)))):
                    wa[k, :, off:off + f] = _pack(p, q)

    def unfold_phi(gT, t):
        dphi, dwT = [], []
        low = lax.broadcasted_iota(jnp.int32, (PF, 512), 1)
        dup = (low >= 3 * 128) & (low < 3 * 128 + KG)
        for g in range(NG):
            r = slice(PF * g, PF * g + PF)
            dphi.append(_nt(jnp.where(dup, 0, _unit(wT_s, (), NG * t + g, PR)), gT[r]))
            dwT.append(_nn(bd_s[r, :], gT[r]).astype(BF16))
        return dphi, dwT

    def ragged(get, k, ext, axis):
        return get(k) if ext is None else _cat([get(k), get(ext)], axis)

    def project(w, xs, marks):
        m = {k: _nn(wunit(wf_s, w, k), ragged(xs, BORD[k], XEXT[k], 0)) for k in PORD}
        marks.extend((m[k], 2 if k else 1) for k in PORD)
        return _join(*_uncombos(m))

    def back_project(w, fs, k):
        return _nn(wunit(wb_s, w, k), ragged(lambda j: fs[j], k, FEXT[k], 0))

    def outer(w, a_s, i, fs, first):
        marks = []
        for k in range(7):
            marks.append((_nt(_unit(a_s, (i,), AORD[k]), fs[BORD[k]]), 1))
            _acc(g_acc, (w, slice(DB * k, DB * k + DB)), first, marks[-1][0])
        for k in range(3):
            marks.append((_nt(_unit(a_s, (i,), 2 * k, n=2), fs[7 + k]), 2))
            _acc(g_acc, (w, slice(DB * (7 + 2 * k), DB * (9 + 2 * k))), first, marks[-1][0])
        return marks

    def outer_result(w):
        c11, c12, c21, c22 = _uncombos([g_acc[w, DB * k:DB * k + DB] for k in range(7)])
        p = [g_acc[w, DB * (7 + 2 * k):DB * (9 + 2 * k)] for k in range(3)]
        low = lax.broadcasted_iota(jnp.int32, (D, 128), 1) < KG
        t = [_cat([c11, c21]), _cat([c12, c22]),
             p[0] + jnp.where(low, p[1], pltpu.roll(p[2], KG, 1)), p[1] + p[2]]
        return [a.astype(BF16) for a in t]

    def mlp_pre(bt_s, i, wb, a, w, k, h=None):
        lhs = ragged(lambda j: _unit(bt_s, (i,), j, 64) if h is None else _unit(bt_s, (i,), 2 * j + h, 32),
                     BORD[k], XEXT[k], 1)
        return _nn(lhs, _up(wb[k, :128 if k else 64, a:a + w]))

    def mlp_gu(i, ch, k, h):
        return mlp_pre(xbt_s, i, wb_gu, ch[0], ch[1], k, h)

    def mlp_dh(i, ch, k, h):
        return mlp_pre(ybt_s, i, wb_d, ch[0] // 2, ch[1] // 2, k, h)

    def mlp_s1(i, n, ch, gum=None, split=True):
        for h in range(2) if gum is None and split else (None,):
            mlp_half(i, n, ch, h, gum)

    def mlp_half(i, n, ch, half, gum=None, dhm=None):
        gum, dhm = dict(gum or {}), dict(dhm or {})
        for k in PORD:
            if k not in dhm:
                dhm[k] = mlp_dh(i, ch, k, half)
            if k not in gum:
                gum[k] = mlp_gu(i, ch, k, half)
        f = ch[1] // 2
        hs, dgus = [], []
        for gu, dh in zip(_uncombos_t(gum), _uncombos_t(dhm)):
            g, u = gu[:, :f], gu[:, f:]
            g2 = g * g
            s = 0.5 * jnp.tanh(g * (C0 + (C0 * C1) * g2)) + 0.5
            gelu = g * s
            dgelu = s + gelu * (1.0 - s) * (2.0 * C0 + (6.0 * C0 * C1) * g2)
            hs.append(gelu * u)
            dgus.append(_cat([dh * u * dgelu, dh * gelu], 1))
        for k, (h, dgu) in enumerate(zip(_combos(*hs), _combos(*dgus))):
            r = slice(None) if half is None else slice(32 * half, 32 * half + 32)
            hc_s[k, r, f * n:f * n + f] = pack_tokens(h)
            dguc_s[k, r, 2 * f * n:2 * f * n + 2 * f] = pack_tokens(dgu)

    def pack_tokens(a):
        r = _rows8(a)
        return _pack(_cat([x for j, x in enumerate(r) if not j & 2]), _cat([x for j, x in enumerate(r) if j & 2]))

    def mlp_out_p(chunks, k):
        a, w = chunks[0][0], sum(c[1] for c in chunks)
        return _nt(_up(wa_d[BORD[k], :, a // 2:(a + w) // 2]), _up(hc_s[k, :, :w // 2]))

    def mlp_dx_p(chunks, k):
        a, w = chunks[0][0], sum(c[1] for c in chunks)
        return _nt(_up(wa_gu[BORD[k], :, a:a + w]), _up(dguc_s[k, :, :w]))

    def mlp_s2b(i, n, ch, mode, hooks={}, holds={}):
        a, w = ch
        marks = []
        f = w // 2
        for a_s, src, acc, wd, dsts in ((ya_s, hc_s, dwd_acc, f, (dwd_st,)),
                                        (xa_s, dguc_s, dwgu_acc, w, (dwg_st, dwu_st))):
            m = []
            for k in range(7):
                v = _nn(_unit(a_s, (i,), AORD[k]), _up(src[BORD[k], :, wd * n:wd * n + wd]))
                idx = (k, slice(None), slice(wd * n, wd * n + wd))
                marks.append((v, wd // 128))
                if len(marks) in hooks:
                    hooks[len(marks)](marks)
                if len(marks) in holds:
                    v = held(v, holds[len(marks)])
                if mode == 'last':
                    m.append(acc[idx] + v)
                else:
                    _acc(acc, idx, mode == 'first', v)
            if mode == 'last':
                q = _uncombos(m)
                for j, dst in enumerate(dsts):
                    dst[:, a:a + w] = _join(*[v[:, f * j:f * j + f] for v in q]).astype(BF16)
        return marks

    def store_sets(i, e, o, a_s, bt_s):
        b = [_pack(p, q) for p, q in zip(_set_x(e), _set_x(o))]
        for k, w in enumerate(b):
            p, q = [_rows8(_pk(v.astype(BF16))) for v in _split(_up(w).T)]
            bt_s[i, 64 * k:64 * k + 64] = _cat([x for pair in zip(p, q) for x in pair])
        a_s[i, :9 * DB // 2] = _cat([_pack(p, q) for p, q in zip(_set_a(e), _set_a(o))])
        return b

    def dy_sets(i, deps=None):
        return [_up(w) for w in store_sets(i, *unpack_paced(_pk(dyT_s[i]), deps, RORD['ab']), ya_s, ybt_s)]

    def all_rows(v):
        v = _tree(jnp.add, _rows8(v))
        return _pair_reduce(jnp.add, [v + pltpu.roll(v, 1, 0)])

    def layernorm(i, deps=(None, None, None)):
        w = _pk(xT_s[i])
        e, o = unpack_paced(w, deps[0], RORD['n'])
        mean = _cat([all_rows(e + o) * (1.0 / D)] * (DB // 8))
        e, o = [v - mean for v in unpack_paced(w, deps[1], RORD['n'])]
        rstd = lax.rsqrt(all_rows(e * e + o * o) * (1.0 / D) + LN_EPS)
        rstd_s[i, 0:8] = rstd
        rstd = _cat([rstd] * (DB // 8))
        e, o = [(v - mean) * rstd for v in unpack_paced(w, deps[2], RORD['ab'])]
        xb_s[i] = _cat(store_sets(i, e, o, xa_s, xbt_s))

    def xproj(i, t, marks=None):
        return project(t, lambda k: _unit(xb_s, (i,), k, 64), [] if marks is None else marks)

    def do_proj(i, yb, marks=None):
        doT_s[i] = _pack16(project(3, lambda k: yb[k], [] if marks is None else marks))

    def key_side(i, pk, v, first, deps=None):
        ones = jnp.ones((8, TS), F32)
        for c in range(NP):
            p = pk[PR * c:PR * c + PR]
            phik = _pack16(_softmax_pair(p if deps is None else held(p, deps[c])))
            phik_s[i, PR * c:PR * c + PR, :] = phik
            vext = _pack16(_cat([v[PR * c:PR * c + PR], ones]))
            vext_s[i, 32 * c:32 * c + 32, :] = vext
            _acc(kv_acc, (0, c), first, _nt(_up(vext), _up(phik)))

    def phase1_tail(i):
        mo = [mlp_out_p(CHUNKS[0], k) for k in range(7)]
        mdx = [mlp_dx_p(CHUNKS[0], k) for k in range(7)]
        for k, (o, dx) in enumerate(zip(mo, mdx)):
            out_acc[i, k] = o
            dxn_acc[i, k] = dx
        return [(o, 1) for o in mo] + [(dx, 2) for dx in mdx]

    c0, c1 = CHUNKS[0]
    start(in_x + in_g + in_y + in_ud + in_c1 + in_kv + in_vo)
    for i in range(1, NT):
        start(xy_in(i))
    start(in_rest)
    wait(in_x)
    zero_s[...] = (_pk(xT_s[0, 0:16, 0:128]) >> 16) >> 16
    layernorm(0)
    wait(in_g)
    prep_mlp([c0], 'g', 'ab')
    wait(in_y)
    g = {k: mlp_pre(xbt_s, 0, wb_gu, 0, 128, k) for k in PORD}
    yb = dy_sets(0)
    wait(in_ud)
    prep_mlp([c0], 'ud', 'b')
    gu = {k: _cat([g[k], mlp_pre(xbt_s, 0, wb_gu, 128, 128, k)], 1) for k in PORD}
    mlp_s1(0, 0, c0, gu)

    def next_chunk(marks):
        prep_mlp([c0], 'ud', 'a', marks, 0.0, 0.9)
        wait(in_c1)

    marks = mlp_s2b(0, 0, c0, 'first', {10: next_chunk})
    prep_mlp([c1], 'dgu', 'b', marks[10:])
    mlp_s1(0, 1, c1)
    folded = []

    def attn_prep(marks):
        prep_mlp([c1], 'd', 'a', marks, 0.0, 0.8)
        wait(in_kv)
        prep_phi()
        prep_wt(384, 2 * D)

    marks = mlp_s2b(0, 1, c1, 'first', {7: attn_prep, 10: lambda m: prep_bd(True),
                                        12: lambda m: folded.extend(prep_qk(1))})
    prep_mlp([c1], 'gu', 'a', marks[7:])
    wait(in_vo)
    marks = []
    pk = xproj(0, 1, marks)
    prep_wt(2 * D, 3 * D)
    prep_wo(paced(marks, 7, 0.0, 0.5))
    prep_v(paced(marks, 7, 0.5))
    marks = []
    do_proj(0, yb, marks)
    v = xproj(0, 2, marks)
    key_side(0, pk, v, True, paced(marks, NP, 0.0, 0.8))
    fold_s[...] = _pk(_cat(folded, 1))

    def phase1(i, mode):
        marks = phase1_tail(i - 1)
        yb = dy_sets(i, paced(marks, 14, 0.0, 0.3))
        layernorm(i, (paced(marks, 7, 0.3, 0.42), paced(marks, 7, 0.44, 0.58), paced(marks, 14, 0.6, 1.0)))
        if mode == 'last':
            prep_mlp(CHUNKS[1], 'd', 'a', marks)
        do_proj(i, yb)
        mlp_s1(i, 0, c0, split=mode != 'mid')
        pk = xproj(i, 1)
        mlp_s1(i, 1, c1, split=mode != 'mid')
        marks = []
        v = xproj(i, 2, marks)
        if mode == 'last':
            prep_mlp(CHUNKS[1][:1], 'gu', 'a', marks, 0.4)
            prep_wt(0, 384)
            folded[:] = prep_qk(0)
        marks = mlp_s2b(i, 0, c0, mode)
        key_side(i, pk, v, False, paced(marks, NP, 0.0, 0.8) if mode == 'mid' else None)
        mlp_s2b(i, 1, c1, mode)

    def loop(f, unroll, pre=None, post=None):
        def body(j, carry):
            tiles = [1 + unroll * j + n for n in range(unroll)]
            for g in (pre, lambda i: f(i, 'mid'), post):
                for i in tiles if g else ():
                    g(i)
            return carry
        lax.fori_loop(0, (NT - 2) // unroll, body, 0)

    loop(phase1, 1, pre=lambda i: wait(xy_in(i)))
    wait(in_rest + xy_in(NT - 1))
    phase1(NT - 1, 'last')
    start(out_mlp[0])
    kv_operands(0)
    prep_mlp(CHUNKS[1], 'dgu', 'b', phase1_tail(NT - 1))

    class Query:
        def __init__(self, i, first=False, marks=None):
            self.i, self.first = i, first
            self.pq = xproj(i, 0, marks)
            self.phi, self.ne, self.o, self.dp = {}, {}, {}, {}

        def fwd(self, cs, deps):
            for c, dep in zip(cs, deps):
                self.phi[c] = _up(_pack16(_softmax_pair(held(self.pq[PR * c:PR * c + PR], dep))))

        def num(self, cs):
            for c in cs:
                self.ne[c] = _rows8(_nn(_up(kvt_s[0, c]), self.phi[c]))

        def bwd(self, cs):
            lo4 = lax.broadcasted_iota(jnp.int32, (8, TS), 0) < 4
            dne = {}
            for c in cs:
                ne, r0 = self.ne[c], PR * c // 16 * 8
                do = _unpack16(doT_s[self.i, r0:r0 + 32])[PR * c % 16:PR * c % 16 + PR]
                r = 1.0 / (ne[7] + DEN_EPS)
                rr = pltpu.roll(r, 4, 0)
                ra = jnp.where(lo4, r, rr)
                rb = jnp.where(lo4, rr, r)
                rs = [ra, ra, ra, r, rb, rb, rb]
                o = [n * w for n, w in zip(ne[:7], rs)]
                dnum = [n * w for n, w in zip(_rows8(do), rs)]
                t = [a * b for a, b in zip(dnum, o)]
                sa = t[0] + t[1] + t[2]
                sb = t[4] + t[5] + t[6]
                e = jnp.where(lo4, sa, sb) + pltpu.roll(jnp.where(lo4, sb, sa), 4, 0) + t[3]
                dne[c] = _cat(dnum + [-e]).astype(BF16)
                self.o[c] = _cat(o)
            for c in cs:
                self.dp[c] = _softmax_pair_bwd(_unpack16(_pk(self.phi[c])), _nn(_up(kv_s[0, c]), dne[c]))
            for c in cs:
                _acc(kv_acc, (1, c), self.first, _nt(dne[c], self.phi[c]))

        def sets(self):
            return [_bf(_set_f(_cat([v[c] for c in range(NP)]))) for v in (self.o, self.dp)]

        def store(self):
            done = []
            for j, st in enumerate(self.sets()):
                qs_s[j] = _pk(_cat(st))
                done.extend(_tree(jnp.bitwise_or, _rows8(_pk(a))) for a in st)
            return done

        def after(self, done, n):
            return [_tree(jnp.bitwise_or, done[j::n]) & zero_s[...] for j in range(n)]

    def phase2(i, mode):
        first = mode == 'first'
        ch = CHUNKS[1]

        def s1(n):
            mlp_s1(i, n, ch[n])

        s1(0)
        if first:
            q = Query(i, True)
            marks = mlp_s2b(i, 0, ch[0], mode)
            for c, dep in enumerate(paced(marks, NP, 0.0, 0.8)):
                q.fwd([c], [dep])
                q.num([c])
            s1(1)
            for c in range(0, NP, 2):
                q.bwd((c, c + 1))
            marks = mlp_s2b(i, 1, ch[1], mode, holds={11: prep_qk_t(0, folded), 14: prep_wo_t()})
            deps = paced(marks, 14, 0.45, 0.95)
            for c in range(NP):
                q.o[c] = _cat([held(o, deps[RORD['b'].index((7 * c + j) // 4)]) for j, o in enumerate(_rows8(q.o[c]))])
            s1(2)
            ob, dpb = q.sets()
            marks = outer(3, ya_s, i, ob, first)
            marks += outer(0, xa_s, i, dpb, first)
        else:
            ob, dpb = [[_unit(qs_s, (j,), k, 64) for k in range(10)] for j in range(2)]
            if mode == 'mid':
                outer(3, ya_s, i, ob, first)
            s1(1)
            if mode == 'mid':
                outer(0, xa_s, i, dpb, first)
            s1(2)
        if mode == 'last':
            mlp_s2b(i, 0, ch[0], mode)
            kv_operands(1)
            plan = {}
        else:
            q = Query(i + 1, marks=marks if first else None)
            plan = QPLAN[mode]
            if first:
                prep_mlp(ch[1:], 'gu', 'a', marks, 0.25, 0.9)
        marks, holds = [], {}

        def step(n):
            for op, cs in plan.get(n, ()):
                if op == 'f':
                    q.fwd(cs, paced(marks[-1:], len(cs)))
                else:
                    (q.num if op == 'n' else q.bwd)(cs)

        for k in range(7):
            marks.append((dxn_acc[i, k] + mlp_dx_p(ch, k) + back_project(0, dpb, k), 8))
            dxn_acc[i, k] = marks[-1][0]
            step(k)
        for k in range(7):
            marks.append((out_acc[i, k] + mlp_out_p(ch, k) + back_project(3, ob, k), 5))
            out_acc[i, k] = marks[-1][0]
            step(7 + k)
        if mode == 'last':
            outer(3, ya_s, i, ob, first)
            outer(0, xa_s, i, dpb, first)
        if mode == 'last':
            prep_mlp(CHUNKS[2], 'dgu', 'ab', marks, 0.0, 0.7)
            prep_v_t(paced(marks, 7, 0.7, 0.8))
            prep_qk_t(1, [_up(fold_s[:, 128 * j:128 * j + 128]) for j in range(4)], paced(marks, 7, 0.8, 0.9))
        for n in range({'first': 2, 'mid': 0, 'last': 1}[mode], 3):
            if n == 2 and mode != 'last':
                at = range(10, 15) if first else range(4, 14)
                holds = dict(zip(at, q.after(q.store(), len(at))))
            mlp_s2b(i, n, ch[n], mode, {j: lambda m, j=j: step(14 * n + 13 + j) for j in range(1, 15)}, holds)

    phase2(0, 'first')
    loop(phase2, 1)
    phase2(NT - 1, 'last')
    start(out_mlp[1])

    def key_bwd(i):
        dv_all, dp_all = [], []
        for c in range(NP):
            phik = _up(phik_s[i, PR * c:PR * c + PR, :])
            dphik = _nn(_up(kv_s[1, c]), _up(vext_s[i, 32 * c:32 * c + 32, :]))
            dv_all.append(_nn(_up(kvt_s[1, c]), phik)[0:PR])
            dp_all.append(_softmax_pair_bwd(_unpack16(_pk(phik)), dphik))
        return _bf(_set_f(_cat(dp_all))), _bf(_set_f(_cat(dv_all)))

    def dx_products(i, dkb, dvb, deps={}):
        acc = {k: held(dxn_acc[i, k], deps[k]) if k in deps else dxn_acc[i, k] for k in PORD}
        return {k: acc[k] + back_project(2, dvb, k) + back_project(1, dkb, k) + mlp_dx_p(CHUNKS[2], k)
                for k in PORD}

    def rows_of(a_s, i, r, n, dep):
        return _cat([tied(a_s[i, DB * h + r // 2:DB * h + (r + n) // 2], dep) for h in range(2)], 1)

    def finish_dx(i, m, marks, upper_done=None):
        q = _uncombos_t(m)
        s1, s2 = [None, None], [None, None]
        for j in (1, 2, 0, 3):
            h = j & 1
            for r in range(0, DB, 32):
                d = q[j][r:r + 32]
                dxn_s[DB * (j >> 1) + r:DB * (j >> 1) + r + 32, SB * h:SB * h + SB] = d
                t1 = _tree(jnp.add, _rows8(d))
                w = DB * h + (DB * (j >> 1) + r) // 2
                t2 = _tree(jnp.add, _rows8(d * tied(xa_s[i, w:w + 16], tie(t1 if s2[h] is None else s2[h]))))
                s1[h], s2[h] = (t1, t2) if s1[h] is None else (s1[h] + t1, s2[h] + t2)
        m1, m2 = [_cat([all_rows(v) * (1.0 / D)] * 2) for v in (_cat(s1, 1), _cat(s2, 1))]
        rstd = _cat([rstd_s[i, 0:8]] * 2)
        for r, dep in zip(range(0, D, 16), paced(marks, D // 16)):
            t = dxn_s[r:r + 16] - (rows_of(xa_s, i, r, 16, dep) * m2 + m1)
            t = rows_of(ya_s, i, r, 16, dep) + rstd * t
            dx_st[i, r:r + 16] = t.astype(BF16)
            if upper_done and r + 16 == DB:
                upper_done()

    def finish_out(i):
        m = {k: out_acc[i, k] + mlp_out_p(CHUNKS[2], k) for k in TORD}
        q = _uncombos_t(m)

        def store(h):
            r = slice(DB * h, DB * h + DB)
            out_st[i, r] = (xT_s[i, r].astype(F32) + _cat(q[2 * h:2 * h + 2], 1)).astype(BF16)

        return [(m[k], 1) for k in TORD], store

    def phase3(i, mode):
        first = mode == 'first'
        ch = CHUNKS[2]
        if first:
            mlp_s1(i, 0, ch[0])
            dkb, dvb = key_bwd(i)
        else:
            dkb, dvb = key_bwd(i)
            mlp_s1(i, 0, ch[0])
        mlp_s1(i, 1, ch[1])
        outer(2, xa_s, i, dvb, first)
        outer(1, xa_s, i, dkb, first)
        m = dx_products(i, dkb, dvb)
        store = finish_out(i)[1]
        store(0)
        store(1)
        marks = mlp_s2b(i, 0, ch[0], mode)
        mlp_s2b(i, 1, ch[1], mode)
        finish_dx(i, m, marks)

    def tiles_t(t):
        return _cat([untile([a[lo:hi] for a in t]) for lo, hi in TILES], 1)

    phase3(0, 'first')
    prep_bd(False)
    dwo_t = outer_result(3)
    dwo_st[...] = _cat([a.T for a in dwo_t[:3]] + [dwo_t[3].T[KG:]])
    start([c_dwo] + tile_out(0))
    loop(phase3, 2, post=lambda i: start(tile_out(i)))

    i = NT - 1
    ch = CHUNKS[2]
    dkb, dvb = key_bwd(i)
    mlp_s1(i, 0, ch[0])
    dphi_q, dwT_q = unfold_phi(tiles_t(outer_result(0)), 0)
    dwT_q = _cat(dwT_q)
    dwqkv_st[:, 0:384] = untile([dwT_q[:384, 128 * j:128 * j + 128] for j in range(4)])
    start(out_wqkv[:1])
    mlp_s1(i, 1, ch[1])
    outer(1, xa_s, i, dkb, False)
    outer(2, xa_s, i, dvb, False)
    gv = outer_result(2)
    dwqkv_st[:, 2 * D:3 * D] = _cat(gv[:3] + [gv[3][:, KG:]], 1)
    start(out_wqkv[2:])
    dphi_k, dwT_k = unfold_phi(tiles_t(outer_result(1)), 1)
    mlp_s2b(i, 0, ch[0], 'last')
    start(out_mlp[2])
    dwT = _cat([dwT_q[384:]] + dwT_k)
    dwk = untile([dwT[:, 128 * j:128 * j + 128] for j in range(4)])
    dwqkv_st[:, 384:2 * D] = dwk
    done = [_pk(dwk[r - 16:r, 128 * j:128 * j + 128]) for j in range(4) for r in (128, 256, 384, 448)]
    mask, sel = bd_consts()
    for g in range(NG):
        dg = jnp.where(mask, dphi_q[g] + dphi_k[g], 0.0).astype(BF16)
        tmpa_s[PF * g:PF * g + PF, :] = _nt(dg, sel)
    for d in range(DH):
        dwphi_st[H * d:H * d + H, :] = tmpa_s[pl.ds(d, H, stride=DH), :].astype(BF16)
    mlp_s2b(i, 1, ch[1], 'last')
    start(out_mlp[3] + [out_wqkv[1], c_dwphi])
    m = dx_products(i, dkb, dvb, {PORD[0]: _tree(jnp.bitwise_or, done) & zero_s[...]})
    marks, store = finish_out(i)
    store(0)
    finish_dx(i, m, marks[1:6], lambda: start(tile_out(i, 0, DB)))
    store(1)
    start(tile_out(i, DB, DB))

    wait(sum(out_mlp, []) + out_wqkv + [c_dwo, c_dwphi])
    for i in range(NT - 1):
        wait(tile_out(i))
    wait(tile_out(NT - 1, 0, DB) + tile_out(NT - 1, DB, DB))


@jax.jit
def pallas_parallel_sum__linear_kernel_hedgehog__glu_gated_geglu__prompt_kernel(
    A_x: jax.Array,
    A_wqkv: jax.Array,
    A_w_phi: jax.Array,
    A_wo: jax.Array,
    B_x: jax.Array,
    B_w_gate: jax.Array,
    B_w_up: jax.Array,
    B_w_down: jax.Array,
    grad_out: jax.Array,
):
    del B_x
    xT = A_x.reshape(S, D).T
    dyT = grad_out.reshape(S, D).T
    wphi2 = A_w_phi.transpose(1, 0, 2).reshape(D, DH)
    wdT = B_w_down.T

    V = pltpu.VMEM
    dma = pltpu.SemaphoreType.DMA
    scratch = [
        V((NT, D, TS), BF16), V((NT, D, TS), BF16),
        V((NT, 32, TS), F32), V((NT, DB, TS), U32),
        V((NT, 1024, SB), U32), V((NT, 1024, SB), U32),
        V((NT, 640, SB), U32), V((NT, 640, 128), U32), V((NT, 640, 128), U32),
        V((2, 640, SB), U32),
        V((D, 3 * D), BF16), V((D, DH), BF16), V((D, D), BF16),
        V((D, DF), BF16), V((D, DF), BF16), V((D, DF), BF16),
        V((3 * DB, 512), U32), V((D, PF), BF16),
        V((4, 7, DB // 2, 256), U32), V((4, 7, DB // 2, 256), U32),
        V((7, DB // 2, DF), U32), V((7, DB // 2, DF // 2), U32),
        V((7, 128, DF), U32), V((7, 128, DF // 2), U32),
        V((D, DH), F32), V((D, DH), F32),
        V((7, SB // 2, 384), U32), V((7, SB // 2, 768), U32),
        V((NT, NP * PR, TS), U32), V((NT, NP * 32, TS), U32),
        V((2, NP, PE, PF), F32), V((2, NP, PE // 2, PF), U32), V((2, NP, PR, PE), U32),
        V((NT, 8, DB, SB), F32), V((NT, 8, DB, SB), F32),
        V((7, DB, 768), F32), V((7, DB, 384), F32),
        V((4, 13 * DB, 128), F32),
        V((DB, 512), U32), V((8, 128), U32), V((D, TS), F32),
        V((NT, D, TS), BF16), V((NT, D, TS), BF16),
        V((D, 3 * D), BF16), V((D, DH), BF16), V((D, D), BF16),
        V((D, DF), BF16), V((D, DF), BF16), V((D, DF), BF16),
        dma((NT + 8,)),
    ]
    sds = jax.ShapeDtypeStruct
    out_shape = (
        sds((D, S), BF16), sds((D, S), BF16), sds((D, 3 * D), BF16), sds((D, DH), BF16),
        sds((D, D), BF16), sds((D, DF), BF16), sds((D, DF), BF16), sds((D, DF), BF16),
    )
    any_spec = pl.BlockSpec(memory_space=pl.ANY)
    outT, dxT, dwqkv, dwphi2, dwo, dwg, dwu, dwdT = pl.pallas_call(
        _kernel,
        out_shape=out_shape,
        in_specs=[any_spec] * 8,
        out_specs=[any_spec] * 8,
        scratch_shapes=scratch,
        compiler_params=pltpu.CompilerParams(vmem_limit_bytes=120 * 1024 * 1024),
        name="hedgehog_geglu",
    )(xT, A_wqkv, wphi2, A_wo, B_w_gate, B_w_up, wdT, dyT)
    return (
        outT.T.reshape(1, S, D),
        dxT.T.reshape(1, S, D),
        dwqkv,
        dwphi2.reshape(DH, H, DH).transpose(1, 0, 2),
        dwo,
        dwg,
        dwu,
        dwdT.T,
    )
```

```python
import math

import jax
import jax.numpy as jnp
from jax import lax
import jax.experimental.pallas as pl
import jax.experimental.pallas.tpu as pltpu

S, D, H, DH, DF = 2048, 448, 16, 28, 1792
NP = H // 2
PR = 2 * DH
PF = 2 * PR
PE = PR + 8
NG = H // 4
TS = 256
NT = S // TS
SB, DB = TS // 2, D // 2
AORD = (6, 5, 0, 3, 4, 7, 8)
PORD = (1, 3, 2, 4, 0, 6, 5)
TORD = (1, 3, 0, 4, 6, 2, 5)
RORD = {'ab': (0, 7, 4, 11, 1, 8, 5, 12, 2, 9, 6, 13, 3, 10), 'a': (0, 7, 1, 8, 2, 9, 3, 10, 4, 11, 5, 12, 6, 13),
        'b': (0, 4, 1, 5, 2, 6, 3, 7, 8, 9, 10, 11, 12, 13), 'n': tuple(range(14))}
XEXT = (None, 7, 8, 9, 7, 8, 9)
FEXT = (None, 8, 9, 9, 7, 8, 7)
KS, KG = 256, 64
BORD = (0, 2, 6, 5, 3, 4, 1)
CHUNKS = (((0, 256), (256, 256)),
          ((512, 256), (768, 256), (1024, 256)),
          ((1280, 256), (1536, 256)))
QPLAN = {
    'mid': {0: [('f', (0, 1))], 1: [('f', (2,))], 2: [('f', (3,))], 3: [('f', (4,))], 4: [('f', (5,))], 5: [('f', (6,)), ('n', (0, 1, 2, 3))], 6: [('f', (7,))], 7: [('b', (0, 1))], 10: [('b', (2, 3))], 13: [('n', (4, 5, 6, 7))], 20: [('b', (4, 5))], 27: [('b', (6, 7))]},
    'first': {0: [('f', (0, 1))], 1: [('f', (2, 3))], 2: [('f', (4, 5))], 3: [('f', (6, 7)), ('n', (0, 1, 2, 3))],
              5: [('b', (0, 1))], 7: [('b', (2, 3)), ('n', (4, 5, 6, 7))], 9: [('b', (4, 5))], 12: [('b', (6, 7))]},
}
LN_EPS = 1e-5
DEN_EPS = 1e-6
C0 = math.sqrt(2.0 / math.pi)
C1 = 0.044715
F32, BF16, U32 = jnp.float32, jnp.bfloat16, jnp.uint32


def _nn(a, b):
    return lax.dot_general(a, b, (((1,), (0,)), ((), ())), preferred_element_type=F32)


def _nt(a, b):
    return lax.dot_general(a, b, (((1,), (1,)), ((), ())), preferred_element_type=F32)


def _tn(a, b):
    return lax.dot_general(a, b, (((0,), (0,)), ((), ())), preferred_element_type=F32)


def _tree(op, xs):
    xs = list(xs)
    while len(xs) > 1:
        nxt = [op(xs[i], xs[i + 1]) for i in range(0, len(xs) - 1, 2)]
        if len(xs) % 2:
            nxt.append(xs[-1])
        xs = nxt
    return xs[0]


def _rows8(a):
    return [a[8 * i:8 * i + 8] for i in range(a.shape[0] // 8)]


def _pair_reduce(op, rows):
    v = _tree(op, rows)
    v = op(v, pltpu.roll(v, 2, 0))
    return op(v, pltpu.roll(v, 4, 0))


def _softmax_pair(p):
    rows = _rows8(p)
    mx = _pair_reduce(jnp.maximum, rows)
    mn = _pair_reduce(jnp.minimum, rows)
    ep = [jnp.exp(r - mx) for r in rows]
    en = [jnp.exp(mn - r) for r in rows]
    rp = 1.0 / _pair_reduce(jnp.add, ep)
    rn = 1.0 / _pair_reduce(jnp.add, en)
    return jnp.concatenate([e * rp for e in ep] + [e * rn for e in en], axis=0)


def _softmax_pair_bwd(phi, dphi):
    pr, dr = _rows8(phi), _rows8(dphi)
    t = [a * b for a, b in zip(pr, dr)]
    sp = _pair_reduce(jnp.add, t[:7])
    sn = _pair_reduce(jnp.add, t[7:])
    out = [(t[i] - t[7 + i]) - (pr[i] * sp - pr[7 + i] * sn) for i in range(7)]
    return jnp.concatenate(out, axis=0)


def _pk(a):
    return pltpu.bitcast(a, U32)


def _up(a):
    return pltpu.bitcast(a, BF16)


def _cat(xs, axis=0):
    return jnp.concatenate(xs, axis=axis)


def _split(a):
    w = _pk(a)
    return [pltpu.unpack_elementwise(w, index=j, packed_dtype=BF16, unpacked_dtype=F32) for j in range(2)]


def _pack(e, o):
    return pltpu.pack_elementwise([e, o], packed_dtype=BF16)


def _pack16(a):
    r = _rows8(a)
    return _pack(_cat(r[0::2]), _cat(r[1::2]))


def _unpack16(w):
    e, o = [_rows8(pltpu.unpack_elementwise(w, index=j, packed_dtype=BF16, unpacked_dtype=F32)) for j in range(2)]
    return _cat([x for p in zip(e, o) for x in p])


def _bf(xs):
    return [a.astype(BF16) for a in xs]


def _combos(x11, x12, x21, x22):
    return [x11 + x22, x21 + x22, x11, x22, x11 + x12, x21 - x11, x12 - x22]


def _combos_t(x11, x12, x21, x22):
    return _combos(x11, x21, x12, x22)


def _uncombos(m):
    return (m[0] + m[3] - m[4] + m[6], m[2] + m[4], m[1] + m[3], m[0] - m[1] + m[2] + m[5])


def _uncombos_t(m):
    c11, c12, c21, c22 = _uncombos(m)
    return c11, c21, c12, c22


def _quarters(x):
    r, c = x.shape[0] // 2, x.shape[1] // 2
    return x[:r, :c], x[:r, c:], x[r:, :c], x[r:, c:]


def _join(x11, x12, x21, x22):
    return _cat([_cat([x11, x12], 1), _cat([x21, x22], 1)])


def _set_a(x):
    x11, x12, x21, x22 = _quarters(x)
    return [x11, x21, x12, x22, x11 + x12, x21 + x22, x11 + x22, x21 - x11, x12 - x22]


def _groups(x):
    n = x.shape[0] // 7
    return x[:4 * n], [x[(4 + j) * n:(5 + j) * n] for j in range(3)]


def _halves(x, axis=1):
    n = x.shape[axis] // 2
    return (x[:, :n], x[:, n:]) if axis else (x[:n], x[n:])


def _set_x(x):
    top, g = _groups(x)
    (l1, r1), (l2, r2), (l3, r3) = [_halves(a) for a in g]
    return _combos(*_quarters(top)) + [_cat([l2, r3]), _cat([r1, l2 + r2]), _cat([l1, l3 + r3])]


def _set_w(x):
    top, g = _groups(x)
    (l1, r1), (l2, r2), (l3, r3) = [_halves(a) for a in g]
    d1 = r1 - l1
    ext = [[], [r2, -r3], [l1, l2], [r1, r3], [-l2, l3], [d1, r2 - l2], [-d1, l3 - r3]]
    return [_cat([c] + e) for c, e in zip(_combos_t(*_quarters(top)), ext)]


def _set_f(x):
    top, g = _groups(x)
    (l1, r1), (l2, r2), (l3, r3) = [_halves(a) for a in g]
    return _combos_t(*_quarters(top)) + [_cat([l1, l2 - r2]), _cat([r1, r3 - l3]), _cat([r2, l3])]


def _wf_set(t):
    low = lax.broadcasted_iota(jnp.int32, (t[0].shape[0] // 2, 128), 1) < KG
    (a0, b0), (a1, b1), (a2, b2), (a3, b3) = [_halves(a, 0) for a in t]
    d2 = b2 - a2
    ext = [None, jnp.where(low, b3, -b3), a2, jnp.where(low, b2, b3), jnp.where(low, -a3, a3), d2,
           jnp.where(low, -d2, a3 - b3)]
    return [c if e is None else _cat([c, e], 1) for c, e in zip(_combos(a0, a1, b0, b1), ext)]


def _wb_set(t):
    low = lax.broadcasted_iota(jnp.int32, (t[0].shape[0] // 2, 128), 1) < KG
    (a0, b0), (a1, b1), (a2, b2), (a3, b3) = [_halves(a, 0) for a in t]
    a13, b13 = jnp.where(low, a2, a3), jnp.where(low, b2, b3)
    ext = [None, a13, b3, a3, b2, a13 + b13, a2 + b2]
    c = _combos_t(a0, a1, b0, b1)
    return [c[BORD[k]] if e is None else _cat([c[BORD[k]], e], 1) for k, e in enumerate(ext)]


def _unit(ref, idx, k, rows=DB // 2, n=1):
    return _up(ref[idx + (slice(rows * k, rows * (k + n)),)])


def _acc(ref, idx, first, val):
    ref[idx] = val if first else ref[idx] + val


TILES = ((0, 128), (128, 256), (256, 384), (320, 448))


def _kernel(xT_h, wqkv_h, wphi_h, wo_h, wg_h, wu_h, wdT_h, dyT_h,
            outT_h, dxT_h, dwqkv_h, dwphi_h, dwo_h, dwg_h, dwu_h, dwdT_h,
            xT_s, dyT_s, rstd_s, doT_s, xa_s, ya_s, xb_s, xbt_s, ybt_s, qs_s,
            wqkv_s, wphi_s, wo_s, wg_s, wu_s, wdT_s,
            wT_s, bd_s, wf_s, wb_s,
            wa_gu, wa_d, wb_gu, wb_d, tmpa_s, tmpb_s,
            hc_s, dguc_s, phik_s, vext_s, kv_acc, kvt_s, kv_s,
            out_acc, dxn_acc, dwgu_acc, dwd_acc, g_acc,
            fold_s, zero_s, dxn_s, out_st, dx_st, dwqkv_st, dwphi_st, dwo_st, dwg_st, dwu_st, dwd_st,
            sem):
    def cols(src, dst, lo, hi, k):
        return pltpu.make_async_copy(src.at[:, pl.ds(lo, hi - lo)], dst.at[:, pl.ds(lo, hi - lo)], sem.at[k])

    def x_copy(i, k):
        return pltpu.make_async_copy(xT_h.at[:, pl.ds(i * TS, TS)], xT_s.at[i], sem.at[k])

    def dy_copy(i, k):
        return pltpu.make_async_copy(dyT_h.at[:, pl.ds(i * TS, TS)], dyT_s.at[i], sem.at[k])

    def xy_in(i):
        return [dy_copy(i, i), x_copy(i, i)]

    def mlp_in(lo, hi, k, mats=slice(None)):
        return [cols(src, dst, lo, hi, k) for src, dst in ((wg_h, wg_s), (wu_h, wu_s), (wdT_h, wdT_s))[mats]]

    def mlp_out(chunks, k):
        lo, hi = chunks[0][0], chunks[-1][0] + chunks[-1][1]
        return [cols(src, dst, lo, hi, k) for src, dst in ((dwg_st, dwg_h), (dwu_st, dwu_h), (dwd_st, dwdT_h))]

    def tile_out(i, r=0, n=D):
        return [pltpu.make_async_copy(src.at[i, pl.ds(r, n)], dst.at[pl.ds(r, n), pl.ds(i * TS, TS)], sem.at[NT + 5])
                for src, dst in ((dx_st, dxT_h), (out_st, outT_h))]

    in_x = [x_copy(0, 0)]
    in_g = mlp_in(0, 256, NT, slice(0, 1))
    in_y = [dy_copy(0, NT + 7)]
    in_ud = mlp_in(0, 256, NT + 1, slice(1, 3))
    in_c1 = mlp_in(256, 512, NT + 2)
    in_kv = [pltpu.make_async_copy(wphi_h, wphi_s, sem.at[NT + 3]), cols(wqkv_h, wqkv_s, 384, 2 * D, NT + 3)]
    in_vo = [pltpu.make_async_copy(wo_h, wo_s, sem.at[NT + 6]), cols(wqkv_h, wqkv_s, 2 * D, 3 * D, NT + 6)]
    in_rest = [cols(wqkv_h, wqkv_s, 0, 384, NT + 4)] + mlp_in(512, DF, NT + 4)
    out_mlp = [mlp_out(g, NT + 5) for g in (CHUNKS[0], CHUNKS[1], CHUNKS[2][:1], CHUNKS[2][1:])]
    out_wqkv = [cols(dwqkv_st, dwqkv_h, lo, hi, NT + 5) for lo, hi in ((0, 384), (384, 2 * D), (2 * D, 3 * D))]
    c_dwphi = pltpu.make_async_copy(dwphi_st, dwphi_h, sem.at[NT + 5])
    c_dwo = pltpu.make_async_copy(dwo_st, dwo_h, sem.at[NT + 5])

    def start(cs):
        for c in cs:
            c.start()

    def wait(cs):
        for c in cs:
            c.wait()

    def tied(w, dep):
        return _up(w | _cat([dep] * (w.shape[0] // 8))).astype(F32)

    def tie(v):
        return lax.bitcast_convert_type(v[:8, :128], U32) & zero_s[...]

    def paced(marks, n, lo=0.0, hi=1.0):
        total, deps = sum(t for _, t in marks), []
        for j in range(n):
            pos = (lo + (hi - lo) * j / n) * total
            for v, t in marks:
                if pos < t:
                    break
                pos -= t
            deps.append(tie(v[8 * min(int(pos / t * (v.shape[0] // 8)), v.shape[0] // 8 - 1):]))
        return deps

    def unpack_paced(w, deps, order):
        if deps is not None:
            per = len(order) // len(deps)
            w = w | _cat([_cat([deps[order.index(j) // per]] * (w.shape[1] // 128), 1)
                          for j in range(len(order)) for _ in range(2)])
        return [pltpu.unpack_elementwise(w, index=j, packed_dtype=BF16, unpacked_dtype=F32) for j in range(2)]

    def held(a, dep):
        top = lax.bitcast_convert_type(a[:8], U32) | _cat([dep] * (a.shape[1] // 128), 1)
        top = lax.bitcast_convert_type(top, F32)
        return _cat([top, a[8:]]) if a.shape[0] > 8 else top

    def bd_consts(perm=False):
        def col(shape):
            c = lax.broadcasted_iota(jnp.int32, shape, 1)
            return (c & -16) + 2 * (c & 7) + ((c >> 3) & 1) if perm else c

        r = lax.broadcasted_iota(jnp.int32, (PF, PF), 0)
        c = col((PF, PF))
        row_head = ((r >= DH).astype(jnp.int32) + (r >= 2 * DH).astype(jnp.int32)
                    + (r >= 3 * DH).astype(jnp.int32))
        mask = row_head == 2 * (c >= PR).astype(jnp.int32) + (c & 1)
        sc = col((DH, PF))
        sr = lax.broadcasted_iota(jnp.int32, (DH, PF), 0)
        sel = jnp.where(((sc - PR * (sc >= PR).astype(jnp.int32)) >> 1) == sr, 1.0, 0.0).astype(BF16)
        return mask, sel

    def kv_operands(s):
        def source(p):
            return (p & -16) + ((p & 15) >> 1) + 8 * (p & 1)

        def restore(a):
            return _unpack16(_pk(a.astype(BF16))).astype(BF16)

        r = lax.broadcasted_iota(jnp.int32, (PE, PF), 0)
        c = source(lax.broadcasted_iota(jnp.int32, (PE, PF), 1))
        r = r if s else source(r)
        row_head = jnp.where(r < PR, (r >= DH).astype(jnp.int32), (r >= PR + 4).astype(jnp.int32))
        mask = row_head == (c & 1)
        for p in range(NP):
            m = jnp.where(mask, kv_acc[s, p], 0.0)
            rows, cols = (m.astype(BF16), _up(_pack16(m))) if s else (restore(m), restore(m))
            kvt_s[s, p] = _pk(rows)
            kv_s[s, p] = _pk(restore(cols.astype(F32).T))

    def untile(t):
        return _cat([t[0].T, t[1].T, t[2].T, t[3].T[KG:]])

    def prep_phi():
        tmpa_s[...] = wphi_s[...].astype(F32)
        for d in range(DH):
            tmpb_s[pl.ds(d, H, stride=DH), :] = tmpa_s[H * d:H * d + H, :]

    def prep_bd(perm):
        mask, sel = bd_consts(perm)
        expand = _nn(tmpb_s[...].astype(BF16), sel)
        for g in range(NG):
            bd_s[PF * g:PF * g + PF, :] = jnp.where(mask, expand[PF * g:PF * g + PF], 0.0).astype(BF16)

    def prep_wt(lo, hi):
        for j, (a, b) in enumerate(TILES):
            wT_s[lo // 2:hi // 2, 128 * j:128 * j + 128] = _pk(wqkv_s[a:b, lo:hi].T)

    def fold(t):
        w = _rows8(_cat([_tn(bd_s[PF * g:PF * g + PF, :], _unit(wT_s, (), NG * t + g, PR)) for g in range(NG)]))
        return [[v[:, 128 * j:128 * j + 128] for j in range(4)] for v in (_cat(w[0::2]), _cat(w[1::2]))]

    def store_set(ref, t, make, e, o):
        done = []
        for k, (p, q) in enumerate(zip(make(e), make(o))):
            w = _pack(p, q)
            ref[t, k, :, :p.shape[1]] = w
            done.extend(w[r:r + 8, -128:] for r in (0, 56, 104))
        return _tree(jnp.bitwise_or, done) & zero_s[...]

    def split_tiles(tiles, deps=None):
        return zip(*[unpack_paced(_pk(a), deps, RORD['a']) for a in tiles])

    def wunit(ref, t, k):
        return _up(ref[t, k, :, :256 if k else 128])

    def prep_qk(t):
        e, o = fold(t)
        store_set(wf_s, t, _wf_set, e, o)
        return [_up(_pack(p, q)) for p, q in zip(e, o)]

    def prep_qk_t(t, w, deps=None):
        return store_set(wb_s, t, _wb_set, *split_tiles([untile([c[a:b] for c in w]) for a, b in TILES], deps))

    def prep_v(deps=None):
        w = _unit(wT_s, (), 2, DB)
        store_set(wf_s, 2, _wf_set, *split_tiles([w[:, 128 * j:128 * j + 128] for j in range(4)], deps))

    def prep_v_t(deps=None):
        store_set(wb_s, 2, _wb_set, *split_tiles([wqkv_s[:, 2 * D + a:2 * D + b] for a, b in TILES], deps))

    def prep_wo(deps=None):
        store_set(wf_s, 3, _wf_set, *split_tiles([wo_s[:, a:b] for a, b in TILES], deps))

    def prep_wo_t(deps=None):
        return store_set(wb_s, 3, _wb_set, *split_tiles([wo_s[a:b, :].T for a, b in TILES], deps))

    def prep_mlp(chunks, mats, part, marks=None, lo=0.0, hi=1.0):
        items = [(ch, m) for ch in chunks for m in mats]
        deps = None if marks is None else paced(marks, 7 * len(items), lo, hi)
        for n, ((a, w), m) in enumerate(items):
            f = w // 2
            ref, off, wa, wb = {'g': (wg_s, a, wa_gu, wb_gu), 'u': (wu_s, a + f, wa_gu, wb_gu),
                                'd': (wdT_s, a // 2, wa_d, wb_d)}[m]
            e, o = unpack_paced(_pk(ref[:, a:a + w]), deps and deps[7 * n:7 * n + 7], RORD[part])
            if 'b' in part:
                for k, (p, q) in enumerate(zip(_set_w(e), _set_w(o))):
                    wb[k, :p.shape[0], off:off + f] = _pack(p, q)
            if 'a' in part:
                for k, (p, q) in enumerate(zip(_combos_t(*_quarters(e)), _combos_t(*_quarters(o)))):
                    wa[k, :, off:off + f] = _pack(p, q)

    def unfold_phi(gT, t):
        dphi, dwT = [], []
        low = lax.broadcasted_iota(jnp.int32, (PF, 512), 1)
        dup = (low >= 3 * 128) & (low < 3 * 128 + KG)
        for g in range(NG):
            r = slice(PF * g, PF * g + PF)
            dphi.append(_nt(jnp.where(dup, 0, _unit(wT_s, (), NG * t + g, PR)), gT[r]))
            dwT.append(_nn(bd_s[r, :], gT[r]).astype(BF16))
        return dphi, dwT

    def ragged(get, k, ext, axis):
        return get(k) if ext is None else _cat([get(k), get(ext)], axis)

    def project(w, xs, marks):
        m = {k: _nn(wunit(wf_s, w, k), ragged(xs, BORD[k], XEXT[k], 0)) for k in PORD}
        marks.extend((m[k], 2 if k else 1) for k in PORD)
        return _join(*_uncombos(m))

    def back_project(w, fs, k):
        return _nn(wunit(wb_s, w, k), ragged(lambda j: fs[j], k, FEXT[k], 0))

    def outer(w, a_s, i, fs, first):
        marks = []
        for k in range(7):
            marks.append((_nt(_unit(a_s, (i,), AORD[k]), fs[BORD[k]]), 1))
            _acc(g_acc, (w, slice(DB * k, DB * k + DB)), first, marks[-1][0])
        for k in range(3):
            marks.append((_nt(_unit(a_s, (i,), 2 * k, n=2), fs[7 + k]), 2))
            _acc(g_acc, (w, slice(DB * (7 + 2 * k), DB * (9 + 2 * k))), first, marks[-1][0])
        return marks

    def outer_result(w):
        c11, c12, c21, c22 = _uncombos([g_acc[w, DB * k:DB * k + DB] for k in range(7)])
        p = [g_acc[w, DB * (7 + 2 * k):DB * (9 + 2 * k)] for k in range(3)]
        low = lax.broadcasted_iota(jnp.int32, (D, 128), 1) < KG
        t = [_cat([c11, c21]), _cat([c12, c22]),
             p[0] + jnp.where(low, p[1], pltpu.roll(p[2], KG, 1)), p[1] + p[2]]
        return [a.astype(BF16) for a in t]

    def mlp_pre(bt_s, i, wb, a, w, k, h=None):
        lhs = ragged(lambda j: _unit(bt_s, (i,), j, 64) if h is None else _unit(bt_s, (i,), 2 * j + h, 32),
                     BORD[k], XEXT[k], 1)
        return _nn(lhs, _up(wb[k, :128 if k else 64, a:a + w]))

    def mlp_gu(i, ch, k, h):
        return mlp_pre(xbt_s, i, wb_gu, ch[0], ch[1], k, h)

    def mlp_dh(i, ch, k, h):
        return mlp_pre(ybt_s, i, wb_d, ch[0] // 2, ch[1] // 2, k, h)

    def mlp_s1(i, n, ch, gum=None, split=True):
        for h in range(2) if gum is None and split else (None,):
            mlp_half(i, n, ch, h, gum)

    def mlp_half(i, n, ch, half, gum=None, dhm=None):
        gum, dhm = dict(gum or {}), dict(dhm or {})
        for k in PORD:
            if k not in dhm:
                dhm[k] = mlp_dh(i, ch, k, half)
            if k not in gum:
                gum[k] = mlp_gu(i, ch, k, half)
        f = ch[1] // 2
        hs, dgus = [], []
        for gu, dh in zip(_uncombos_t(gum), _uncombos_t(dhm)):
            g, u = gu[:, :f], gu[:, f:]
            g2 = g * g
            s = 0.5 * jnp.tanh(g * (C0 + (C0 * C1) * g2)) + 0.5
            gelu = g * s
            dgelu = s + gelu * (1.0 - s) * (2.0 * C0 + (6.0 * C0 * C1) * g2)
            hs.append(gelu * u)
            dgus.append(_cat([dh * u * dgelu, dh * gelu], 1))
        for k, (h, dgu) in enumerate(zip(_combos(*hs), _combos(*dgus))):
            r = slice(None) if half is None else slice(32 * half, 32 * half + 32)
            hc_s[k, r, f * n:f * n + f] = pack_tokens(h)
            dguc_s[k, r, 2 * f * n:2 * f * n + 2 * f] = pack_tokens(dgu)

    def pack_tokens(a):
        r = _rows8(a)
        return _pack(_cat([x for j, x in enumerate(r) if not j & 2]), _cat([x for j, x in enumerate(r) if j & 2]))

    def mlp_out_p(chunks, k):
        a, w = chunks[0][0], sum(c[1] for c in chunks)
        return _nt(_up(wa_d[BORD[k], :, a // 2:(a + w) // 2]), _up(hc_s[k, :, :w // 2]))

    def mlp_dx_p(chunks, k):
        a, w = chunks[0][0], sum(c[1] for c in chunks)
        return _nt(_up(wa_gu[BORD[k], :, a:a + w]), _up(dguc_s[k, :, :w]))

    def mlp_s2b(i, n, ch, mode, hooks={}, holds={}):
        a, w = ch
        marks = []
        f = w // 2
        for a_s, src, acc, wd, dsts in ((ya_s, hc_s, dwd_acc, f, (dwd_st,)),
                                        (xa_s, dguc_s, dwgu_acc, w, (dwg_st, dwu_st))):
            m = []
            for k in range(7):
                v = _nn(_unit(a_s, (i,), AORD[k]), _up(src[BORD[k], :, wd * n:wd * n + wd]))
                idx = (k, slice(None), slice(wd * n, wd * n + wd))
                marks.append((v, wd // 128))
                if len(marks) in hooks:
                    hooks[len(marks)](marks)
                if len(marks) in holds:
                    v = held(v, holds[len(marks)])
                if mode == 'last':
                    m.append(acc[idx] + v)
                else:
                    _acc(acc, idx, mode == 'first', v)
            if mode == 'last':
                q = _uncombos(m)
                for j, dst in enumerate(dsts):
                    dst[:, a:a + w] = _join(*[v[:, f * j:f * j + f] for v in q]).astype(BF16)
        return marks

    def store_sets(i, e, o, a_s, bt_s):
        b = [_pack(p, q) for p, q in zip(_set_x(e), _set_x(o))]
        for k, w in enumerate(b):
            p, q = [_rows8(_pk(v.astype(BF16))) for v in _split(_up(w).T)]
            bt_s[i, 64 * k:64 * k + 64] = _cat([x for pair in zip(p, q) for x in pair])
        a_s[i, :9 * DB // 2] = _cat([_pack(p, q) for p, q in zip(_set_a(e), _set_a(o))])
        return b

    def dy_sets(i, deps=None):
        return [_up(w) for w in store_sets(i, *unpack_paced(_pk(dyT_s[i]), deps, RORD['ab']), ya_s, ybt_s)]

    def all_rows(v):
        v = _tree(jnp.add, _rows8(v))
        return _pair_reduce(jnp.add, [v + pltpu.roll(v, 1, 0)])

    def layernorm(i, deps=(None, None, None)):
        w = _pk(xT_s[i])
        e, o = unpack_paced(w, deps[0], RORD['n'])
        mean = _cat([all_rows(e + o) * (1.0 / D)] * (DB // 8))
        e, o = [v - mean for v in unpack_paced(w, deps[1], RORD['n'])]
        rstd = lax.rsqrt(all_rows(e * e + o * o) * (1.0 / D) + LN_EPS)
        rstd_s[i, 0:8] = rstd
        rstd = _cat([rstd] * (DB // 8))
        e, o = [(v - mean) * rstd for v in unpack_paced(w, deps[2], RORD['ab'])]
        xb_s[i] = _cat(store_sets(i, e, o, xa_s, xbt_s))

    def xproj(i, t, marks=None):
        return project(t, lambda k: _unit(xb_s, (i,), k, 64), [] if marks is None else marks)

    def do_proj(i, yb, marks=None):
        doT_s[i] = _pack16(project(3, lambda k: yb[k], [] if marks is None else marks))

    def key_side(i, pk, v, first, deps=None):
        ones = jnp.ones((8, TS), F32)
        for c in range(NP):
            p = pk[PR * c:PR * c + PR]
            phik = _pack16(_softmax_pair(p if deps is None else held(p, deps[c])))
            phik_s[i, PR * c:PR * c + PR, :] = phik
            vext = _pack16(_cat([v[PR * c:PR * c + PR], ones]))
            vext_s[i, 32 * c:32 * c + 32, :] = vext
            _acc(kv_acc, (0, c), first, _nt(_up(vext), _up(phik)))

    def phase1_tail(i):
        mo = [mlp_out_p(CHUNKS[0], k) for k in range(7)]
        mdx = [mlp_dx_p(CHUNKS[0], k) for k in range(7)]
        for k, (o, dx) in enumerate(zip(mo, mdx)):
            out_acc[i, k] = o
            dxn_acc[i, k] = dx
        return [(o, 1) for o in mo] + [(dx, 2) for dx in mdx]

    c0, c1 = CHUNKS[0]
    start(in_x + in_g + in_y + in_ud + in_c1 + in_kv + in_vo)
    for i in range(1, NT):
        start(xy_in(i))
    start(in_rest)
    wait(in_x)
    zero_s[...] = (_pk(xT_s[0, 0:16, 0:128]) >> 16) >> 16
    layernorm(0)
    wait(in_g)
    prep_mlp([c0], 'g', 'ab')
    wait(in_y)
    g = {k: mlp_pre(xbt_s, 0, wb_gu, 0, 128, k) for k in PORD}
    yb = dy_sets(0)
    wait(in_ud)
    prep_mlp([c0], 'ud', 'b')
    gu = {k: _cat([g[k], mlp_pre(xbt_s, 0, wb_gu, 128, 128, k)], 1) for k in PORD}
    mlp_s1(0, 0, c0, gu)

    def next_chunk(marks):
        prep_mlp([c0], 'ud', 'a', marks, 0.0, 0.9)
        wait(in_c1)

    marks = mlp_s2b(0, 0, c0, 'first', {10: next_chunk})
    prep_mlp([c1], 'dgu', 'b', marks[10:])
    mlp_s1(0, 1, c1)
    folded = []

    def attn_prep(marks):
        prep_mlp([c1], 'd', 'a', marks, 0.0, 0.8)
        wait(in_kv)
        prep_phi()
        prep_wt(384, 2 * D)

    marks = mlp_s2b(0, 1, c1, 'first', {7: attn_prep, 10: lambda m: prep_bd(True),
                                        12: lambda m: folded.extend(prep_qk(1))})
    prep_mlp([c1], 'gu', 'a', marks[7:])
    wait(in_vo)
    marks = []
    pk = xproj(0, 1, marks)
    prep_wt(2 * D, 3 * D)
    prep_wo(paced(marks, 7, 0.0, 0.5))
    prep_v(paced(marks, 7, 0.5))
    marks = []
    do_proj(0, yb, marks)
    v = xproj(0, 2, marks)
    key_side(0, pk, v, True, paced(marks, NP, 0.0, 0.8))
    fold_s[...] = _pk(_cat(folded, 1))

    def phase1(i, mode):
        marks = phase1_tail(i - 1)
        yb = dy_sets(i, paced(marks, 14, 0.0, 0.3))
        layernorm(i, (paced(marks, 7, 0.3, 0.42), paced(marks, 7, 0.44, 0.58), paced(marks, 14, 0.6, 1.0)))
        if mode == 'last':
            prep_mlp(CHUNKS[1], 'd', 'a', marks)
        do_proj(i, yb)
        mlp_s1(i, 0, c0)
        pk = xproj(i, 1)
        mlp_s1(i, 1, c1, split=mode != 'mid')
        marks = []
        v = xproj(i, 2, marks)
        if mode == 'last':
            prep_mlp(CHUNKS[1][:1], 'gu', 'a', marks, 0.4)
            prep_wt(0, 384)
            folded[:] = prep_qk(0)
        marks = mlp_s2b(i, 0, c0, mode)
        key_side(i, pk, v, False, paced(marks, NP, 0.0, 0.8) if mode == 'mid' else None)
        mlp_s2b(i, 1, c1, mode)

    def loop(f, unroll, pre=None, post=None):
        def body(j, carry):
            tiles = [1 + unroll * j + n for n in range(unroll)]
            for g in (pre, lambda i: f(i, 'mid'), post):
                for i in tiles if g else ():
                    g(i)
            return carry
        lax.fori_loop(0, (NT - 2) // unroll, body, 0)

    loop(phase1, 1, pre=lambda i: wait(xy_in(i)))
    wait(in_rest + xy_in(NT - 1))
    phase1(NT - 1, 'last')
    kv_operands(0)
    prep_mlp(CHUNKS[1], 'dgu', 'b', phase1_tail(NT - 1))

    class Query:
        def __init__(self, i, first=False, marks=None):
            self.i, self.first = i, first
            self.pq = xproj(i, 0, marks)
            self.phi, self.ne, self.o, self.dp = {}, {}, {}, {}

        def fwd(self, cs, deps):
            for c, dep in zip(cs, deps):
                self.phi[c] = _up(_pack16(_softmax_pair(held(self.pq[PR * c:PR * c + PR], dep))))

        def num(self, cs):
            for c in cs:
                self.ne[c] = _rows8(_nn(_up(kvt_s[0, c]), self.phi[c]))

        def bwd(self, cs):
            lo4 = lax.broadcasted_iota(jnp.int32, (8, TS), 0) < 4
            dne = {}
            for c in cs:
                ne, r0 = self.ne[c], PR * c // 16 * 8
                do = _unpack16(doT_s[self.i, r0:r0 + 32])[PR * c % 16:PR * c % 16 + PR]
                r = 1.0 / (ne[7] + DEN_EPS)
                rr = pltpu.roll(r, 4, 0)
                ra = jnp.where(lo4, r, rr)
                rb = jnp.where(lo4, rr, r)
                rs = [ra, ra, ra, r, rb, rb, rb]
                o = [n * w for n, w in zip(ne[:7], rs)]
                dnum = [n * w for n, w in zip(_rows8(do), rs)]
                t = [a * b for a, b in zip(dnum, o)]
                sa = t[0] + t[1] + t[2]
                sb = t[4] + t[5] + t[6]
                e = jnp.where(lo4, sa, sb) + pltpu.roll(jnp.where(lo4, sb, sa), 4, 0) + t[3]
                dne[c] = _cat(dnum + [-e]).astype(BF16)
                self.o[c] = _cat(o)
            for c in cs:
                self.dp[c] = _softmax_pair_bwd(_unpack16(_pk(self.phi[c])), _nn(_up(kv_s[0, c]), dne[c]))
            for c in cs:
                _acc(kv_acc, (1, c), self.first, _nt(dne[c], self.phi[c]))

        def sets(self):
            return [_bf(_set_f(_cat([v[c] for c in range(NP)]))) for v in (self.o, self.dp)]

        def store(self):
            done = []
            for j, st in enumerate(self.sets()):
                qs_s[j] = _pk(_cat(st))
                done.extend(_tree(jnp.bitwise_or, _rows8(_pk(a))) for a in st)
            return done

        def after(self, done, n):
            return [_tree(jnp.bitwise_or, done[j::n]) & zero_s[...] for j in range(n)]

    def phase2(i, mode):
        first = mode == 'first'
        ch = CHUNKS[1]

        def s1(n):
            mlp_s1(i, n, ch[n])

        s1(0)
        if first:
            q = Query(i, True)
            marks = mlp_s2b(i, 0, ch[0], mode)
            for c, dep in enumerate(paced(marks, NP, 0.0, 0.8)):
                q.fwd([c], [dep])
                q.num([c])
            s1(1)
            for c in range(0, NP, 2):
                q.bwd((c, c + 1))
            marks = mlp_s2b(i, 1, ch[1], mode, holds={14: prep_qk_t(0, folded)})
            deps = paced(marks, 14, 0.45, 0.95)
            for c in range(NP):
                q.o[c] = _cat([held(o, deps[RORD['b'].index((7 * c + j) // 4)]) for j, o in enumerate(_rows8(q.o[c]))])
            s1(2)
            ob, dpb = q.sets()
            marks = outer(3, ya_s, i, ob, first)
            marks += outer(0, xa_s, i, dpb, first)
        else:
            ob, dpb = [[_unit(qs_s, (j,), k, 64) for k in range(10)] for j in range(2)]
            s1(1)
            s1(2)
        if mode == 'last':
            mlp_s2b(i, 0, ch[0], mode)
            kv_operands(1)
            prep_bd(False)
            plan = {}
        else:
            q = Query(i + 1, marks=marks if first else None)
            plan = QPLAN[mode]
            if first:
                prep_mlp(ch[1:], 'gu', 'a', marks, 0.25, 0.9)
        marks, holds = [], {}

        def step(n):
            for op, cs in plan.get(n, ()):
                if op == 'f':
                    q.fwd(cs, paced(marks[-1:], len(cs)))
                else:
                    (q.num if op == 'n' else q.bwd)(cs)

        for k in range(7):
            acc = held(dxn_acc[i, k], prep_wo_t()) if first and k == 5 else dxn_acc[i, k]
            marks.append((acc + mlp_dx_p(ch, k) + back_project(0, dpb, k), 8))
            dxn_acc[i, k] = marks[-1][0]
            step(k)
        for k in range(7):
            marks.append((out_acc[i, k] + mlp_out_p(ch, k) + back_project(3, ob, k), 5))
            out_acc[i, k] = marks[-1][0]
            step(7 + k)
        if not first:
            outer(3, ya_s, i, ob, first)
            outer(0, xa_s, i, dpb, first)
        if mode == 'last':
            prep_mlp(CHUNKS[2], 'dgu', 'ab', marks, 0.0, 0.78)
            prep_v_t(paced(marks, 7, 0.78, 0.89))
            prep_qk_t(1, [_up(fold_s[:, 128 * j:128 * j + 128]) for j in range(4)], paced(marks, 7, 0.89))
        for n in range({'first': 2, 'mid': 0, 'last': 1}[mode], 3):
            if n == 2 and mode != 'last':
                at = range(10, 15) if first else range(4, 14)
                holds = dict(zip(at, q.after(q.store(), len(at))))
            mlp_s2b(i, n, ch[n], mode, {j: lambda m, j=j: step(14 * n + 13 + j) for j in range(1, 15)}, holds)

    phase2(0, 'first')
    start(out_mlp[0])
    loop(phase2, 1)
    phase2(NT - 1, 'last')

    def key_bwd(i):
        dv_all, dp_all = [], []
        for c in range(NP):
            phik = _up(phik_s[i, PR * c:PR * c + PR, :])
            dphik = _nn(_up(kv_s[1, c]), _up(vext_s[i, 32 * c:32 * c + 32, :]))
            dv_all.append(_nn(_up(kvt_s[1, c]), phik)[0:PR])
            dp_all.append(_softmax_pair_bwd(_unpack16(_pk(phik)), dphik))
        return _bf(_set_f(_cat(dp_all))), _bf(_set_f(_cat(dv_all)))

    def dx_products(i, dkb, dvb, deps={}, hooks={}):
        m = {}
        for k in PORD:
            acc = held(dxn_acc[i, k], deps[k]) if k in deps else dxn_acc[i, k]
            m[k] = acc + back_project(2, dvb, k) + back_project(1, dkb, k) + mlp_dx_p(CHUNKS[2], k)
            if k in hooks:
                hooks[k]()
        return m

    def rows_of(a_s, i, r, n, dep):
        return _cat([tied(a_s[i, DB * h + r // 2:DB * h + (r + n) // 2], dep) for h in range(2)], 1)

    def finish_dx(i, m, marks, upper_done=None):
        q = _uncombos_t(m)
        s1, s2 = [None, None], [None, None]
        for j in (1, 2, 0, 3):
            h = j & 1
            for r in range(0, DB, 32):
                d = q[j][r:r + 32]
                dxn_s[DB * (j >> 1) + r:DB * (j >> 1) + r + 32, SB * h:SB * h + SB] = d
                t1 = _tree(jnp.add, _rows8(d))
                w = DB * h + (DB * (j >> 1) + r) // 2
                t2 = _tree(jnp.add, _rows8(d * tied(xa_s[i, w:w + 16], tie(t1 if s2[h] is None else s2[h]))))
                s1[h], s2[h] = (t1, t2) if s1[h] is None else (s1[h] + t1, s2[h] + t2)
        m1, m2 = [_cat([all_rows(v) * (1.0 / D)] * 2) for v in (_cat(s1, 1), _cat(s2, 1))]
        rstd = _cat([rstd_s[i, 0:8]] * 2)
        for r, dep in zip(range(0, D, 16), paced(marks, D // 16)):
            t = dxn_s[r:r + 16] - (rows_of(xa_s, i, r, 16, dep) * m2 + m1)
            t = rows_of(ya_s, i, r, 16, dep) + rstd * t
            dx_st[i, r:r + 16] = t.astype(BF16)
            if upper_done and r + 16 == DB:
                upper_done()

    def finish_out(i):
        m = {k: out_acc[i, k] + mlp_out_p(CHUNKS[2], k) for k in TORD}
        q = _uncombos_t(m)

        def store(h):
            r = slice(DB * h, DB * h + DB)
            out_st[i, r] = (xT_s[i, r].astype(F32) + _cat(q[2 * h:2 * h + 2], 1)).astype(BF16)

        return [(m[k], 1) for k in TORD], store

    def phase3(i, mode, extra=None):
        first = mode == 'first'
        ch = CHUNKS[2]
        if first:
            mlp_s1(i, 0, ch[0])
            dkb, dvb = key_bwd(i)
        else:
            dkb, dvb = key_bwd(i)
            mlp_s1(i, 0, ch[0])
        mlp_s1(i, 1, ch[1])
        outer(2, xa_s, i, dvb, first)
        outer(1, xa_s, i, dkb, first)
        m = dx_products(i, dkb, dvb)
        store = finish_out(i)[1]
        store(0)
        store(1)
        if extra:
            extra()
        marks = mlp_s2b(i, 0, ch[0], mode)
        mlp_s2b(i, 1, ch[1], mode)
        finish_dx(i, m, marks)

    def tiles_t(t):
        return _cat([untile([a[lo:hi] for a in t]) for lo, hi in TILES], 1)

    query_grads = []

    def unfold_query():
        dphi, dwT = unfold_phi(tiles_t(outer_result(0)), 0)
        dwT = _cat(dwT)
        dwqkv_st[:, 0:384] = untile([dwT[:384, 128 * j:128 * j + 128] for j in range(4)])
        query_grads.extend((dphi, dwT[384:]))

    phase3(0, 'first', unfold_query)
    dphi_q, dwT_q = query_grads
    dwo_t = outer_result(3)
    dwo_st[...] = _cat([a.T for a in dwo_t[:3]] + [dwo_t[3].T[KG:]])
    start(out_mlp[1] + [c_dwo] + tile_out(0) + out_wqkv[:1])
    loop(phase3, 2, post=lambda i: start(tile_out(i)))

    i = NT - 1
    ch = CHUNKS[2]
    dkb, dvb = key_bwd(i)
    mlp_s1(i, 0, ch[0])
    mlp_s1(i, 1, ch[1])
    outer(1, xa_s, i, dkb, False)
    outer(2, xa_s, i, dvb, False)
    gv = outer_result(2)
    dwqkv_st[:, 2 * D:3 * D] = _cat(gv[:3] + [gv[3][:, KG:]], 1)
    start(out_wqkv[2:])
    dphi_k, dwT_k = unfold_phi(tiles_t(outer_result(1)), 1)
    mask, sel = bd_consts()
    dg = [jnp.where(mask, dphi_q[g] + dphi_k[g], 0.0).astype(BF16) for g in range(NG)]
    ready = _tree(jnp.bitwise_or, [w for a in dg for w in _rows8(_pk(a))])
    mlp_s2b(i, 0, ch[0], 'last', holds={10: _cat([ready, zero_s[:, :128 - PF]], 1) & zero_s[...]})
    start(out_mlp[2])
    dwT = _cat([dwT_q] + dwT_k)
    dwk = untile([dwT[:, 128 * j:128 * j + 128] for j in range(4)])
    dwqkv_st[:, 384:2 * D] = dwk
    done = [_pk(dwk[r - 16:r, 128 * j:128 * j + 128]) for j in range(4) for r in (128, 256, 384, 448)]
    for g in range(NG):
        tmpa_s[PF * g:PF * g + PF, :] = _nt(dg[g], sel)
    for d in range(DH):
        dwphi_st[H * d:H * d + H, :] = tmpa_s[pl.ds(d, H, stride=DH), :].astype(BF16)
    mlp_s2b(i, 1, ch[1], 'last', holds={12: _tree(jnp.bitwise_or, done) & zero_s[...]})
    start([out_wqkv[1]] + out_mlp[3] + [c_dwphi])
    m = dx_products(i, dkb, dvb)
    marks, store = finish_out(i)
    store(0)
    finish_dx(i, m, marks[1:6], lambda: start(tile_out(i, 0, DB)))
    store(1)
    start(tile_out(i, DB, DB))

    wait(sum(out_mlp, []) + out_wqkv + [c_dwo, c_dwphi])
    for i in range(NT - 1):
        wait(tile_out(i))
    wait(tile_out(NT - 1, 0, DB) + tile_out(NT - 1, DB, DB))


@jax.jit
def pallas_parallel_sum__linear_kernel_hedgehog__glu_gated_geglu__prompt_kernel(
    A_x: jax.Array,
    A_wqkv: jax.Array,
    A_w_phi: jax.Array,
    A_wo: jax.Array,
    B_x: jax.Array,
    B_w_gate: jax.Array,
    B_w_up: jax.Array,
    B_w_down: jax.Array,
    grad_out: jax.Array,
):
    del B_x
    xT = A_x.reshape(S, D).T
    dyT = grad_out.reshape(S, D).T
    wphi2 = A_w_phi.transpose(1, 0, 2).reshape(D, DH)
    wdT = B_w_down.T

    V = pltpu.VMEM
    dma = pltpu.SemaphoreType.DMA
    scratch = [
        V((NT, D, TS), BF16), V((NT, D, TS), BF16),
        V((NT, 32, TS), F32), V((NT, DB, TS), U32),
        V((NT, 1024, SB), U32), V((NT, 1024, SB), U32),
        V((NT, 640, SB), U32), V((NT, 640, 128), U32), V((NT, 640, 128), U32),
        V((2, 640, SB), U32),
        V((D, 3 * D), BF16), V((D, DH), BF16), V((D, D), BF16),
        V((D, DF), BF16), V((D, DF), BF16), V((D, DF), BF16),
        V((3 * DB, 512), U32), V((D, PF), BF16),
        V((4, 7, DB // 2, 256), U32), V((4, 7, DB // 2, 256), U32),
        V((7, DB // 2, DF), U32), V((7, DB // 2, DF // 2), U32),
        V((7, 128, DF), U32), V((7, 128, DF // 2), U32),
        V((D, DH), F32), V((D, DH), F32),
        V((7, SB // 2, 384), U32), V((7, SB // 2, 768), U32),
        V((NT, NP * PR, TS), U32), V((NT, NP * 32, TS), U32),
        V((2, NP, PE, PF), F32), V((2, NP, PE // 2, PF), U32), V((2, NP, PR, PE), U32),
        V((NT, 8, DB, SB), F32), V((NT, 8, DB, SB), F32),
        V((7, DB, 768), F32), V((7, DB, 384), F32),
        V((4, 13 * DB, 128), F32),
        V((DB, 512), U32), V((8, 128), U32), V((D, TS), F32),
        V((NT, D, TS), BF16), V((NT, D, TS), BF16),
        V((D, 3 * D), BF16), V((D, DH), BF16), V((D, D), BF16),
        V((D, DF), BF16), V((D, DF), BF16), V((D, DF), BF16),
        dma((NT + 8,)),
    ]
    sds = jax.ShapeDtypeStruct
    out_shape = (
        sds((D, S), BF16), sds((D, S), BF16), sds((D, 3 * D), BF16), sds((D, DH), BF16),
        sds((D, D), BF16), sds((D, DF), BF16), sds((D, DF), BF16), sds((D, DF), BF16),
    )
    any_spec = pl.BlockSpec(memory_space=pl.ANY)
    outT, dxT, dwqkv, dwphi2, dwo, dwg, dwu, dwdT = pl.pallas_call(
        _kernel,
        out_shape=out_shape,
        in_specs=[any_spec] * 8,
        out_specs=[any_spec] * 8,
        scratch_shapes=scratch,
        compiler_params=pltpu.CompilerParams(vmem_limit_bytes=120 * 1024 * 1024),
        name="hedgehog_geglu",
    )(xT, A_wqkv, wphi2, A_wo, B_w_gate, B_w_up, wdT, dyT)
    return (
        outT.T.reshape(1, S, D),
        dxT.T.reshape(1, S, D),
        dwqkv,
        dwphi2.reshape(DH, H, DH).transpose(1, 0, 2),
        dwo,
        dwg,
        dwu,
        dwdT.T,
    )
```

```python
import math

import jax
import jax.numpy as jnp
from jax import lax
import jax.experimental.pallas as pl
import jax.experimental.pallas.tpu as pltpu

S, D, H, DH, DF = 2048, 448, 16, 28, 1792
NP = H // 2
PR = 2 * DH
PF = 2 * PR
PE = PR + 8
NG = H // 4
TS = 256
NT = S // TS
SB, DB = TS // 2, D // 2
AORD = (6, 5, 0, 3, 4, 7, 8)
PORD = (1, 3, 2, 4, 0, 6, 5)
TORD = (1, 3, 0, 4, 6, 2, 5)
RORD = {'ab': (0, 7, 4, 11, 1, 8, 5, 12, 2, 9, 6, 13, 3, 10), 'a': (0, 7, 1, 8, 2, 9, 3, 10, 4, 11, 5, 12, 6, 13),
        'b': (0, 4, 1, 5, 2, 6, 3, 7, 8, 9, 10, 11, 12, 13), 'n': tuple(range(14))}
XEXT = (None, 7, 8, 9, 7, 8, 9)
FEXT = (None, 8, 9, 9, 7, 8, 7)
KS, KG = 256, 64
BORD = (0, 2, 6, 5, 3, 4, 1)
CHUNKS = (((0, 256), (256, 256)),
          ((512, 256), (768, 256), (1024, 256)),
          ((1280, 256), (1536, 256)))
QPLAN = {
    'mid': {0: [('f', (0, 1))], 1: [('f', (2,))], 2: [('f', (3,))], 3: [('f', (4,))], 4: [('f', (5,))], 5: [('f', (6,)), ('n', (0, 1, 2, 3))], 6: [('f', (7,))], 7: [('b', (0, 1))], 10: [('b', (2, 3))], 13: [('n', (4, 5, 6, 7))], 20: [('b', (4, 5))], 27: [('b', (6, 7))]},
    'first': {0: [('f', (0, 1))], 1: [('f', (2, 3))], 2: [('f', (4, 5))], 3: [('f', (6, 7)), ('n', (0, 1, 2, 3))],
              5: [('b', (0, 1))], 7: [('b', (2, 3)), ('n', (4, 5, 6, 7))], 9: [('b', (4, 5))], 12: [('b', (6, 7))]},
}
LN_EPS = 1e-5
DEN_EPS = 1e-6
C0 = math.sqrt(2.0 / math.pi)
C1 = 0.044715
F32, BF16, U32 = jnp.float32, jnp.bfloat16, jnp.uint32


def _nn(a, b):
    return lax.dot_general(a, b, (((1,), (0,)), ((), ())), preferred_element_type=F32)


def _nt(a, b):
    return lax.dot_general(a, b, (((1,), (1,)), ((), ())), preferred_element_type=F32)


def _tn(a, b):
    return lax.dot_general(a, b, (((0,), (0,)), ((), ())), preferred_element_type=F32)


def _tree(op, xs):
    xs = list(xs)
    while len(xs) > 1:
        nxt = [op(xs[i], xs[i + 1]) for i in range(0, len(xs) - 1, 2)]
        if len(xs) % 2:
            nxt.append(xs[-1])
        xs = nxt
    return xs[0]


def _rows8(a):
    return [a[8 * i:8 * i + 8] for i in range(a.shape[0] // 8)]


def _pair_reduce(op, rows):
    v = _tree(op, rows)
    v = op(v, pltpu.roll(v, 2, 0))
    return op(v, pltpu.roll(v, 4, 0))


def _softmax_pair(p):
    rows = _rows8(p)
    mx = _pair_reduce(jnp.maximum, rows)
    mn = _pair_reduce(jnp.minimum, rows)
    ep = [jnp.exp(r - mx) for r in rows]
    en = [jnp.exp(mn - r) for r in rows]
    rp = 1.0 / _pair_reduce(jnp.add, ep)
    rn = 1.0 / _pair_reduce(jnp.add, en)
    return jnp.concatenate([e * rp for e in ep] + [e * rn for e in en], axis=0)


def _softmax_pair_bwd(phi, dphi):
    pr, dr = _rows8(phi), _rows8(dphi)
    t = [a * b for a, b in zip(pr, dr)]
    sp = _pair_reduce(jnp.add, t[:7])
    sn = _pair_reduce(jnp.add, t[7:])
    out = [(t[i] - t[7 + i]) - (pr[i] * sp - pr[7 + i] * sn) for i in range(7)]
    return jnp.concatenate(out, axis=0)


def _pk(a):
    return pltpu.bitcast(a, U32)


def _up(a):
    return pltpu.bitcast(a, BF16)


def _cat(xs, axis=0):
    return jnp.concatenate(xs, axis=axis)


def _split(a):
    w = _pk(a)
    return [pltpu.unpack_elementwise(w, index=j, packed_dtype=BF16, unpacked_dtype=F32) for j in range(2)]


def _pack(e, o):
    return pltpu.pack_elementwise([e, o], packed_dtype=BF16)


def _pack16(a):
    r = _rows8(a)
    return _pack(_cat(r[0::2]), _cat(r[1::2]))


def _unpack16(w):
    e, o = [_rows8(pltpu.unpack_elementwise(w, index=j, packed_dtype=BF16, unpacked_dtype=F32)) for j in range(2)]
    return _cat([x for p in zip(e, o) for x in p])


def _bf(xs):
    return [a.astype(BF16) for a in xs]


def _combos(x11, x12, x21, x22):
    return [x11 + x22, x21 + x22, x11, x22, x11 + x12, x21 - x11, x12 - x22]


def _combos_t(x11, x12, x21, x22):
    return _combos(x11, x21, x12, x22)


def _uncombos(m):
    return (m[0] + m[3] - m[4] + m[6], m[2] + m[4], m[1] + m[3], m[0] - m[1] + m[2] + m[5])


def _uncombos_t(m):
    c11, c12, c21, c22 = _uncombos(m)
    return c11, c21, c12, c22


def _quarters(x):
    r, c = x.shape[0] // 2, x.shape[1] // 2
    return x[:r, :c], x[:r, c:], x[r:, :c], x[r:, c:]


def _join(x11, x12, x21, x22):
    return _cat([_cat([x11, x12], 1), _cat([x21, x22], 1)])


def _set_a(x):
    x11, x12, x21, x22 = _quarters(x)
    return [x11, x21, x12, x22, x11 + x12, x21 + x22, x11 + x22, x21 - x11, x12 - x22]


def _groups(x):
    n = x.shape[0] // 7
    return x[:4 * n], [x[(4 + j) * n:(5 + j) * n] for j in range(3)]


def _halves(x, axis=1):
    n = x.shape[axis] // 2
    return (x[:, :n], x[:, n:]) if axis else (x[:n], x[n:])


def _set_x(x):
    top, g = _groups(x)
    (l1, r1), (l2, r2), (l3, r3) = [_halves(a) for a in g]
    return _combos(*_quarters(top)) + [_cat([l2, r3]), _cat([r1, l2 + r2]), _cat([l1, l3 + r3])]


def _set_w(x):
    top, g = _groups(x)
    (l1, r1), (l2, r2), (l3, r3) = [_halves(a) for a in g]
    d1 = r1 - l1
    ext = [[], [r2, -r3], [l1, l2], [r1, r3], [-l2, l3], [d1, r2 - l2], [-d1, l3 - r3]]
    return [_cat([c] + e) for c, e in zip(_combos_t(*_quarters(top)), ext)]


def _set_f(x):
    top, g = _groups(x)
    (l1, r1), (l2, r2), (l3, r3) = [_halves(a) for a in g]
    return _combos_t(*_quarters(top)) + [_cat([l1, l2 - r2]), _cat([r1, r3 - l3]), _cat([r2, l3])]


def _wf_set(t):
    low = lax.broadcasted_iota(jnp.int32, (t[0].shape[0] // 2, 128), 1) < KG
    (a0, b0), (a1, b1), (a2, b2), (a3, b3) = [_halves(a, 0) for a in t]
    d2 = b2 - a2
    ext = [None, jnp.where(low, b3, -b3), a2, jnp.where(low, b2, b3), jnp.where(low, -a3, a3), d2,
           jnp.where(low, -d2, a3 - b3)]
    return [c if e is None else _cat([c, e], 1) for c, e in zip(_combos(a0, a1, b0, b1), ext)]


def _wb_set(t):
    low = lax.broadcasted_iota(jnp.int32, (t[0].shape[0] // 2, 128), 1) < KG
    (a0, b0), (a1, b1), (a2, b2), (a3, b3) = [_halves(a, 0) for a in t]
    a13, b13 = jnp.where(low, a2, a3), jnp.where(low, b2, b3)
    ext = [None, a13, b3, a3, b2, a13 + b13, a2 + b2]
    c = _combos_t(a0, a1, b0, b1)
    return [c[BORD[k]] if e is None else _cat([c[BORD[k]], e], 1) for k, e in enumerate(ext)]


def _unit(ref, idx, k, rows=DB // 2, n=1):
    return _up(ref[idx + (slice(rows * k, rows * (k + n)),)])


def _acc(ref, idx, first, val):
    ref[idx] = val if first else ref[idx] + val


TILES = ((0, 128), (128, 256), (256, 384), (320, 448))


def _kernel(xT_h, wqkv_h, wphi_h, wo_h, wg_h, wu_h, wdT_h, dyT_h,
            outT_h, dxT_h, dwqkv_h, dwphi_h, dwo_h, dwg_h, dwu_h, dwdT_h,
            xT_s, dyT_s, rstd_s, doT_s, xa_s, ya_s, xb_s, xbt_s, ybt_s, qs_s,
            wqkv_s, wphi_s, wo_s, wg_s, wu_s, wdT_s,
            wT_s, bd_s, wf_s, wb_s,
            wa_gu, wa_d, wb_gu, wb_d, tmpa_s, tmpb_s,
            hc_s, dguc_s, phik_s, vext_s, kv_acc, kvt_s, kv_s,
            out_acc, dxn_acc, dwgu_acc, dwd_acc, g_acc,
            fold_s, zero_s, dxn_s, out_st, dx_st, dwqkv_st, dwphi_st, dwo_st, dwg_st, dwu_st, dwd_st,
            sem):
    def cols(src, dst, lo, hi, k):
        return pltpu.make_async_copy(src.at[:, pl.ds(lo, hi - lo)], dst.at[:, pl.ds(lo, hi - lo)], sem.at[k])

    def x_copy(i, k):
        return pltpu.make_async_copy(xT_h.at[:, pl.ds(i * TS, TS)], xT_s.at[i], sem.at[k])

    def dy_copy(i, k):
        return pltpu.make_async_copy(dyT_h.at[:, pl.ds(i * TS, TS)], dyT_s.at[i], sem.at[k])

    def xy_in(i):
        return [dy_copy(i, i), x_copy(i, i)]

    def mlp_in(lo, hi, k, mats=slice(None)):
        return [cols(src, dst, lo, hi, k) for src, dst in ((wg_h, wg_s), (wu_h, wu_s), (wdT_h, wdT_s))[mats]]

    def mlp_out(chunks, k):
        lo, hi = chunks[0][0], chunks[-1][0] + chunks[-1][1]
        return [cols(src, dst, lo, hi, k) for src, dst in ((dwg_st, dwg_h), (dwu_st, dwu_h), (dwd_st, dwdT_h))]

    def tile_out(i, r=0, n=D):
        return [pltpu.make_async_copy(src.at[i, pl.ds(r, n)], dst.at[pl.ds(r, n), pl.ds(i * TS, TS)], sem.at[NT + 5])
                for src, dst in ((dx_st, dxT_h), (out_st, outT_h))]

    in_x = [x_copy(0, 0)]
    in_g = mlp_in(0, 256, NT, slice(0, 1))
    in_y = [dy_copy(0, NT + 7)]
    in_ud = mlp_in(0, 256, NT + 1, slice(1, 3))
    in_c1 = mlp_in(256, 512, NT + 2)
    in_kv = [pltpu.make_async_copy(wphi_h, wphi_s, sem.at[NT + 3]), cols(wqkv_h, wqkv_s, 384, 2 * D, NT + 3)]
    in_vo = [pltpu.make_async_copy(wo_h, wo_s, sem.at[NT + 6]), cols(wqkv_h, wqkv_s, 2 * D, 3 * D, NT + 6)]
    in_rest = [cols(wqkv_h, wqkv_s, 0, 384, NT + 4)] + mlp_in(512, DF, NT + 4)
    out_mlp = [mlp_out(g, NT + 5) for g in (CHUNKS[0], CHUNKS[1], CHUNKS[2][:1], CHUNKS[2][1:])]
    out_wqkv = [cols(dwqkv_st, dwqkv_h, lo, hi, NT + 5) for lo, hi in ((0, 384), (384, 2 * D), (2 * D, 3 * D))]
    c_dwphi = pltpu.make_async_copy(dwphi_st, dwphi_h, sem.at[NT + 5])
    c_dwo = pltpu.make_async_copy(dwo_st, dwo_h, sem.at[NT + 5])

    def start(cs):
        for c in cs:
            c.start()

    def wait(cs):
        for c in cs:
            c.wait()

    def tied(w, dep):
        return _up(w | _cat([dep] * (w.shape[0] // 8))).astype(F32)

    def tie(v):
        return lax.bitcast_convert_type(v[:8, :128], U32) & zero_s[...]

    def paced(marks, n, lo=0.0, hi=1.0):
        total, deps = sum(t for _, t in marks), []
        for j in range(n):
            pos = (lo + (hi - lo) * j / n) * total
            for v, t in marks:
                if pos < t:
                    break
                pos -= t
            deps.append(tie(v[8 * min(int(pos / t * (v.shape[0] // 8)), v.shape[0] // 8 - 1):]))
        return deps

    def unpack_paced(w, deps, order):
        if deps is not None:
            per = len(order) // len(deps)
            w = w | _cat([_cat([deps[order.index(j) // per]] * (w.shape[1] // 128), 1)
                          for j in range(len(order)) for _ in range(2)])
        return [pltpu.unpack_elementwise(w, index=j, packed_dtype=BF16, unpacked_dtype=F32) for j in range(2)]

    def held(a, dep):
        top = lax.bitcast_convert_type(a[:8], U32) | _cat([dep] * (a.shape[1] // 128), 1)
        top = lax.bitcast_convert_type(top, F32)
        return _cat([top, a[8:]]) if a.shape[0] > 8 else top

    def bd_consts(perm=False):
        def col(shape):
            c = lax.broadcasted_iota(jnp.int32, shape, 1)
            return (c & -16) + 2 * (c & 7) + ((c >> 3) & 1) if perm else c

        r = lax.broadcasted_iota(jnp.int32, (PF, PF), 0)
        c = col((PF, PF))
        row_head = ((r >= DH).astype(jnp.int32) + (r >= 2 * DH).astype(jnp.int32)
                    + (r >= 3 * DH).astype(jnp.int32))
        mask = row_head == 2 * (c >= PR).astype(jnp.int32) + (c & 1)
        sc = col((DH, PF))
        sr = lax.broadcasted_iota(jnp.int32, (DH, PF), 0)
        sel = jnp.where(((sc - PR * (sc >= PR).astype(jnp.int32)) >> 1) == sr, 1.0, 0.0).astype(BF16)
        return mask, sel

    def kv_operands(s):
        def source(p):
            return (p & -16) + ((p & 15) >> 1) + 8 * (p & 1)

        def restore(a):
            return _unpack16(_pk(a.astype(BF16))).astype(BF16)

        r = lax.broadcasted_iota(jnp.int32, (PE, PF), 0)
        c = source(lax.broadcasted_iota(jnp.int32, (PE, PF), 1))
        r = r if s else source(r)
        row_head = jnp.where(r < PR, (r >= DH).astype(jnp.int32), (r >= PR + 4).astype(jnp.int32))
        mask = row_head == (c & 1)
        for p in range(NP):
            m = jnp.where(mask, kv_acc[s, p], 0.0)
            rows, cols = (m.astype(BF16), _up(_pack16(m))) if s else (restore(m), restore(m))
            kvt_s[s, p] = _pk(rows)
            kv_s[s, p] = _pk(restore(cols.astype(F32).T))

    def untile(t):
        return _cat([t[0].T, t[1].T, t[2].T, t[3].T[KG:]])

    def prep_phi():
        tmpa_s[...] = wphi_s[...].astype(F32)
        for d in range(DH):
            tmpb_s[pl.ds(d, H, stride=DH), :] = tmpa_s[H * d:H * d + H, :]

    def prep_bd(perm):
        mask, sel = bd_consts(perm)
        expand = _nn(tmpb_s[...].astype(BF16), sel)
        for g in range(NG):
            bd_s[PF * g:PF * g + PF, :] = jnp.where(mask, expand[PF * g:PF * g + PF], 0.0).astype(BF16)

    def prep_wt(lo, hi):
        for j, (a, b) in enumerate(TILES):
            wT_s[lo // 2:hi // 2, 128 * j:128 * j + 128] = _pk(wqkv_s[a:b, lo:hi].T)

    def fold(t):
        w = _rows8(_cat([_tn(bd_s[PF * g:PF * g + PF, :], _unit(wT_s, (), NG * t + g, PR)) for g in range(NG)]))
        return [[v[:, 128 * j:128 * j + 128] for j in range(4)] for v in (_cat(w[0::2]), _cat(w[1::2]))]

    def store_set(ref, t, make, e, o):
        done = []
        for k, (p, q) in enumerate(zip(make(e), make(o))):
            w = _pack(p, q)
            ref[t, k, :, :p.shape[1]] = w
            done.extend(w[r:r + 8, -128:] for r in (0, 56, 104))
        return _tree(jnp.bitwise_or, done) & zero_s[...]

    def split_tiles(tiles, deps=None):
        return zip(*[unpack_paced(_pk(a), deps, RORD['a']) for a in tiles])

    def wunit(ref, t, k):
        return _up(ref[t, k, :, :256 if k else 128])

    def prep_qk(t):
        e, o = fold(t)
        store_set(wf_s, t, _wf_set, e, o)
        return [_up(_pack(p, q)) for p, q in zip(e, o)]

    def prep_qk_t(t, w, deps=None):
        return store_set(wb_s, t, _wb_set, *split_tiles([untile([c[a:b] for c in w]) for a, b in TILES], deps))

    def prep_v(deps=None):
        w = _unit(wT_s, (), 2, DB)
        store_set(wf_s, 2, _wf_set, *split_tiles([w[:, 128 * j:128 * j + 128] for j in range(4)], deps))

    def prep_v_t(deps=None):
        store_set(wb_s, 2, _wb_set, *split_tiles([wqkv_s[:, 2 * D + a:2 * D + b] for a, b in TILES], deps))

    def prep_wo(deps=None):
        store_set(wf_s, 3, _wf_set, *split_tiles([wo_s[:, a:b] for a, b in TILES], deps))

    def prep_wo_t(deps=None):
        return store_set(wb_s, 3, _wb_set, *split_tiles([wo_s[a:b, :].T for a, b in TILES], deps))

    def prep_mlp(chunks, mats, part, marks=None, lo=0.0, hi=1.0):
        items = [(ch, m) for ch in chunks for m in mats]
        deps = None if marks is None else paced(marks, 7 * len(items), lo, hi)
        for n, ((a, w), m) in enumerate(items):
            f = w // 2
            ref, off, wa, wb = {'g': (wg_s, a, wa_gu, wb_gu), 'u': (wu_s, a + f, wa_gu, wb_gu),
                                'd': (wdT_s, a // 2, wa_d, wb_d)}[m]
            e, o = unpack_paced(_pk(ref[:, a:a + w]), deps and deps[7 * n:7 * n + 7], RORD[part])
            if 'b' in part:
                for k, (p, q) in enumerate(zip(_set_w(e), _set_w(o))):
                    wb[k, :p.shape[0], off:off + f] = _pack(p, q)
            if 'a' in part:
                for k, (p, q) in enumerate(zip(_combos_t(*_quarters(e)), _combos_t(*_quarters(o)))):
                    wa[k, :, off:off + f] = _pack(p, q)

    def unfold_phi(gT, t):
        dphi, dwT = [], []
        low = lax.broadcasted_iota(jnp.int32, (PF, 512), 1)
        dup = (low >= 3 * 128) & (low < 3 * 128 + KG)
        for g in range(NG):
            r = slice(PF * g, PF * g + PF)
            dphi.append(_nt(jnp.where(dup, 0, _unit(wT_s, (), NG * t + g, PR)), gT[r]))
            dwT.append(_nn(bd_s[r, :], gT[r]).astype(BF16))
        return dphi, dwT

    def ragged(get, k, ext, axis):
        return get(k) if ext is None else _cat([get(k), get(ext)], axis)

    def project(w, xs, marks):
        m = {k: _nn(wunit(wf_s, w, k), ragged(xs, BORD[k], XEXT[k], 0)) for k in PORD}
        marks.extend((m[k], 2 if k else 1) for k in PORD)
        return _join(*_uncombos(m))

    def back_project(w, fs, k):
        return _nn(wunit(wb_s, w, k), ragged(lambda j: fs[j], k, FEXT[k], 0))

    def outer(w, a_s, i, fs, first):
        marks = []
        for k in range(7):
            marks.append((_nt(_unit(a_s, (i,), AORD[k]), fs[BORD[k]]), 1))
            _acc(g_acc, (w, slice(DB * k, DB * k + DB)), first, marks[-1][0])
        for k in range(3):
            marks.append((_nt(_unit(a_s, (i,), 2 * k, n=2), fs[7 + k]), 2))
            _acc(g_acc, (w, slice(DB * (7 + 2 * k), DB * (9 + 2 * k))), first, marks[-1][0])
        return marks

    def outer_result(w):
        c11, c12, c21, c22 = _uncombos([g_acc[w, DB * k:DB * k + DB] for k in range(7)])
        p = [g_acc[w, DB * (7 + 2 * k):DB * (9 + 2 * k)] for k in range(3)]
        low = lax.broadcasted_iota(jnp.int32, (D, 128), 1) < KG
        t = [_cat([c11, c21]), _cat([c12, c22]),
             p[0] + jnp.where(low, p[1], pltpu.roll(p[2], KG, 1)), p[1] + p[2]]
        return [a.astype(BF16) for a in t]

    def mlp_pre(bt_s, i, wb, a, w, k, h=None):
        lhs = ragged(lambda j: _unit(bt_s, (i,), j, 64) if h is None else _unit(bt_s, (i,), 2 * j + h, 32),
                     BORD[k], XEXT[k], 1)
        return _nn(lhs, _up(wb[k, :128 if k else 64, a:a + w]))

    def mlp_gu(i, ch, k, h):
        return mlp_pre(xbt_s, i, wb_gu, ch[0], ch[1], k, h)

    def mlp_dh(i, ch, k, h):
        return mlp_pre(ybt_s, i, wb_d, ch[0] // 2, ch[1] // 2, k, h)

    def mlp_s1(i, n, ch, gum=None, split=True):
        for h in range(2) if gum is None and split else (None,):
            mlp_half(i, n, ch, h, gum)

    def mlp_half(i, n, ch, half, gum=None, dhm=None):
        gum, dhm = dict(gum or {}), dict(dhm or {})
        for k in PORD:
            if k not in dhm:
                dhm[k] = mlp_dh(i, ch, k, half)
            if k not in gum:
                gum[k] = mlp_gu(i, ch, k, half)
        f = ch[1] // 2
        hs, dgus = [], []
        for gu, dh in zip(_uncombos_t(gum), _uncombos_t(dhm)):
            g, u = gu[:, :f], gu[:, f:]
            g2 = g * g
            s = 0.5 * jnp.tanh(g * (C0 + (C0 * C1) * g2)) + 0.5
            gelu = g * s
            dgelu = s + gelu * (1.0 - s) * (2.0 * C0 + (6.0 * C0 * C1) * g2)
            hs.append(gelu * u)
            dgus.append(_cat([dh * u * dgelu, dh * gelu], 1))
        for k, (h, dgu) in enumerate(zip(_combos(*hs), _combos(*dgus))):
            r = slice(None) if half is None else slice(32 * half, 32 * half + 32)
            hc_s[k, r, f * n:f * n + f] = pack_tokens(h)
            dguc_s[k, r, 2 * f * n:2 * f * n + 2 * f] = pack_tokens(dgu)

    def pack_tokens(a):
        r = _rows8(a)
        return _pack(_cat([x for j, x in enumerate(r) if not j & 2]), _cat([x for j, x in enumerate(r) if j & 2]))

    def mlp_out_p(chunks, k):
        a, w = chunks[0][0], sum(c[1] for c in chunks)
        return _nt(_up(wa_d[BORD[k], :, a // 2:(a + w) // 2]), _up(hc_s[k, :, :w // 2]))

    def mlp_dx_p(chunks, k):
        a, w = chunks[0][0], sum(c[1] for c in chunks)
        return _nt(_up(wa_gu[BORD[k], :, a:a + w]), _up(dguc_s[k, :, :w]))

    def mlp_s2b(i, n, ch, mode, hooks={}, holds={}):
        a, w = ch
        marks = []
        f = w // 2
        for a_s, src, acc, wd, dsts in ((ya_s, hc_s, dwd_acc, f, (dwd_st,)),
                                        (xa_s, dguc_s, dwgu_acc, w, (dwg_st, dwu_st))):
            m = []
            for k in range(7):
                v = _nn(_unit(a_s, (i,), AORD[k]), _up(src[BORD[k], :, wd * n:wd * n + wd]))
                idx = (k, slice(None), slice(wd * n, wd * n + wd))
                marks.append((v, wd // 128))
                if len(marks) in hooks:
                    hooks[len(marks)](marks)
                if len(marks) in holds:
                    v = held(v, holds[len(marks)])
                if mode == 'last':
                    m.append(acc[idx] + v)
                else:
                    _acc(acc, idx, mode == 'first', v)
            if mode == 'last':
                q = _uncombos(m)
                for j, dst in enumerate(dsts):
                    dst[:, a:a + w] = _join(*[v[:, f * j:f * j + f] for v in q]).astype(BF16)
        return marks

    def store_sets(i, e, o, a_s, bt_s):
        b = [_pack(p, q) for p, q in zip(_set_x(e), _set_x(o))]
        for k, w in enumerate(b):
            p, q = [_rows8(_pk(v.astype(BF16))) for v in _split(_up(w).T)]
            bt_s[i, 64 * k:64 * k + 64] = _cat([x for pair in zip(p, q) for x in pair])
        a_s[i, :9 * DB // 2] = _cat([_pack(p, q) for p, q in zip(_set_a(e), _set_a(o))])
        return b

    def dy_sets(i, deps=None):
        return [_up(w) for w in store_sets(i, *unpack_paced(_pk(dyT_s[i]), deps, RORD['ab']), ya_s, ybt_s)]

    def all_rows(v):
        v = _tree(jnp.add, _rows8(v))
        return _pair_reduce(jnp.add, [v + pltpu.roll(v, 1, 0)])

    def layernorm(i, deps=(None, None, None)):
        w = _pk(xT_s[i])
        e, o = unpack_paced(w, deps[0], RORD['n'])
        mean = _cat([all_rows(e + o) * (1.0 / D)] * (DB // 8))
        e, o = [v - mean for v in unpack_paced(w, deps[1], RORD['n'])]
        rstd = lax.rsqrt(all_rows(e * e + o * o) * (1.0 / D) + LN_EPS)
        rstd_s[i, 0:8] = rstd
        rstd = _cat([rstd] * (DB // 8))
        e, o = [(v - mean) * rstd for v in unpack_paced(w, deps[2], RORD['ab'])]
        xb_s[i] = _cat(store_sets(i, e, o, xa_s, xbt_s))

    def xproj(i, t, marks=None):
        return project(t, lambda k: _unit(xb_s, (i,), k, 64), [] if marks is None else marks)

    def do_proj(i, yb, marks=None):
        doT_s[i] = _pack16(project(3, lambda k: yb[k], [] if marks is None else marks))

    def key_side(i, pk, v, first, deps=None):
        ones = jnp.ones((8, TS), F32)
        for c in range(NP):
            p = pk[PR * c:PR * c + PR]
            phik = _pack16(_softmax_pair(p if deps is None else held(p, deps[c])))
            phik_s[i, PR * c:PR * c + PR, :] = phik
            vext = _pack16(_cat([v[PR * c:PR * c + PR], ones]))
            vext_s[i, 32 * c:32 * c + 32, :] = vext
            _acc(kv_acc, (0, c), first, _nt(_up(vext), _up(phik)))

    def phase1_tail(i):
        mo = [mlp_out_p(CHUNKS[0], k) for k in range(7)]
        mdx = [mlp_dx_p(CHUNKS[0], k) for k in range(7)]
        for k, (o, dx) in enumerate(zip(mo, mdx)):
            out_acc[i, k] = o
            dxn_acc[i, k] = dx
        return [(o, 1) for o in mo] + [(dx, 2) for dx in mdx]

    c0, c1 = CHUNKS[0]
    start(in_x + in_g + in_y + in_ud + in_c1 + in_kv + in_vo)
    for i in range(1, NT):
        start(xy_in(i))
    start(in_rest)
    wait(in_x)
    zero_s[...] = (_pk(xT_s[0, 0:16, 0:128]) >> 16) >> 16
    layernorm(0)
    wait(in_g)
    prep_mlp([c0], 'g', 'ab')
    wait(in_y)
    g = {k: mlp_pre(xbt_s, 0, wb_gu, 0, 128, k) for k in PORD}
    yb = dy_sets(0)
    wait(in_ud)
    prep_mlp([c0], 'ud', 'b')
    gu = {k: _cat([g[k], mlp_pre(xbt_s, 0, wb_gu, 128, 128, k)], 1) for k in PORD}
    mlp_s1(0, 0, c0, gu)

    def next_chunk(marks):
        prep_mlp([c0], 'ud', 'a', marks, 0.0, 0.9)
        wait(in_c1)

    marks = mlp_s2b(0, 0, c0, 'first', {10: next_chunk})
    prep_mlp([c1], 'dgu', 'b', marks[10:])
    mlp_s1(0, 1, c1)
    folded = []

    def attn_prep(marks):
        prep_mlp([c1], 'd', 'a', marks, 0.0, 0.8)
        wait(in_kv)
        prep_phi()
        prep_wt(384, 2 * D)

    marks = mlp_s2b(0, 1, c1, 'first', {7: attn_prep, 10: lambda m: prep_bd(True),
                                        12: lambda m: folded.extend(prep_qk(1))})
    prep_mlp([c1], 'gu', 'a', marks[7:])
    wait(in_vo)
    marks = []
    pk = xproj(0, 1, marks)
    prep_wt(2 * D, 3 * D)
    prep_wo(paced(marks, 7, 0.0, 0.5))
    prep_v(paced(marks, 7, 0.5))
    marks = []
    do_proj(0, yb, marks)
    v = xproj(0, 2, marks)
    key_side(0, pk, v, True, paced(marks, NP, 0.0, 0.8))
    fold_s[...] = _pk(_cat(folded, 1))

    def phase1(i, mode):
        marks = phase1_tail(i - 1)
        yb = dy_sets(i, paced(marks, 14, 0.0, 0.3))
        layernorm(i, (paced(marks, 7, 0.3, 0.42), paced(marks, 7, 0.44, 0.58), paced(marks, 14, 0.6, 1.0)))
        if mode == 'last':
            prep_mlp(CHUNKS[1], 'd', 'a', marks)
        do_proj(i, yb)
        mlp_s1(i, 0, c0)
        pk = xproj(i, 1)
        mlp_s1(i, 1, c1, split=mode != 'mid')
        marks = []
        v = xproj(i, 2, marks)
        if mode == 'last':
            prep_mlp(CHUNKS[1][:1], 'gu', 'a', marks, 0.4)
            prep_wt(0, 384)
            folded[:] = prep_qk(0)
        marks = mlp_s2b(i, 0, c0, mode)
        key_side(i, pk, v, False, paced(marks, NP, 0.0, 0.8) if mode == 'mid' else None)
        mlp_s2b(i, 1, c1, mode)

    def loop(f, unroll, pre=None, post=None):
        def body(j, carry):
            tiles = [1 + unroll * j + n for n in range(unroll)]
            for g in (pre, lambda i: f(i, 'mid'), post):
                for i in tiles if g else ():
                    g(i)
            return carry
        lax.fori_loop(0, (NT - 2) // unroll, body, 0)

    loop(phase1, 1, pre=lambda i: wait(xy_in(i)))
    wait(in_rest + xy_in(NT - 1))
    phase1(NT - 1, 'last')
    kv_operands(0)
    prep_mlp(CHUNKS[1], 'dgu', 'b', phase1_tail(NT - 1))

    class Query:
        def __init__(self, i, first=False, marks=None):
            self.i, self.first = i, first
            self.pq = xproj(i, 0, marks)
            self.phi, self.ne, self.o, self.dp = {}, {}, {}, {}

        def fwd(self, cs, deps):
            for c, dep in zip(cs, deps):
                self.phi[c] = _up(_pack16(_softmax_pair(held(self.pq[PR * c:PR * c + PR], dep))))

        def num(self, cs):
            for c in cs:
                self.ne[c] = _rows8(_nn(_up(kvt_s[0, c]), self.phi[c]))

        def bwd(self, cs):
            lo4 = lax.broadcasted_iota(jnp.int32, (8, TS), 0) < 4
            dne = {}
            for c in cs:
                ne, r0 = self.ne[c], PR * c // 16 * 8
                do = _unpack16(doT_s[self.i, r0:r0 + 32])[PR * c % 16:PR * c % 16 + PR]
                r = 1.0 / (ne[7] + DEN_EPS)
                rr = pltpu.roll(r, 4, 0)
                ra = jnp.where(lo4, r, rr)
                rb = jnp.where(lo4, rr, r)
                rs = [ra, ra, ra, r, rb, rb, rb]
                o = [n * w for n, w in zip(ne[:7], rs)]
                dnum = [n * w for n, w in zip(_rows8(do), rs)]
                t = [a * b for a, b in zip(dnum, o)]
                sa = t[0] + t[1] + t[2]
                sb = t[4] + t[5] + t[6]
                e = jnp.where(lo4, sa, sb) + pltpu.roll(jnp.where(lo4, sb, sa), 4, 0) + t[3]
                dne[c] = _cat(dnum + [-e]).astype(BF16)
                self.o[c] = _cat(o)
            for c in cs:
                self.dp[c] = _softmax_pair_bwd(_unpack16(_pk(self.phi[c])), _nn(_up(kv_s[0, c]), dne[c]))
            for c in cs:
                _acc(kv_acc, (1, c), self.first, _nt(dne[c], self.phi[c]))

        def sets(self):
            return [_bf(_set_f(_cat([v[c] for c in range(NP)]))) for v in (self.o, self.dp)]

        def store(self):
            done = []
            for j, st in enumerate(self.sets()):
                qs_s[j] = _pk(_cat(st))
                done.extend(_tree(jnp.bitwise_or, _rows8(_pk(a))) for a in st)
            return done

        def after(self, done, n):
            return [_tree(jnp.bitwise_or, done[j::n]) & zero_s[...] for j in range(n)]

    def phase2(i, mode):
        first = mode == 'first'
        ch = CHUNKS[1]

        def s1(n):
            mlp_s1(i, n, ch[n])

        s1(0)
        if first:
            q = Query(i, True)
            marks = mlp_s2b(i, 0, ch[0], mode)
            for c, dep in enumerate(paced(marks, NP, 0.0, 0.8)):
                q.fwd([c], [dep])
                q.num([c])
            s1(1)
            for c in range(0, NP, 2):
                q.bwd((c, c + 1))
            marks = mlp_s2b(i, 1, ch[1], mode, holds={14: prep_qk_t(0, folded)})
            deps = paced(marks, 14, 0.45, 0.95)
            for c in range(NP):
                q.o[c] = _cat([held(o, deps[RORD['b'].index((7 * c + j) // 4)]) for j, o in enumerate(_rows8(q.o[c]))])
            s1(2)
            ob, dpb = q.sets()
            marks = outer(3, ya_s, i, ob, first)
            marks += outer(0, xa_s, i, dpb, first)
        else:
            ob, dpb = [[_unit(qs_s, (j,), k, 64) for k in range(10)] for j in range(2)]
            s1(1)
            s1(2)
        if mode == 'last':
            mlp_s2b(i, 0, ch[0], mode)
            kv_operands(1)
            prep_bd(False)
            plan = {}
        else:
            q = Query(i + 1, marks=marks if first else None)
            plan = QPLAN[mode]
            if first:
                prep_mlp(ch[1:], 'gu', 'a', marks, 0.25, 0.9)
        marks, holds = [], {}

        def step(n):
            for op, cs in plan.get(n, ()):
                if op == 'f':
                    q.fwd(cs, paced(marks[-1:], len(cs)))
                else:
                    (q.num if op == 'n' else q.bwd)(cs)

        for k in range(7):
            acc = held(dxn_acc[i, k], prep_wo_t()) if first and k == 5 else dxn_acc[i, k]
            marks.append((acc + mlp_dx_p(ch, k) + back_project(0, dpb, k), 8))
            dxn_acc[i, k] = marks[-1][0]
            step(k)
        for k in range(7):
            marks.append((out_acc[i, k] + mlp_out_p(ch, k) + back_project(3, ob, k), 5))
            out_acc[i, k] = marks[-1][0]
            step(7 + k)
        if not first:
            outer(3, ya_s, i, ob, first)
            outer(0, xa_s, i, dpb, first)
        if mode == 'last':
            prep_mlp(CHUNKS[2], 'dgu', 'ab', marks, 0.0, 0.78)
            prep_v_t(paced(marks, 7, 0.78, 0.89))
            prep_qk_t(1, [_up(fold_s[:, 128 * j:128 * j + 128]) for j in range(4)], paced(marks, 7, 0.89))
        for n in range({'first': 2, 'mid': 0, 'last': 1}[mode], 3):
            if n == 2 and mode != 'last':
                at = range(10, 15) if first else range(4, 14)
                holds = dict(zip(at, q.after(q.store(), len(at))))
            mlp_s2b(i, n, ch[n], mode, {j: lambda m, j=j: step(14 * n + 13 + j) for j in range(1, 15)}, holds)

    phase2(0, 'first')
    start(out_mlp[0])
    loop(phase2, 1)
    phase2(NT - 1, 'last')

    def key_bwd(i):
        dv_all, dp_all = [], []
        for cs in ((c, c + 1) for c in range(0, NP, 2)):
            phik = {c: _up(phik_s[i, PR * c:PR * c + PR, :]) for c in cs}
            for c in cs:
                dphik = _nn(_up(kv_s[1, c]), _up(vext_s[i, 32 * c:32 * c + 32, :]))
                dp_all.append(_softmax_pair_bwd(_unpack16(_pk(phik[c])), dphik))
            for c in cs:
                dv_all.append(_nn(_up(kvt_s[1, c]), phik[c])[0:PR])
        return _bf(_set_f(_cat(dp_all))), _bf(_set_f(_cat(dv_all)))

    def dx_products(i, dkb, dvb, deps={}, hooks={}):
        m = {}
        for k in PORD:
            acc = held(dxn_acc[i, k], deps[k]) if k in deps else dxn_acc[i, k]
            m[k] = acc + back_project(2, dvb, k) + back_project(1, dkb, k) + mlp_dx_p(CHUNKS[2], k)
            if k in hooks:
                hooks[k]()
        return m

    def rows_of(a_s, i, r, n, dep):
        return _cat([tied(a_s[i, DB * h + r // 2:DB * h + (r + n) // 2], dep) for h in range(2)], 1)

    def finish_dx(i, m, marks, upper_done=None):
        q = _uncombos_t(m)
        s1, s2 = [None, None], [None, None]
        for j in (1, 2, 0, 3):
            h = j & 1
            for r in range(0, DB, 32):
                d = q[j][r:r + 32]
                dxn_s[DB * (j >> 1) + r:DB * (j >> 1) + r + 32, SB * h:SB * h + SB] = d
                t1 = _tree(jnp.add, _rows8(d))
                w = DB * h + (DB * (j >> 1) + r) // 2
                t2 = _tree(jnp.add, _rows8(d * tied(xa_s[i, w:w + 16], tie(t1 if s2[h] is None else s2[h]))))
                s1[h], s2[h] = (t1, t2) if s1[h] is None else (s1[h] + t1, s2[h] + t2)
        m1, m2 = [_cat([all_rows(v) * (1.0 / D)] * 2) for v in (_cat(s1, 1), _cat(s2, 1))]
        rstd = _cat([rstd_s[i, 0:8]] * 2)
        for r, dep in zip(range(0, D, 16), paced(marks, D // 16)):
            t = dxn_s[r:r + 16] - (rows_of(xa_s, i, r, 16, dep) * m2 + m1)
            t = rows_of(ya_s, i, r, 16, dep) + rstd * t
            dx_st[i, r:r + 16] = t.astype(BF16)
            if upper_done and r + 16 == DB:
                upper_done()

    def finish_out(i):
        m = {k: out_acc[i, k] + mlp_out_p(CHUNKS[2], k) for k in TORD}
        q = _uncombos_t(m)

        def store(h):
            r = slice(DB * h, DB * h + DB)
            out_st[i, r] = (xT_s[i, r].astype(F32) + _cat(q[2 * h:2 * h + 2], 1)).astype(BF16)

        return [(m[k], 1) for k in TORD], store

    def phase3(i, mode, extra=None):
        first = mode == 'first'
        ch = CHUNKS[2]
        mlp_s1(i, 0, ch[0])
        dkb, dvb = key_bwd(i)
        mlp_s1(i, 1, ch[1])
        outer(2, xa_s, i, dvb, first)
        outer(1, xa_s, i, dkb, first)
        m = dx_products(i, dkb, dvb)
        store = finish_out(i)[1]
        store(0)
        store(1)
        if extra:
            extra()
        marks = mlp_s2b(i, 0, ch[0], mode)
        mlp_s2b(i, 1, ch[1], mode)
        finish_dx(i, m, marks)

    def tiles_t(t):
        return _cat([untile([a[lo:hi] for a in t]) for lo, hi in TILES], 1)

    query_grads = []

    def unfold_query():
        dphi, dwT = unfold_phi(tiles_t(outer_result(0)), 0)
        dwT = _cat(dwT)
        dwqkv_st[:, 0:384] = untile([dwT[:384, 128 * j:128 * j + 128] for j in range(4)])
        query_grads.extend((dphi, dwT[384:]))

    phase3(0, 'first', unfold_query)
    dphi_q, dwT_q = query_grads
    dwo_t = outer_result(3)
    dwo_st[...] = _cat([a.T for a in dwo_t[:3]] + [dwo_t[3].T[KG:]])
    start(out_mlp[1] + [c_dwo] + tile_out(0) + out_wqkv[:1])
    loop(phase3, 2, post=lambda i: start(tile_out(i)))

    i = NT - 1
    ch = CHUNKS[2]
    dkb, dvb = key_bwd(i)
    mlp_s1(i, 0, ch[0])
    mlp_s1(i, 1, ch[1])
    outer(1, xa_s, i, dkb, False)
    outer(2, xa_s, i, dvb, False)
    gv = outer_result(2)
    dwqkv_st[:, 2 * D:3 * D] = _cat(gv[:3] + [gv[3][:, KG:]], 1)
    start(out_wqkv[2:])
    dphi_k, dwT_k = unfold_phi(tiles_t(outer_result(1)), 1)
    mask, sel = bd_consts()
    dg = [jnp.where(mask, dphi_q[g] + dphi_k[g], 0.0).astype(BF16) for g in range(NG)]
    ready = _tree(jnp.bitwise_or, [w for a in dg for w in _rows8(_pk(a))])
    mlp_s2b(i, 0, ch[0], 'last', holds={10: _cat([ready, zero_s[:, :128 - PF]], 1) & zero_s[...]})
    start(out_mlp[2])
    dwT = _cat([dwT_q] + dwT_k)
    dwk = untile([dwT[:, 128 * j:128 * j + 128] for j in range(4)])
    dwqkv_st[:, 384:2 * D] = dwk
    done = [_pk(dwk[r - 16:r, 128 * j:128 * j + 128]) for j in range(4) for r in (128, 256, 384, 448)]
    for g in range(NG):
        tmpa_s[PF * g:PF * g + PF, :] = _nt(dg[g], sel)
    for d in range(DH):
        dwphi_st[H * d:H * d + H, :] = tmpa_s[pl.ds(d, H, stride=DH), :].astype(BF16)
    mlp_s2b(i, 1, ch[1], 'last', holds={12: _tree(jnp.bitwise_or, done) & zero_s[...]})
    start([out_wqkv[1]] + out_mlp[3] + [c_dwphi])
    m = dx_products(i, dkb, dvb)
    marks, store = finish_out(i)
    store(0)
    finish_dx(i, m, marks[1:6], lambda: start(tile_out(i, 0, DB)))
    store(1)
    start(tile_out(i, DB, DB))

    wait(sum(out_mlp, []) + out_wqkv + [c_dwo, c_dwphi])
    for i in range(NT - 1):
        wait(tile_out(i))
    wait(tile_out(NT - 1, 0, DB) + tile_out(NT - 1, DB, DB))


@jax.jit
def pallas_parallel_sum__linear_kernel_hedgehog__glu_gated_geglu__prompt_kernel(
    A_x: jax.Array,
    A_wqkv: jax.Array,
    A_w_phi: jax.Array,
    A_wo: jax.Array,
    B_x: jax.Array,
    B_w_gate: jax.Array,
    B_w_up: jax.Array,
    B_w_down: jax.Array,
    grad_out: jax.Array,
):
    del B_x
    xT = A_x.reshape(S, D).T
    dyT = grad_out.reshape(S, D).T
    wphi2 = A_w_phi.transpose(1, 0, 2).reshape(D, DH)
    wdT = B_w_down.T

    V = pltpu.VMEM
    dma = pltpu.SemaphoreType.DMA
    scratch = [
        V((NT, D, TS), BF16), V((NT, D, TS), BF16),
        V((NT, 32, TS), F32), V((NT, DB, TS), U32),
        V((NT, 1024, SB), U32), V((NT, 1024, SB), U32),
        V((NT, 640, SB), U32), V((NT, 640, 128), U32), V((NT, 640, 128), U32),
        V((2, 640, SB), U32),
        V((D, 3 * D), BF16), V((D, DH), BF16), V((D, D), BF16),
        V((D, DF), BF16), V((D, DF), BF16), V((D, DF), BF16),
        V((3 * DB, 512), U32), V((D, PF), BF16),
        V((4, 7, DB // 2, 256), U32), V((4, 7, DB // 2, 256), U32),
        V((7, DB // 2, DF), U32), V((7, DB // 2, DF // 2), U32),
        V((7, 128, DF), U32), V((7, 128, DF // 2), U32),
        V((D, DH), F32), V((D, DH), F32),
        V((7, SB // 2, 384), U32), V((7, SB // 2, 768), U32),
        V((NT, NP * PR, TS), U32), V((NT, NP * 32, TS), U32),
        V((2, NP, PE, PF), F32), V((2, NP, PE // 2, PF), U32), V((2, NP, PR, PE), U32),
        V((NT, 8, DB, SB), F32), V((NT, 8, DB, SB), F32),
        V((7, DB, 768), F32), V((7, DB, 384), F32),
        V((4, 13 * DB, 128), F32),
        V((DB, 512), U32), V((8, 128), U32), V((D, TS), F32),
        V((NT, D, TS), BF16), V((NT, D, TS), BF16),
        V((D, 3 * D), BF16), V((D, DH), BF16), V((D, D), BF16),
        V((D, DF), BF16), V((D, DF), BF16), V((D, DF), BF16),
        dma((NT + 8,)),
    ]
    sds = jax.ShapeDtypeStruct
    out_shape = (
        sds((D, S), BF16), sds((D, S), BF16), sds((D, 3 * D), BF16), sds((D, DH), BF16),
        sds((D, D), BF16), sds((D, DF), BF16), sds((D, DF), BF16), sds((D, DF), BF16),
    )
    any_spec = pl.BlockSpec(memory_space=pl.ANY)
    outT, dxT, dwqkv, dwphi2, dwo, dwg, dwu, dwdT = pl.pallas_call(
        _kernel,
        out_shape=out_shape,
        in_specs=[any_spec] * 8,
        out_specs=[any_spec] * 8,
        scratch_shapes=scratch,
        compiler_params=pltpu.CompilerParams(vmem_limit_bytes=120 * 1024 * 1024),
        name="hedgehog_geglu",
    )(xT, A_wqkv, wphi2, A_wo, B_w_gate, B_w_up, wdT, dyT)
    return (
        outT.T.reshape(1, S, D),
        dxT.T.reshape(1, S, D),
        dwqkv,
        dwphi2.reshape(DH, H, DH).transpose(1, 0, 2),
        dwo,
        dwg,
        dwu,
        dwdT.T,
    )
```
